```python
import jax
import jax.numpy as jnp

def _softmax(x, axis=-1):
    return jax.nn.softmax(x, axis=axis)

def _gelu(x):
    return jax.nn.gelu(x, approximate=True)

def _silu(x):
    return jax.nn.silu(x)

def _sigmoid(x):
    return jax.nn.sigmoid(x)

def _layernorm(x, axis=-1, eps=1e-05):
    m = jnp.mean(x, axis=axis, keepdims=True)
    v = jnp.var(x, axis=axis, keepdims=True)
    return (x - m) / jnp.sqrt(v + eps)

def _scatter_add(tgt, idx, src, axis=0):
    return tgt.at[idx].add(src)

def _segment_sum(src, seg, n):
    return jax.ops.segment_sum(src, seg, n)

class _Rng:

    def __init__(self, key):
        self._k = key

    def _next(self):
        self._k, sub = jax.random.split(self._k)
        return sub

    def normal(self, shape):
        return jax.random.normal(self._next(), shape, dtype=jnp.bfloat16)

    def randint(self, lo, hi, shape):
        return jax.random.randint(self._next(), shape, lo, hi, dtype=jnp.int32)

    def uniform(self, shape, lo=0.0, hi=1.0):
        return jax.random.uniform(self._next(), shape, jnp.bfloat16, lo, hi)

    def permutation(self, n):
        return jax.random.permutation(self._next(), n)
kernel_name = 'concat_heads__memory_aug_recurrent_mem_tr__compressed_kv_cla__prompt'

def setup_inputs():
    _rng = _Rng(jax.random.key(int.from_bytes(__import__("os").urandom(4), "little")))
    _w = lambda a: (lambda t: t.astype(jnp.bfloat16) if jnp.issubdtype(t.dtype, jnp.floating) else t)(jnp.asarray(a))

    def _A_setup():
        B, S, Dm = (1, 2048, 448)
        H, Dh = (16, 256)
        M, seg = (8, 32)
        seg = min(seg, S)
        S = S // seg * seg
        return {'x': _w((lambda *s: _rng.normal(s) * 0.05)(B, S, Dm)), 'mem0': _w((lambda *s: _rng.normal(s) * 0.05)(B, M, Dm)), 'Wq': _w((lambda *s: _rng.normal(s) * 0.05)(Dm, H, Dh) * Dm ** (-0.5)), 'Wk': _w((lambda *s: _rng.normal(s) * 0.05)(Dm, H, Dh) * Dm ** (-0.5)), 'Wv': _w((lambda *s: _rng.normal(s) * 0.05)(Dm, H, Dh) * Dm ** (-0.5)), 'Wo': _w((lambda *s: _rng.normal(s) * 0.05)(H, Dh, Dm) * (H * Dh) ** (-0.5)), 'seg_len': seg}
    _A_in = _A_setup()

    def _B_setup():
        B, H, Sq, Sk, D, M = (1, 16, 2048, 2048, 256, 448)
        Dc = 4 * D
        return {'x': _w((lambda *s: _rng.normal(s) * 0.05)(B, Sq, M)), 'c_kv': _w((lambda *s: _rng.normal(s) * 0.05)(B, Sk, Dc)), 'w_q': _w((lambda *s: _rng.normal(s) * 0.05)(M, H, D) * M ** (-0.5)), 'w_uk': _w((lambda *s: _rng.normal(s) * 0.05)(Dc, H, D) * Dc ** (-0.5)), 'w_uv': _w((lambda *s: _rng.normal(s) * 0.05)(Dc, H, D) * Dc ** (-0.5)), 'w_o': _w((lambda *s: _rng.normal(s) * 0.05)(H, D, M) * (H * D) ** (-0.5))}
    _B_in = _B_setup()
    return {'A_x': _A_in['x'], 'A_mem0': _A_in['mem0'], 'A_Wq': _A_in['Wq'], 'A_Wk': _A_in['Wk'], 'A_Wv': _A_in['Wv'], 'A_Wo': _A_in['Wo'], 'A_seg_len': _A_in['seg_len'], 'B_x': _B_in['x'], 'B_c_kv': _B_in['c_kv'], 'B_w_q': _B_in['w_q'], 'B_w_uk': _B_in['w_uk'], 'B_w_uv': _B_in['w_uv'], 'B_w_o': _B_in['w_o']}

def reference(A_x, A_mem0, A_Wq, A_Wk, A_Wv, A_Wo, A_seg_len, B_x, B_c_kv, B_w_q, B_w_uk, B_w_uv, B_w_o):

    def _A_ref(x, mem0, Wq, Wk, Wv, Wo, seg_len):
        B, S, Dm = x.shape
        H, Dh = (Wq.shape[1], Wq.shape[2])
        M = mem0.shape[1]
        scale = Dh ** (-0.5)
        n_seg = S // seg_len
        L = M + seg_len
        idx = jnp.arange(L)
        mask = (idx[:, None] < M) | (idx[:, None] >= idx[None, :])
        mem = mem0
        outs = []
        for s in range(n_seg):
            xs = x[:, s * seg_len:(s + 1) * seg_len, :].copy()
            h = jnp.concatenate([mem, xs], axis=1)
            q = jnp.einsum('btd,dhe->bhte', h, Wq)
            k = jnp.einsum('btd,dhe->bhte', h, Wk)
            v = jnp.einsum('btd,dhe->bhte', h, Wv)
            scores = jnp.einsum('bhqe,bhke->bhqk', q, k) * scale
            scores = jnp.where(mask[None, None], scores, -1000000000.0)
            p = _softmax(scores, axis=-1)
            o = jnp.einsum('bhqk,bhke->bhqe', p, v)
            o = jnp.einsum('bhte,hed->btd', o, Wo)
            mem = o[:, :M, :].copy()
            outs.append(o[:, M:, :])
        return jnp.concatenate(outs, axis=1)

    def _B_ref(x, c_kv, w_q, w_uk, w_uv, w_o):
        B, Sq, M = (x.shape[0], x.shape[1], x.shape[2])
        Sk = c_kv.shape[1]
        H, D = (w_q.shape[1], w_q.shape[2])
        q = jnp.einsum('bqm,mhd->bhqd', x, w_q)
        k = jnp.einsum('bkc,chd->bhkd', c_kv, w_uk)
        v = jnp.einsum('bkc,chd->bhkd', c_kv, w_uv)
        scores = jnp.einsum('bhqd,bhkd->bhqk', q, k) * D ** (-0.5)
        off = Sk - Sq
        qi = jnp.arange(Sq)[:, None]
        kj = jnp.arange(Sk)[None, :]
        cmask = kj <= qi + off
        scores = jnp.where(cmask[None, None], scores, -1000000000.0)
        p = _softmax(scores, axis=-1)
        ctx = jnp.einsum('bhqk,bhkd->bhqd', p, v)
        return jnp.einsum('bhqd,hdm->bqm', ctx, w_o)
    a = _A_ref(A_x, A_mem0, A_Wq, A_Wk, A_Wv, A_Wo, A_seg_len)
    b = _B_ref(B_x, B_c_kv, B_w_q, B_w_uk, B_w_uv, B_w_o)
    return jnp.concatenate([a, b], axis=-1)
```

```python
import functools

import jax
import jax.numpy as jnp
from jax import lax
from jax.experimental import pallas as pl
from jax.experimental.pallas import tpu as pltpu

BF = jnp.bfloat16
F32 = jnp.float32
U32 = jnp.uint32
NT = (((1,), (1,)), ((), ()))
NEG = -1000000000.0


def _bf(x32):
    return pltpu.bitcast(x32, BF)


def _u32(xb):
    return pltpu.bitcast(xb, U32)


def _dot(a, b):
    return jnp.dot(a, b, preferred_element_type=F32)


def _dot_nt(a, b):
    return lax.dot_general(a, b, NT, preferred_element_type=F32)


def _deint(raw32, j, nrows):
    ev = raw32[pl.ds(j, nrows // 2, stride=16), :]
    od = raw32[pl.ds(j + 8, nrows // 2, stride=16), :]
    lo = (ev & jnp.uint32(0xFFFF)) | (od << 16)
    hi = (ev >> 16) | (od & jnp.uint32(0xFFFF0000))
    return lo, hi


def _softmax_rows(sc, mask):
    sc = jnp.where(mask, sc, NEG)
    m = jnp.max(sc, axis=1, keepdims=True)
    p = jnp.exp(sc - m)
    l = jnp.sum(p, axis=1, keepdims=True)
    return p * (1.0 / l)


def _kernel(xa_hbm, mem0_ref, awq_hbm, awk_hbm, awv_hbm, awo_hbm,
            xb_hbm, c_hbm, bwq_hbm, bwuk_hbm, bwuv_hbm, bwo_hbm,
            out_hbm,
            xbt, xb, c, bwq_raw, bwuk_raw, bwuv_raw, bwot, bwq_d, wkv_d, q_all, kv, acct, s_buf, p_buf,
            xat, xa, a_raw, awot, aw_d, awo_d, mem, zq, zk, zv, ox, obuf,
            sems, osems,
            *, S, DM, H, E, DC, M, SEG):
    HE = H * E
    NSEG = S // SEG
    scale = E ** -0.5

    def halves(src, dst, s0):
        return [pltpu.make_async_copy(src.at[:, pl.ds(i * 128, 128)], dst.at[i], sems.at[s0 + i])
                for i in range(2)]

    cp_bwq = halves(bwq_hbm, bwq_raw, 0)
    cp_xb = pltpu.make_async_copy(xb_hbm, xbt, sems.at[2])
    cp_c = pltpu.make_async_copy(c_hbm, c, sems.at[3])
    cp_wuk = halves(bwuk_hbm, bwuk_raw, 4)
    cp_wuv = halves(bwuv_hbm, bwuv_raw, 6)
    cp_bwo = pltpu.make_async_copy(bwo_hbm, bwot, sems.at[8])
    cp_aw = [halves(w, a_raw.at[i], 9 + 2 * i) for i, w in enumerate((awq_hbm, awk_hbm, awv_hbm))]
    cp_aw = cp_aw[0] + cp_aw[1] + cp_aw[2]
    cp_xa = pltpu.make_async_copy(xa_hbm, xat, sems.at[15])
    cp_awo = pltpu.make_async_copy(awo_hbm, awot, sems.at[16])

    cp_xb.start()
    cp_bwq[0].start()
    cp_bwq[1].start()
    cp_xb.wait()
    for i in range(S // 128):
        xb[i * 128:(i + 1) * 128, :] = xbt[:, i * 128:(i + 1) * 128].T
    for half in range(2):
        cp_bwq[half].wait()
        if half == 1:
            for cp in cp_wuk + [cp_c] + cp_wuv + [cp_bwo]:
                cp.start()
        r32 = bwq_raw.at[half].bitcast(U32)
        for j in range(H // 2):
            lo, hi = _deint(r32, j, DM)
            bwq_d[:, pl.ds((2 * j) * E + half * 128, 128)] = lo
            bwq_d[:, pl.ds((2 * j + 1) * E + half * 128, 128)] = hi

    TQP = 512
    PADL = 512 - DM
    ZR = 512 // 16
    scale2 = scale * 1.4426950408889634

    def q_step(t):
        i = lax.shift_right_logical(t, 2)
        n = lax.bitwise_and(t, 3)
        r0 = pl.multiple_of(i * TQP, TQP)
        c0 = pl.multiple_of(n * 4 * E, 4 * E)
        z = _dot(xb[pl.ds(r0, TQP), :], _bf(bwq_d[:, pl.ds(c0, 4 * E)])) * scale2
        z = _u32(z.astype(BF))
        rr = pl.ds(pl.multiple_of(i * (TQP // 2), TQP // 2), TQP // 2)
        for hh in range(4):
            q_all[n * 4 + hh, rr, :] = z[:, hh * E:(hh + 1) * E]
        acct[pl.ds(pl.multiple_of(t * ZR, ZR), ZR), :] = jnp.zeros((ZR, S), F32)

    def deint_kv(raw, w_i, t):
        for half in range(2):
            r32 = raw.at[half].bitcast(U32).at[pl.ds(pl.multiple_of(t * 2048, 2048), 2048)]
            rows = pl.ds(pl.multiple_of(t * 128, 128), 128)
            for j in range(H // 2):
                lo, hi = _deint(r32, j, 256)
                wkv_d[2 * j, rows, pl.ds(w_i * E + half * 128, 128)] = lo
                wkv_d[2 * j + 1, rows, pl.ds(w_i * E + half * 128, 128)] = hi

    def q_plain(t, carry):
        q_step(t)
        return carry

    def q_uk(t, carry):
        q_step(t)
        deint_kv(bwuk_raw, 0, t - 8)
        return carry

    def q_uv(t, carry):
        q_step(t)
        deint_kv(bwuv_raw, 1, t - 12)
        return carry

    lax.fori_loop(0, 8, q_plain, 0)
    for cp in cp_wuk:
        cp.wait()
    for cp in cp_aw + [cp_xa, cp_awo]:
        cp.start()
    lax.fori_loop(8, 12, q_uk, 0)
    for cp in cp_wuv:
        cp.wait()
    lax.fori_loop(12, 16, q_uv, 0)
    cp_c.wait()

    TQ = 256
    NQ = S // TQ
    HQ = TQ // 2

    def kv_chunk(h, slot, i):
        z = _dot(c[pl.ds(i * TQ, TQ), :], _bf(wkv_d[h]))
        kv[slot, pl.ds(i * TQ // 2, TQ // 2), :] = _u32(z.astype(BF))

    def kv0(i, carry):
        z = _dot(c[pl.ds(pl.multiple_of(i * 512, 512), 512), :], _bf(wkv_d[0]))
        kv[0, pl.ds(pl.multiple_of(i * 256, 256), 256), :] = _u32(z.astype(BF))
        return carry

    lax.fori_loop(0, S // 512, kv0, 0)
    cp_bwo.wait()
    for cp in cp_aw + [cp_xa, cp_awo]:
        cp.wait()

    RG = 16

    def attention(h, slot, filler):
        wot_h = bwot[pl.ds(pl.multiple_of(h * DM, DM), DM), :]
        row = lax.broadcasted_iota(jnp.int32, (TQ, HQ), 0)
        col = lax.broadcasted_iota(jnp.int32, (TQ, HQ), 1)
        tri_main = row >= col
        tri_tail = tri_main[0:HQ]
        pending = None

        def out_proj(pending):
            pi, pctx = pending
            acct[PADL:PADL + DM, pl.ds(pi * TQ, TQ)] += _dot_nt(wot_h, pctx)

        for idx, i in enumerate(range(NQ - 1, -1, -1)):
            b = idx % 2
            n = (i + 1) * TQ
            nm = n - HQ
            nf = n - TQ
            q = _bf(q_all[h, pl.ds(i * TQ // 2, TQ // 2), :])
            if nf > 0:
                s_buf[b, :, 0:nf] = _dot_nt(q, _bf(kv[slot, pl.ds(0, nf // 2), 0:E]))
            s_mid = _dot_nt(q, _bf(kv[slot, pl.ds(nf // 2, HQ // 2), 0:E]))
            s_buf[b, :, nf:nm] = jnp.where(tri_main, s_mid, NEG)
            s_tail = _dot_nt(q[HQ:TQ], _bf(kv[slot, pl.ds(nm // 2, HQ // 2), 0:E]))
            s_buf[b, HQ:TQ, nm:n] = jnp.where(tri_tail, s_tail, NEG)
            if pending is not None:
                out_proj(pending)
            filler(idx)
            ls = []
            for g in range(TQ // RG):
                ne = nm if g * RG < HQ else n
                sg = s_buf[b, g * RG:(g + 1) * RG, 0:ne]
                m = jnp.max(sg, axis=1, keepdims=True)
                pg = jnp.exp2(sg - m)
                ls.append(jnp.sum(pg, axis=1, keepdims=True))
                p_buf[b, g * RG // 2:(g + 1) * RG // 2, 0:ne] = _u32(pg.astype(BF))
            l = jnp.concatenate(ls, axis=0)
            ctx = _dot(_bf(p_buf[b, :, 0:nm]), _bf(kv[slot, pl.ds(0, nm // 2), E:2 * E]))
            ctx_t = _dot(_bf(p_buf[b, HQ // 2:TQ // 2, nm:n]), _bf(kv[slot, pl.ds(nm // 2, HQ // 2), E:2 * E]))
            ctx = jnp.concatenate([ctx[0:HQ], ctx[HQ:TQ] + ctx_t], axis=0)
            pending = (i, (ctx * (1.0 / l)).astype(BF))
        out_proj(pending)

    def deint_a(t):
        rows = pl.ds(pl.multiple_of(t * 16, 16), 16)
        for w_i in range(3):
            for half in range(2):
                r32 = a_raw.at[w_i, half].bitcast(U32).at[pl.ds(pl.multiple_of(t * 256, 256), 256)]
                for j in range(H // 2):
                    lo, hi = _deint(r32, j, 32)
                    aw_d[rows, pl.ds(w_i * HE + (2 * j) * E + half * 128, 128)] = lo
                    aw_d[rows, pl.ds(w_i * HE + (2 * j + 1) * E + half * 128, 128)] = hi

    def prep_a(t):
        awo_d[pl.ds(pl.multiple_of(t * E, E), E), :] = awot[pl.ds(pl.multiple_of(t * DM, DM), DM), :].T
        cc = pl.ds(pl.multiple_of(t * 128, 128), 128)
        xa[cc, :] = xat[:, cc].T

    def head(h, carry):
        slot = lax.bitwise_and(h, 1)

        def filler(idx):
            kv_chunk(h + 1, 1 - slot, idx)
            if idx == 0:
                deint_a(jnp.minimum(h, DM // 32 - 1))
            if idx == 1:
                prep_a(h)

        attention(h, slot, filler)
        return carry

    lax.fori_loop(0, H - 1, head, 0)

    def last_filler(idx):
        if idx == 1:
            prep_a(H - 1)

    attention(H - 1, (H - 1) % 2, last_filler)

    def bout(i, carry):
        r = pl.ds(pl.multiple_of(i * 256, 256), 256)
        obuf[r, DM - PADL:2 * DM] = acct[:, r].astype(BF).T
        return carry

    lax.fori_loop(0, S // 256, bout, 0)

    L = 48
    LV = M + SEG
    mem[...] = jnp.concatenate([mem0_ref[...].astype(F32), jnp.zeros((8, DM), F32)], axis=0).astype(BF)
    zk[...] = jnp.zeros_like(zk)
    zv[...] = jnp.zeros_like(zv)
    ox[...] = jnp.zeros_like(ox)
    z0 = _dot(xa[0:SEG, :], _bf(aw_d[...]))
    zq[0] = (z0[:, 0:HE] * scale).astype(BF)
    zk[0, 0:SEG, :] = z0[:, HE:2 * HE].astype(BF)
    zv[0, 0:SEG, :] = z0[:, 2 * HE:3 * HE].astype(BF)

    OC = 8
    NOC = NSEG // OC
    ORS = OC * SEG

    def out_copy(k):
        r = pl.ds(pl.multiple_of(k * ORS, ORS), ORS)
        return pltpu.make_async_copy(obuf.at[r, :], out_hbm.at[r, :], osems.at[k])

    def seg(s, carry):
        colm = lax.broadcasted_iota(jnp.int32, (H * M, L), 1)
        mask_m = colm < LV
        rowx = lax.bitwise_and(lax.broadcasted_iota(jnp.int32, (H * SEG, L), 0), SEG - 1)
        colx = lax.broadcasted_iota(jnp.int32, (H * SEG, L), 1)
        mask_x = (colx < LV) & ((rowx >= colx) | (colx >= SEG))
        cur = lax.bitwise_and(s, 1)
        nxt = 1 - cur
        rn = pl.multiple_of(jnp.minimum(s + 1, NSEG - 1) * SEG, SEG)
        lhs = jnp.concatenate([xa[pl.ds(rn, SEG), :], mem[...]], axis=0)
        zqk = _dot(lhs, _bf(aw_d[:, 0:2 * HE]))
        zq[nxt] = (zqk[0:SEG, 0:HE] * scale).astype(BF)
        qm = (zqk[SEG:LV, 0:HE] * scale).astype(BF)
        zk[nxt, 0:SEG, :] = zqk[0:SEG, HE:2 * HE].astype(BF)
        zk[cur, SEG:LV, :] = zqk[SEG:LV, HE:2 * HE].astype(BF)
        sm = jnp.concatenate(
            [_dot_nt(qm[:, h * E:(h + 1) * E], zk[cur, :, h * E:(h + 1) * E]) for h in range(H)], axis=0)
        zvv = _dot(lhs, _bf(aw_d[:, 2 * HE:3 * HE]))
        zv[nxt, 0:SEG, :] = zvv[0:SEG].astype(BF)
        zv[cur, SEG:LV, :] = zvv[SEG:LV].astype(BF)
        pm = _softmax_rows(sm, mask_m)
        om = jnp.concatenate(
            [_dot(pm[h * M:(h + 1) * M].astype(BF), zv[cur, :, h * E:(h + 1) * E]) for h in range(H)], axis=1)
        sx = jnp.concatenate(
            [_dot_nt(zq[cur, :, h * E:(h + 1) * E], zk[cur, :, h * E:(h + 1) * E]) for h in range(H)], axis=0)
        om16 = jnp.concatenate([om, jnp.zeros((8, HE), F32)], axis=0).astype(BF)
        lhs2 = jnp.concatenate([ox[...], om16], axis=0)
        o = _dot(lhs2, awo_d[...]).astype(BF)
        rp = pl.multiple_of(jnp.maximum(s - 1, 0) * SEG, SEG)
        obuf[pl.ds(rp, SEG), 0:DM] = o[0:SEG]
        mem[...] = o[SEG:L]
        px = _softmax_rows(sx, mask_x).astype(BF)
        for h in range(H):
            ox[:, h * E:(h + 1) * E] = _dot(px[h * SEG:(h + 1) * SEG], zv[cur, :, h * E:(h + 1) * E]).astype(BF)

        @pl.when(jnp.logical_and(lax.bitwise_and(s, OC - 1) == 0, s > 0))
        def _():
            out_copy(lax.shift_right_logical(s, 3) - 1).start()

        return carry

    lax.fori_loop(0, NSEG, seg, 0)
    obuf[S - SEG:S, 0:DM] = _dot(ox[...], awo_d[...]).astype(BF)
    out_copy(NOC - 1).start()
    for k in range(NOC):
        out_copy(k).wait()


@functools.partial(jax.jit, static_argnames=("A_seg_len",))
def pallas_concat_heads__memory_aug_recurrent_mem_tr__compressed_kv_cla__prompt_kernel(
    A_x, A_mem0, A_Wq, A_Wk, A_Wv, A_Wo, A_seg_len,
    B_x, B_c_kv, B_w_q, B_w_uk, B_w_uv, B_w_o,
):
    _, S, DM = A_x.shape
    _, H, E = A_Wq.shape
    M = A_mem0.shape[1]
    DC = B_c_kv.shape[2]
    SEG = int(A_seg_len)
    assert (S, DM, H, E, M, DC, SEG) == (2048, 448, 16, 256, 8, 1024, 32)
    HE = H * E
    any_spec = pl.BlockSpec(memory_space=pl.ANY)
    vm = pltpu.VMEM
    scratch = [
        vm((DM, S), BF), vm((S, DM), BF), vm((S, DC), BF),
        vm((2, DM * H, 128), BF), vm((2, DC * H, 128), BF), vm((2, DC * H, 128), BF),
        vm((H * DM, E), BF),
        vm((DM // 2, HE), U32), vm((H, DC // 2, 2 * E), U32),
        vm((H, S // 2, E), U32), vm((2, S // 2, 2 * E), U32),
        vm((512, S), F32),
        vm((2, 256, S), F32), vm((2, 128, S), U32),
        vm((DM, S), BF), vm((S, DM), BF),
        vm((3, 2, DM * H, 128), BF), vm((H * DM, E), BF),
        vm((DM // 2, 3 * HE), U32), vm((HE, DM), BF),
        vm((16, DM), BF),
        vm((2, SEG, HE), BF), vm((2, 48, HE), BF), vm((2, 48, HE), BF),
        vm((SEG, HE), BF),
        vm((S, 2 * DM), BF),
        pltpu.SemaphoreType.DMA((17,)), pltpu.SemaphoreType.DMA((8,)),
    ]
    out = pl.pallas_call(
        functools.partial(_kernel, S=S, DM=DM, H=H, E=E, DC=DC, M=M, SEG=SEG),
        out_shape=jax.ShapeDtypeStruct((S, 2 * DM), BF),
        in_specs=[any_spec, pl.BlockSpec(memory_space=pltpu.VMEM)] + [any_spec] * 10,
        out_specs=any_spec,
        scratch_shapes=scratch,
        compiler_params=pltpu.CompilerParams(vmem_limit_bytes=126 * 1024 * 1024),
    )(
        jnp.swapaxes(A_x, 1, 2).reshape(DM, S), A_mem0.reshape(M, DM),
        A_Wq.reshape(DM * H, E), A_Wk.reshape(DM * H, E), A_Wv.reshape(DM * H, E),
        jnp.swapaxes(A_Wo, 1, 2).reshape(H * DM, E),
        jnp.swapaxes(B_x, 1, 2).reshape(DM, S), B_c_kv.reshape(S, DC),
        B_w_q.reshape(DM * H, E), B_w_uk.reshape(DC * H, E), B_w_uv.reshape(DC * H, E),
        jnp.swapaxes(B_w_o, 1, 2).reshape(H * DM, E),
    )
    return out.reshape(1, S, 2 * DM)
```

```python
import functools
import os

import jax
import jax.numpy as jnp
from jax import lax
from jax.experimental import pallas as pl
from jax.experimental.pallas import tpu as pltpu

BF = jnp.bfloat16
F32 = jnp.float32
U32 = jnp.uint32
NT = (((1,), (1,)), ((), ()))
NEG = -1000000000.0


def _bf(x32):
    return pltpu.bitcast(x32, BF)


def _u32(xb):
    return pltpu.bitcast(xb, U32)


def _dot(a, b):
    return jnp.dot(a, b, preferred_element_type=F32)


def _dot_nt(a, b):
    return lax.dot_general(a, b, NT, preferred_element_type=F32)


def _deint(raw32, j, nrows):
    ev = raw32[pl.ds(j, nrows // 2, stride=16), :]
    od = raw32[pl.ds(j + 8, nrows // 2, stride=16), :]
    lo = (ev & jnp.uint32(0xFFFF)) | (od << 16)
    hi = (ev >> 16) | (od & jnp.uint32(0xFFFF0000))
    return lo, hi


def _zero_after(x):
    return (pltpu.bitcast(x, U32) >> 16) >> 16


def _softmax_rows(sc, mask):
    sc = jnp.where(mask, sc, NEG)
    m = jnp.max(sc, axis=1, keepdims=True)
    p = jnp.exp(sc - m)
    l = jnp.sum(p, axis=1, keepdims=True)
    return p * (1.0 / l)


def _kernel(xa_hbm, mem0_ref, awq_hbm, awk_hbm, awv_hbm, awo_hbm,
            xb_hbm, c_hbm, bwq_hbm, bwuk_hbm, bwuv_hbm, bwo_hbm,
            out_hbm,
            xbt, xb, c, bwq_raw, bwuk_raw, bwuv_raw, bwot, bwq_d, wkv_d, q_all, kv, acct, s_buf0, s_buf1, p_buf0, p_buf1,
            xat, xa, a_raw, awot, aw_d, awo_d, mem, zq, zk, zv, ox, obuf,
            sems, osems,
            *, S, DM, H, E, DC, M, SEG):
    HE = H * E
    NSEG = S // SEG
    scale = E ** -0.5
    s_buf = (s_buf0, s_buf1)
    p_buf = (p_buf0, p_buf1)

    def halves(src, dst, s0):
        return [pltpu.make_async_copy(src.at[:, pl.ds(i * 128, 128)], dst.at[i], sems.at[s0 + i])
                for i in range(2)]

    cp_bwq = halves(bwq_hbm, bwq_raw, 0)
    cp_xb = pltpu.make_async_copy(xb_hbm, xbt, sems.at[2])
    cp_c = pltpu.make_async_copy(c_hbm, c, sems.at[3])
    cp_wuk = halves(bwuk_hbm, bwuk_raw, 4)
    cp_wuv = halves(bwuv_hbm, bwuv_raw, 6)
    cp_bwo = pltpu.make_async_copy(bwo_hbm, bwot, sems.at[8])
    cp_aw = [halves(w, a_raw.at[i], 9 + 2 * i) for i, w in enumerate((awq_hbm, awk_hbm, awv_hbm))]
    cp_aw = cp_aw[0] + cp_aw[1] + cp_aw[2]
    cp_xa = pltpu.make_async_copy(xa_hbm, xat, sems.at[15])
    cp_awo = pltpu.make_async_copy(awo_hbm, awot, sems.at[16])

    cp_xb.start()
    cp_bwq[0].start()
    cp_bwq[1].start()
    cp_xb.wait()
    for i in range(S // 128):
        xb[i * 128:(i + 1) * 128, :] = xbt[:, i * 128:(i + 1) * 128].T
    for half in range(2):
        cp_bwq[half].wait()
        if half == 1:
            for cp in cp_wuk + [cp_c] + cp_wuv + [cp_bwo]:
                cp.start()
        r32 = bwq_raw.at[half].bitcast(U32)
        for j in range(H // 2):
            lo, hi = _deint(r32, j, DM)
            bwq_d[:, pl.ds((2 * j) * E + half * 128, 128)] = lo
            bwq_d[:, pl.ds((2 * j + 1) * E + half * 128, 128)] = hi

    TQP = 512
    PADL = 512 - DM
    ZR = 512 // 16
    scale2 = scale * 1.4426950408889634

    def q_step(t):
        i = lax.shift_right_logical(t, 2)
        n = lax.bitwise_and(t, 3)
        r0 = pl.multiple_of(i * TQP, TQP)
        c0 = pl.multiple_of(n * 4 * E, 4 * E)
        z = _dot(xb[pl.ds(r0, TQP), :], _bf(bwq_d[:, pl.ds(c0, 4 * E)])) * scale2
        z = _u32(z.astype(BF))
        rr = pl.ds(pl.multiple_of(i * (TQP // 2), TQP // 2), TQP // 2)
        for hh in range(4):
            q_all[n * 4 + hh, rr, :] = z[:, hh * E:(hh + 1) * E]
        acct[pl.ds(pl.multiple_of(t * ZR, ZR), ZR), :] = jnp.zeros((ZR, S), F32)

    def deint_kv(raw, w_i, t):
        for half in range(2):
            r32 = raw.at[half].bitcast(U32).at[pl.ds(pl.multiple_of(t * 2048, 2048), 2048)]
            rows = pl.ds(pl.multiple_of(t * 128, 128), 128)
            for j in range(H // 2):
                lo, hi = _deint(r32, j, 256)
                wkv_d[2 * j, rows, pl.ds(w_i * E + half * 128, 128)] = lo
                wkv_d[2 * j + 1, rows, pl.ds(w_i * E + half * 128, 128)] = hi

    def q_plain(t, carry):
        q_step(t)
        return carry

    def q_uk(t, carry):
        q_step(t)
        deint_kv(bwuk_raw, 0, t - 8)
        return carry

    def q_uv(t, carry):
        q_step(t)
        deint_kv(bwuv_raw, 1, t - 12)
        return carry

    lax.fori_loop(0, 8, q_plain, 0)
    for cp in cp_wuk:
        cp.wait()
    for cp in cp_aw + [cp_xa, cp_awo]:
        cp.start()
    lax.fori_loop(8, 12, q_uk, 0)
    for cp in cp_wuv:
        cp.wait()
    lax.fori_loop(12, 16, q_uv, 0)
    cp_c.wait()

    TQ = 256
    NQ = S // TQ
    HQ = TQ // 2

    def kv_chunk(h, slot, i):
        z = _dot(c[pl.ds(i * TQ, TQ), :], _bf(wkv_d[h]))
        kv[slot, pl.ds(i * TQ // 2, TQ // 2), :] = _u32(z.astype(BF))

    def kv0(i, carry):
        z = _dot(c[pl.ds(pl.multiple_of(i * 512, 512), 512), :], _bf(wkv_d[0]))
        kv[0, pl.ds(pl.multiple_of(i * 256, 256), 256), :] = _u32(z.astype(BF))
        return carry

    lax.fori_loop(0, S // 512, kv0, 0)
    cp_bwo.wait()
    for cp in cp_aw + [cp_xa, cp_awo]:
        cp.wait()

    RG = int(os.environ.get('RG', 8))
    CHL = [int(v) for v in os.environ.get('CH', '22222222')]
    CHZ = [int(v) for v in os.environ.get('CHZ', '42233468')]

    def attention(h, slot, filler, CHS):
        wot_h = bwot[pl.ds(pl.multiple_of(h * DM, DM), DM), :]
        row = lax.broadcasted_iota(jnp.int32, (TQ, HQ), 0)
        col = lax.broadcasted_iota(jnp.int32, (TQ, HQ), 1)
        tri_main = row >= col
        tri_tail = tri_main[0:HQ]
        blocks = list(range(NQ - 1, -1, -1))

        def scores(idx):
            i, b = blocks[idx], idx % 2
            n = (i + 1) * TQ
            nm = n - HQ
            nf = n - TQ
            q = _bf(q_all[h, pl.ds(i * TQ // 2, TQ // 2), :])
            if nf > 0:
                s_buf[b][:, 0:nf] = _dot_nt(q, _bf(kv[slot, pl.ds(0, nf // 2), 0:E]))
            s_mid = _dot_nt(q, _bf(kv[slot, pl.ds(nf // 2, HQ // 2), 0:E]))
            s_buf[b][:, nf:nm] = jnp.where(tri_main, s_mid, NEG)
            s_tail = _dot_nt(q[HQ:TQ], _bf(kv[slot, pl.ds(nm // 2, HQ // 2), 0:E]))
            s_buf[b][HQ:TQ, nm:n] = jnp.where(tri_tail, s_tail, NEG)

        def softmax(idx):
            i, b, CH = blocks[idx], idx % 2, CHS[idx]
            n = (i + 1) * TQ
            nm = n - HQ
            ls = []
            sms = []
            for g in range(TQ // RG):
                ne = nm if g * RG < HQ else n
                rows = slice(g * RG, (g + 1) * RG)
                mx = s_buf[b][rows, 0:128]
                if g >= CH:
                    mx = mx + sms[g - CH] * 0.0
                for t in range(1, ne // 128):
                    mx = jnp.maximum(mx, s_buf[b][rows, t * 128:(t + 1) * 128])
                m = jnp.broadcast_to(jnp.max(mx, axis=1, keepdims=True), (RG, 128))
                sm = None
                for t0 in range(0, ne, 256):
                    pgs = []
                    for t in range(t0, min(t0 + 256, ne), 128):
                        pg = jnp.exp2(s_buf[b][rows, t:t + 128] - m)
                        sm = pg if sm is None else sm + pg
                        pgs.append(pg)
                    p_buf[b][rows, t0:t0 + 128 * len(pgs)] = jnp.concatenate(pgs, axis=1).astype(BF)
                sms.append(sm)
                ls.append(jnp.sum(sm, axis=1, keepdims=True))
            return jnp.concatenate(ls, axis=0)

        def context(idx, l):
            i, b = blocks[idx], idx % 2
            n = (i + 1) * TQ
            nm = n - HQ
            ctx = _dot(p_buf[b][:, 0:nm], _bf(kv[slot, pl.ds(0, nm // 2), E:2 * E]))
            ctx_t = _dot(p_buf[b][HQ:TQ, nm:n], _bf(kv[slot, pl.ds(nm // 2, HQ // 2), E:2 * E]))
            ctx = jnp.concatenate([ctx[0:HQ], ctx[HQ:TQ] + ctx_t], axis=0)
            return (ctx * (1.0 / l)).astype(BF)

        def out_proj(idx, ctx):
            acct[PADL:PADL + DM, pl.ds(blocks[idx] * TQ, TQ)] += _dot_nt(wot_h, ctx)

        scores(0)
        ctx = None
        for idx in range(NQ):
            l = softmax(idx)
            filler(idx)
            if idx + 1 < NQ:
                scores(idx + 1)
            if ctx is not None:
                out_proj(idx - 1, ctx)
            ctx = context(idx, l)
        out_proj(NQ - 1, ctx)

    def deint_a(t):
        rows = pl.ds(pl.multiple_of(t * 16, 16), 16)
        for w_i in range(3):
            for half in range(2):
                r32 = a_raw.at[w_i, half].bitcast(U32).at[pl.ds(pl.multiple_of(t * 256, 256), 256)]
                for j in range(H // 2):
                    lo, hi = _deint(r32, j, 32)
                    aw_d[rows, pl.ds(w_i * HE + (2 * j) * E + half * 128, 128)] = lo
                    aw_d[rows, pl.ds(w_i * HE + (2 * j + 1) * E + half * 128, 128)] = hi

    def prep_a(t):
        awo_d[pl.ds(pl.multiple_of(t * E, E), E), :] = awot[pl.ds(pl.multiple_of(t * DM, DM), DM), :].T
        cc = pl.ds(pl.multiple_of(t * 128, 128), 128)
        xa[cc, :] = xat[:, cc].T

    def head(h, carry):
        slot = lax.bitwise_and(h, 1)

        def filler(idx):
            kv_chunk(h + 1, 1 - slot, idx)
            if idx == 0:
                deint_a(jnp.minimum(h, DM // 32 - 1))
            if idx == 1:
                prep_a(h)

        attention(h, slot, filler, CHL)
        return carry

    lax.fori_loop(0, H - 1, head, 0)

    def last_filler(idx):
        if idx == 1:
            prep_a(H - 1)

    attention(H - 1, (H - 1) % 2, last_filler, CHZ)

    def bout(i, carry):
        r = pl.ds(pl.multiple_of(i * 256, 256), 256)
        obuf[r, DM - PADL:2 * DM] = acct[:, r].astype(BF).T
        return carry

    lax.fori_loop(0, S // 256, bout, 0)

    L = 48
    LV = M + SEG
    mem[...] = jnp.concatenate([mem0_ref[...].astype(F32), jnp.zeros((8, DM), F32)], axis=0).astype(BF)
    zk[...] = jnp.zeros_like(zk)
    zv[...] = jnp.zeros_like(zv)
    ox[...] = jnp.zeros_like(ox)
    z0 = _dot(xa[0:SEG, :], _bf(aw_d[...]))
    zq[0] = (z0[:, 0:HE] * scale).astype(BF)
    zk[0, 0:SEG, :] = z0[:, HE:2 * HE].astype(BF)
    zv[0, 0:SEG, :] = z0[:, 2 * HE:3 * HE].astype(BF)

    OC = 8
    NOC = NSEG // OC
    ORS = OC * SEG

    def out_copy(k):
        r = pl.ds(pl.multiple_of(k * ORS, ORS), ORS)
        return pltpu.make_async_copy(obuf.at[r, :], out_hbm.at[r, :], osems.at[k])

    def seg(s, carry):
        colm = lax.broadcasted_iota(jnp.int32, (H * M, L), 1)
        mask_m = colm < LV
        rowx = lax.bitwise_and(lax.broadcasted_iota(jnp.int32, (H * SEG, L), 0), SEG - 1)
        colx = lax.broadcasted_iota(jnp.int32, (H * SEG, L), 1)
        mask_x = (colx < LV) & ((rowx >= colx) | (colx >= SEG))
        cur = lax.bitwise_and(s, 1)
        nxt = 1 - cur
        rn = pl.multiple_of(jnp.minimum(s + 1, NSEG - 1) * SEG, SEG)
        lhs = jnp.concatenate([xa[pl.ds(rn, SEG), :], mem[...]], axis=0)
        zqk = _dot(lhs, _bf(aw_d[:, 0:2 * HE]))
        zq[nxt] = (zqk[0:SEG, 0:HE] * scale).astype(BF)
        qm = (zqk[SEG:LV, 0:HE] * scale).astype(BF)
        zk[nxt, 0:SEG, :] = zqk[0:SEG, HE:2 * HE].astype(BF)
        zk[cur, SEG:LV, :] = zqk[SEG:LV, HE:2 * HE].astype(BF)
        sm = jnp.concatenate(
            [_dot_nt(qm[:, h * E:(h + 1) * E], zk[cur, :, h * E:(h + 1) * E]) for h in range(H)], axis=0)
        zvv = _dot(lhs, _bf(aw_d[:, 2 * HE:3 * HE]))
        zv[nxt, 0:SEG, :] = zvv[0:SEG].astype(BF)
        zv[cur, SEG:LV, :] = zvv[SEG:LV].astype(BF)
        pm = _softmax_rows(sm, mask_m)
        om = jnp.concatenate(
            [_dot(pm[h * M:(h + 1) * M].astype(BF), zv[cur, :, h * E:(h + 1) * E]) for h in range(H)], axis=1)
        sx = jnp.concatenate(
            [_dot_nt(zq[cur, :, h * E:(h + 1) * E], zk[cur, :, h * E:(h + 1) * E]) for h in range(H)], axis=0)
        om16 = jnp.concatenate([om, jnp.zeros((8, HE), F32)], axis=0).astype(BF)
        lhs2 = jnp.concatenate([ox[...], om16], axis=0)
        o = _dot(lhs2, awo_d[...]).astype(BF)
        rp = pl.multiple_of(jnp.maximum(s - 1, 0) * SEG, SEG)
        obuf[pl.ds(rp, SEG), 0:DM] = o[0:SEG]
        mem[...] = o[SEG:L]
        px = _softmax_rows(sx, mask_x).astype(BF)
        for h in range(H):
            ox[:, h * E:(h + 1) * E] = _dot(px[h * SEG:(h + 1) * SEG], zv[cur, :, h * E:(h + 1) * E]).astype(BF)

        @pl.when(jnp.logical_and(lax.bitwise_and(s, OC - 1) == 0, s > 0))
        def _():
            out_copy(lax.shift_right_logical(s, 3) - 1).start()

        return carry

    lax.fori_loop(0, NSEG, seg, 0)
    obuf[S - SEG:S, 0:DM] = _dot(ox[...], awo_d[...]).astype(BF)
    out_copy(NOC - 1).start()
    for k in range(NOC):
        out_copy(k).wait()


@functools.partial(jax.jit, static_argnames=("A_seg_len",))
def pallas_concat_heads__memory_aug_recurrent_mem_tr__compressed_kv_cla__prompt_kernel(
    A_x, A_mem0, A_Wq, A_Wk, A_Wv, A_Wo, A_seg_len,
    B_x, B_c_kv, B_w_q, B_w_uk, B_w_uv, B_w_o,
):
    _, S, DM = A_x.shape
    _, H, E = A_Wq.shape
    M = A_mem0.shape[1]
    DC = B_c_kv.shape[2]
    SEG = int(A_seg_len)
    assert (S, DM, H, E, M, DC, SEG) == (2048, 448, 16, 256, 8, 1024, 32)
    HE = H * E
    any_spec = pl.BlockSpec(memory_space=pl.ANY)
    vm = pltpu.VMEM
    scratch = [
        vm((DM, S), BF), vm((S, DM), BF), vm((S, DC), BF),
        vm((2, DM * H, 128), BF), vm((2, DC * H, 128), BF), vm((2, DC * H, 128), BF),
        vm((H * DM, E), BF),
        vm((DM // 2, HE), U32), vm((H, DC // 2, 2 * E), U32),
        vm((H, S // 2, E), U32), vm((2, S // 2, 2 * E), U32),
        vm((512, S), F32),
        vm((256, S), F32), vm((256, S), F32), vm((256, S), BF), vm((256, S), BF),
        vm((DM, S), BF), vm((S, DM), BF),
        vm((3, 2, DM * H, 128), BF), vm((H * DM, E), BF),
        vm((DM // 2, 3 * HE), U32), vm((HE, DM), BF),
        vm((16, DM), BF),
        vm((2, SEG, HE), BF), vm((2, 48, HE), BF), vm((2, 48, HE), BF),
        vm((SEG, HE), BF),
        vm((S, 2 * DM), BF),
        pltpu.SemaphoreType.DMA((17,)), pltpu.SemaphoreType.DMA((8,)),
    ]
    out = pl.pallas_call(
        functools.partial(_kernel, S=S, DM=DM, H=H, E=E, DC=DC, M=M, SEG=SEG),
        out_shape=jax.ShapeDtypeStruct((S, 2 * DM), BF),
        in_specs=[any_spec, pl.BlockSpec(memory_space=pltpu.VMEM)] + [any_spec] * 10,
        out_specs=any_spec,
        scratch_shapes=scratch,
        compiler_params=pltpu.CompilerParams(vmem_limit_bytes=126 * 1024 * 1024),
    )(
        jnp.swapaxes(A_x, 1, 2).reshape(DM, S), A_mem0.reshape(M, DM),
        A_Wq.reshape(DM * H, E), A_Wk.reshape(DM * H, E), A_Wv.reshape(DM * H, E),
        jnp.swapaxes(A_Wo, 1, 2).reshape(H * DM, E),
        jnp.swapaxes(B_x, 1, 2).reshape(DM, S), B_c_kv.reshape(S, DC),
        B_w_q.reshape(DM * H, E), B_w_uk.reshape(DC * H, E), B_w_uv.reshape(DC * H, E),
        jnp.swapaxes(B_w_o, 1, 2).reshape(H * DM, E),
    )
    return out.reshape(1, S, 2 * DM)
```

```python
import functools
import os

import jax
import jax.numpy as jnp
from jax import lax
from jax.experimental import pallas as pl
from jax.experimental.pallas import tpu as pltpu

BF = jnp.bfloat16
F32 = jnp.float32
U32 = jnp.uint32
NT = (((1,), (1,)), ((), ()))
NEG = -1000000000.0


def _bf(x32):
    return pltpu.bitcast(x32, BF)


def _u32(xb):
    return pltpu.bitcast(xb, U32)


def _dot(a, b):
    return jnp.dot(a, b, preferred_element_type=F32)


def _dot_nt(a, b):
    return lax.dot_general(a, b, NT, preferred_element_type=F32)


def _deint(raw32, j, nrows):
    ev = raw32[pl.ds(j, nrows // 2, stride=16), :]
    od = raw32[pl.ds(j + 8, nrows // 2, stride=16), :]
    lo = (ev & jnp.uint32(0xFFFF)) | (od << 16)
    hi = (ev >> 16) | (od & jnp.uint32(0xFFFF0000))
    return lo, hi


def _zero_after(x):
    return (pltpu.bitcast(x, U32) >> 16) >> 16


def _softmax_rows(sc, mask):
    sc = jnp.where(mask, sc, NEG)
    m = jnp.max(sc, axis=1, keepdims=True)
    p = jnp.exp(sc - m)
    l = jnp.sum(p, axis=1, keepdims=True)
    return p * (1.0 / l)


def _kernel(xa_hbm, mem0_ref, awq_hbm, awk_hbm, awv_hbm, awo_hbm,
            xb_hbm, c_hbm, bwq_hbm, bwuk_hbm, bwuv_hbm, bwo_hbm,
            out_hbm,
            xbt, xb, c, bwq_raw, bwuk_raw, bwuv_raw, bwot, bwq_d, wkv_d, q_all, kv, acct, s_buf0, s_buf1, p_buf0, p_buf1,
            xat, xa, a_raw, awot, aw_d, awo_d, mem, zq, zk, zv, ox, obuf,
            sems, osems,
            *, S, DM, H, E, DC, M, SEG):
    HE = H * E
    NSEG = S // SEG
    scale = E ** -0.5
    s_buf = (s_buf0, s_buf1)
    p_buf = (p_buf0, p_buf1)

    def halves(src, dst, s0):
        return [pltpu.make_async_copy(src.at[:, pl.ds(i * 128, 128)], dst.at[i], sems.at[s0 + i])
                for i in range(2)]

    cp_bwq = halves(bwq_hbm, bwq_raw, 0)
    cp_xb = pltpu.make_async_copy(xb_hbm, xbt, sems.at[2])
    cp_c = pltpu.make_async_copy(c_hbm, c, sems.at[3])
    cp_wuk = halves(bwuk_hbm, bwuk_raw, 4)
    cp_wuv = halves(bwuv_hbm, bwuv_raw, 6)
    cp_bwo = pltpu.make_async_copy(bwo_hbm, bwot, sems.at[8])
    cp_aw = [halves(w, a_raw.at[i], 9 + 2 * i) for i, w in enumerate((awq_hbm, awk_hbm, awv_hbm))]
    cp_aw = cp_aw[0] + cp_aw[1] + cp_aw[2]
    cp_xa = pltpu.make_async_copy(xa_hbm, xat, sems.at[15])
    cp_awo = pltpu.make_async_copy(awo_hbm, awot, sems.at[16])

    cp_xb.start()
    cp_bwq[0].start()
    cp_bwq[1].start()
    cp_xb.wait()
    for i in range(S // 128):
        xb[i * 128:(i + 1) * 128, :] = xbt[:, i * 128:(i + 1) * 128].T
    for half in range(2):
        cp_bwq[half].wait()
        if half == 1:
            for cp in cp_wuk + [cp_c] + cp_wuv + [cp_bwo]:
                cp.start()
        r32 = bwq_raw.at[half].bitcast(U32)
        for j in range(H // 2):
            lo, hi = _deint(r32, j, DM)
            bwq_d[:, pl.ds((2 * j) * E + half * 128, 128)] = lo
            bwq_d[:, pl.ds((2 * j + 1) * E + half * 128, 128)] = hi

    TQP = 512
    PADL = 512 - DM
    ZR = 512 // 16
    scale2 = scale * 1.4426950408889634

    def q_step(t):
        i = lax.shift_right_logical(t, 2)
        n = lax.bitwise_and(t, 3)
        r0 = pl.multiple_of(i * TQP, TQP)
        c0 = pl.multiple_of(n * 4 * E, 4 * E)
        z = _dot(xb[pl.ds(r0, TQP), :], _bf(bwq_d[:, pl.ds(c0, 4 * E)])) * scale2
        z = _u32(z.astype(BF))
        rr = pl.ds(pl.multiple_of(i * (TQP // 2), TQP // 2), TQP // 2)
        for hh in range(4):
            q_all[n * 4 + hh, rr, :] = z[:, hh * E:(hh + 1) * E]
        acct[pl.ds(pl.multiple_of(t * ZR, ZR), ZR), :] = jnp.zeros((ZR, S), F32)

    def deint_kv(raw, w_i, t):
        for half in range(2):
            r32 = raw.at[half].bitcast(U32).at[pl.ds(pl.multiple_of(t * 2048, 2048), 2048)]
            rows = pl.ds(pl.multiple_of(t * 128, 128), 128)
            for j in range(H // 2):
                lo, hi = _deint(r32, j, 256)
                wkv_d[2 * j, rows, pl.ds(w_i * E + half * 128, 128)] = lo
                wkv_d[2 * j + 1, rows, pl.ds(w_i * E + half * 128, 128)] = hi

    def q_plain(t, carry):
        q_step(t)
        return carry

    def q_uk(t, carry):
        q_step(t)
        deint_kv(bwuk_raw, 0, t - 8)
        return carry

    def q_uv(t, carry):
        q_step(t)
        deint_kv(bwuv_raw, 1, t - 12)
        return carry

    lax.fori_loop(0, 8, q_plain, 0)
    for cp in cp_wuk:
        cp.wait()
    for cp in cp_aw + [cp_xa, cp_awo]:
        cp.start()
    lax.fori_loop(8, 12, q_uk, 0)
    for cp in cp_wuv:
        cp.wait()
    lax.fori_loop(12, 16, q_uv, 0)
    cp_c.wait()

    TQ = 256
    NQ = S // TQ
    HQ = TQ // 2

    def kv_chunk(h, slot, i):
        z = _dot(c[pl.ds(i * TQ, TQ), :], _bf(wkv_d[h]))
        kv[slot, pl.ds(i * TQ // 2, TQ // 2), :] = _u32(z.astype(BF))

    def kv0(i, carry):
        z = _dot(c[pl.ds(pl.multiple_of(i * 512, 512), 512), :], _bf(wkv_d[0]))
        kv[0, pl.ds(pl.multiple_of(i * 256, 256), 256), :] = _u32(z.astype(BF))
        return carry

    lax.fori_loop(0, S // 512, kv0, 0)
    cp_bwo.wait()
    for cp in cp_aw + [cp_xa, cp_awo]:
        cp.wait()

    RG = int(os.environ.get('RG', 8))
    CHL = [int(v) for v in os.environ.get('CH', '22222222')]
    CHZ = [int(v) for v in os.environ.get('CHZ', '42233468')]

    def attention(h, slot, filler, CHS):
        wot_h = bwot[pl.ds(pl.multiple_of(h * DM, DM), DM), :]
        row = lax.broadcasted_iota(jnp.int32, (TQ, HQ), 0)
        col = lax.broadcasted_iota(jnp.int32, (TQ, HQ), 1)
        tri_main = row >= col
        tri_tail = tri_main[0:HQ]
        blocks = list(range(NQ - 1, -1, -1))

        def scores(idx):
            i, b = blocks[idx], idx % 2
            n = (i + 1) * TQ
            nm = n - HQ
            nf = n - TQ
            q = _bf(q_all[h, pl.ds(i * TQ // 2, TQ // 2), :])
            if nf > 0:
                s_buf[b][:, 0:nf] = _dot_nt(q, _bf(kv[slot, pl.ds(0, nf // 2), 0:E]))
            s_mid = _dot_nt(q, _bf(kv[slot, pl.ds(nf // 2, HQ // 2), 0:E]))
            s_buf[b][:, nf:nm] = jnp.where(tri_main, s_mid, NEG)
            s_tail = _dot_nt(q[HQ:TQ], _bf(kv[slot, pl.ds(nm // 2, HQ // 2), 0:E]))
            s_buf[b][HQ:TQ, nm:n] = jnp.where(tri_tail, s_tail, NEG)

        def softmax(idx):
            i, b, CH = blocks[idx], idx % 2, CHS[idx]
            n = (i + 1) * TQ
            nm = n - HQ
            ls = []
            sms = []
            for g in range(TQ // RG):
                ne = nm if g * RG < HQ else n
                rows = slice(g * RG, (g + 1) * RG)
                mx = s_buf[b][rows, 0:128]
                if g >= CH:
                    mx = mx + sms[g - CH] * 0.0
                for t in range(1, ne // 128):
                    mx = jnp.maximum(mx, s_buf[b][rows, t * 128:(t + 1) * 128])
                m = jnp.broadcast_to(jnp.max(mx, axis=1, keepdims=True), (RG, 128))
                sm = None
                for t0 in range(0, ne, 256):
                    pgs = []
                    for t in range(t0, min(t0 + 256, ne), 128):
                        pg = jnp.exp2(s_buf[b][rows, t:t + 128] - m)
                        sm = pg if sm is None else sm + pg
                        pgs.append(pg)
                    p_buf[b][rows, t0:t0 + 128 * len(pgs)] = jnp.concatenate(pgs, axis=1).astype(BF)
                sms.append(sm)
                ls.append(jnp.sum(sm, axis=1, keepdims=True))
            return jnp.concatenate(ls, axis=0)

        def context(idx, l):
            i, b = blocks[idx], idx % 2
            n = (i + 1) * TQ
            nm = n - HQ
            ctx = _dot(p_buf[b][:, 0:nm], _bf(kv[slot, pl.ds(0, nm // 2), E:2 * E]))
            ctx_t = _dot(p_buf[b][HQ:TQ, nm:n], _bf(kv[slot, pl.ds(nm // 2, HQ // 2), E:2 * E]))
            ctx = jnp.concatenate([ctx[0:HQ], ctx[HQ:TQ] + ctx_t], axis=0)
            return (ctx * (1.0 / l)).astype(BF)

        def out_proj(idx, ctx):
            acct[PADL:PADL + DM, pl.ds(blocks[idx] * TQ, TQ)] += _dot_nt(wot_h, ctx)

        scores(0)
        ctx = None
        for idx in range(NQ):
            l = softmax(idx)
            filler(idx)
            if idx + 1 < NQ:
                scores(idx + 1)
            if ctx is not None:
                out_proj(idx - 1, ctx)
            ctx = context(idx, l)
        out_proj(NQ - 1, ctx)

    def deint_a(t):
        rows = pl.ds(pl.multiple_of(t * 16, 16), 16)
        for w_i in range(3):
            for half in range(2):
                r32 = a_raw.at[w_i, half].bitcast(U32).at[pl.ds(pl.multiple_of(t * 256, 256), 256)]
                for j in range(H // 2):
                    lo, hi = _deint(r32, j, 32)
                    aw_d[rows, pl.ds(w_i * HE + (2 * j) * E + half * 128, 128)] = lo
                    aw_d[rows, pl.ds(w_i * HE + (2 * j + 1) * E + half * 128, 128)] = hi

    def prep_a(t):
        awo_d[pl.ds(pl.multiple_of(t * E, E), E), :] = awot[pl.ds(pl.multiple_of(t * DM, DM), DM), :].T
        cc = pl.ds(pl.multiple_of(t * 128, 128), 128)
        xa[cc, :] = xat[:, cc].T

    def head(h, carry):
        slot = lax.bitwise_and(h, 1)

        def filler(idx):
            kv_chunk(h + 1, 1 - slot, idx)
            if idx == 0:
                deint_a(jnp.minimum(h, DM // 32 - 1))
            if idx == 1:
                prep_a(h)

        attention(h, slot, filler, CHL)
        return carry

    lax.fori_loop(0, H - 1, head, 0)

    L = 48
    LV = M + SEG
    PR = 2 * SEG
    XA = 24
    NP = NSEG // 2

    def last_filler(idx):
        if idx == 1:
            prep_a(H - 1)
        if 2 <= idx < 5:
            w_i = idx - 2
            z0 = _dot(xa[0:PR, :], _bf(aw_d[:, w_i * HE:(w_i + 1) * HE]))
            if w_i == 0:
                z0 = z0 * scale
            dst = (zq, zk, zv)[w_i]
            dst[0, 0:SEG, :] = z0[0:SEG].astype(BF)
            dst[1, 0:SEG, :] = z0[SEG:PR].astype(BF)

    zpad = jnp.zeros((4, L - LV, HE), BF)
    zk[:, LV:L, :] = zpad
    zv[:, LV:L, :] = zpad
    ox[1] = jnp.zeros(ox.shape[1:], BF)
    mem[...] = mem0_ref[...].astype(F32)

    attention(H - 1, (H - 1) % 2, last_filler, CHZ)

    def bout(i, carry):
        r = pl.ds(pl.multiple_of(i * 256, 256), 256)
        obuf[r, DM - PADL:2 * DM] = acct[:, r].astype(BF).T
        return carry

    lax.fori_loop(0, S // 256, bout, 0)

    OC = 4
    NOC = NP // OC
    ORS = OC * PR

    def out_copy(k):
        r = pl.ds(pl.multiple_of(k * ORS, ORS), ORS)
        return pltpu.make_async_copy(obuf.at[r, :], out_hbm.at[r, :], osems.at[k])

    def substep(odd, cur, n0, n1, par, rn, rp, mask_m, mask_x):
        nx = PR - XA if odd else XA
        x0 = XA if odd else 0
        R = nx + M

        def scatter(dst, z):
            if odd:
                dst[n0, XA:SEG, :] = z[0:SEG - XA].astype(BF)
                dst[n1, 0:SEG, :] = z[SEG - XA:nx].astype(BF)
            else:
                dst[n0, 0:XA, :] = z[0:XA].astype(BF)

        lhs = jnp.concatenate([xa[pl.ds(rn + x0, nx), :].astype(F32), mem[...]], axis=0).astype(BF)
        zqk = _dot(lhs, _bf(aw_d[:, 0:2 * HE]))
        zqs = zqk[:, 0:HE] * scale
        scatter(zq, zqs)
        qm = zqs[nx:R].astype(BF)
        scatter(zk, zqk[:, HE:2 * HE])
        zk[cur, SEG:LV, :] = zqk[nx:R, HE:2 * HE].astype(BF)
        sm = jnp.concatenate(
            [_dot_nt(qm[:, h * E:(h + 1) * E], zk[cur, :, h * E:(h + 1) * E]) for h in range(H)], axis=0)
        zvv = _dot(lhs, _bf(aw_d[:, 2 * HE:3 * HE]))
        scatter(zv, zvv)
        zv[cur, SEG:LV, :] = zvv[nx:R].astype(BF)
        pm = _softmax_rows(sm, mask_m)
        o0 = XA + M if odd else 0
        for h in range(H):
            ox[1 - par, o0 + nx:o0 + R, h * E:(h + 1) * E] = _dot(
                pm[h * M:(h + 1) * M].astype(BF), zv[cur, :, h * E:(h + 1) * E]).astype(BF)
        sx = jnp.concatenate(
            [_dot_nt(zq[cur, :, h * E:(h + 1) * E], zk[cur, :, h * E:(h + 1) * E]) for h in range(H)], axis=0)
        o = _dot(ox[1 - par, o0:o0 + R, :], awo_d[...])
        obuf[pl.ds(rp + x0, nx), 0:DM] = o[0:nx].astype(BF)
        mem[...] = o[nx:R]
        px = _softmax_rows(sx, mask_x).astype(BF)
        for h in range(H):
            oh = _dot(px[h * SEG:(h + 1) * SEG], zv[cur, :, h * E:(h + 1) * E])
            cols = slice(h * E, (h + 1) * E)
            if odd:
                ox[par, XA + M + SEG - XA:XA + M + PR - XA, cols] = oh.astype(BF)
            else:
                ox[par, 0:XA, cols] = oh[0:XA].astype(BF)
                ox[par, XA + M:XA + M + SEG - XA, cols] = oh[XA:SEG].astype(BF)

    def pair(t, carry):
        colm = lax.broadcasted_iota(jnp.int32, (H * M, L), 1)
        mask_m = colm < LV
        rowx = lax.bitwise_and(lax.broadcasted_iota(jnp.int32, (H * SEG, L), 0), SEG - 1)
        colx = lax.broadcasted_iota(jnp.int32, (H * SEG, L), 1)
        mask_x = (colx < LV) & ((rowx >= colx) | (colx >= SEG))
        par = lax.bitwise_and(t, 1)
        c0 = 2 * par
        n0 = 2 - c0
        rn = pl.multiple_of(jnp.minimum(t + 1, NP - 1) * PR, PR)
        rp = pl.multiple_of(jnp.maximum(t - 1, 0) * PR, PR)
        substep(False, c0, n0, n0 + 1, par, rn, rp, mask_m, mask_x)
        substep(True, c0 + 1, n0, n0 + 1, par, rn, rp, mask_m, mask_x)

        @pl.when(jnp.logical_and(lax.bitwise_and(t, OC - 1) == 0, t > 0))
        def _():
            out_copy(lax.shift_right_logical(t, 2) - 1).start()

        return carry

    lax.fori_loop(0, NP, pair, 0)
    lp = (NP - 1) % 2
    oxl = jnp.concatenate([ox[lp, 0:XA, :].astype(F32), ox[lp, XA + M:XA + M + PR - XA, :].astype(F32)], axis=0)
    obuf[S - PR:S, 0:DM] = _dot(oxl.astype(BF), awo_d[...]).astype(BF)
    out_copy(NOC - 1).start()
    for k in range(NOC):
        out_copy(k).wait()


@functools.partial(jax.jit, static_argnames=("A_seg_len",))
def pallas_concat_heads__memory_aug_recurrent_mem_tr__compressed_kv_cla__prompt_kernel(
    A_x, A_mem0, A_Wq, A_Wk, A_Wv, A_Wo, A_seg_len,
    B_x, B_c_kv, B_w_q, B_w_uk, B_w_uv, B_w_o,
):
    _, S, DM = A_x.shape
    _, H, E = A_Wq.shape
    M = A_mem0.shape[1]
    DC = B_c_kv.shape[2]
    SEG = int(A_seg_len)
    assert (S, DM, H, E, M, DC, SEG) == (2048, 448, 16, 256, 8, 1024, 32)
    HE = H * E
    any_spec = pl.BlockSpec(memory_space=pl.ANY)
    vm = pltpu.VMEM
    scratch = [
        vm((DM, S), BF), vm((S, DM), BF), vm((S, DC), BF),
        vm((2, DM * H, 128), BF), vm((2, DC * H, 128), BF), vm((2, DC * H, 128), BF),
        vm((H * DM, E), BF),
        vm((DM // 2, HE), U32), vm((H, DC // 2, 2 * E), U32),
        vm((H, S // 2, E), U32), vm((2, S // 2, 2 * E), U32),
        vm((512, S), F32),
        vm((256, S), F32), vm((256, S), F32), vm((256, S), BF), vm((256, S), BF),
        vm((DM, S), BF), vm((S, DM), BF),
        vm((3, 2, DM * H, 128), BF), vm((H * DM, E), BF),
        vm((DM // 2, 3 * HE), U32), vm((HE, DM), BF),
        vm((M, DM), F32),
        vm((4, SEG, HE), BF), vm((4, 48, HE), BF), vm((4, 48, HE), BF),
        vm((2, 80, HE), BF),
        vm((S, 2 * DM), BF),
        pltpu.SemaphoreType.DMA((17,)), pltpu.SemaphoreType.DMA((8,)),
    ]
    out = pl.pallas_call(
        functools.partial(_kernel, S=S, DM=DM, H=H, E=E, DC=DC, M=M, SEG=SEG),
        out_shape=jax.ShapeDtypeStruct((S, 2 * DM), BF),
        in_specs=[any_spec, pl.BlockSpec(memory_space=pltpu.VMEM)] + [any_spec] * 10,
        out_specs=any_spec,
        scratch_shapes=scratch,
        compiler_params=pltpu.CompilerParams(vmem_limit_bytes=126 * 1024 * 1024),
    )(
        jnp.swapaxes(A_x, 1, 2).reshape(DM, S), A_mem0.reshape(M, DM),
        A_Wq.reshape(DM * H, E), A_Wk.reshape(DM * H, E), A_Wv.reshape(DM * H, E),
        jnp.swapaxes(A_Wo, 1, 2).reshape(H * DM, E),
        jnp.swapaxes(B_x, 1, 2).reshape(DM, S), B_c_kv.reshape(S, DC),
        B_w_q.reshape(DM * H, E), B_w_uk.reshape(DC * H, E), B_w_uv.reshape(DC * H, E),
        jnp.swapaxes(B_w_o, 1, 2).reshape(H * DM, E),
    )
    return out.reshape(1, S, 2 * DM)
```

```python
import functools
import os

import jax
import jax.numpy as jnp
from jax import lax
from jax.experimental import pallas as pl
from jax.experimental.pallas import tpu as pltpu

BF = jnp.bfloat16
F32 = jnp.float32
U32 = jnp.uint32
NT = (((1,), (1,)), ((), ()))
NEG = -1000000000.0


def _bf(x32):
    return pltpu.bitcast(x32, BF)


def _u32(xb):
    return pltpu.bitcast(xb, U32)


def _dot(a, b):
    return jnp.dot(a, b, preferred_element_type=F32)


def _dot_nt(a, b):
    return lax.dot_general(a, b, NT, preferred_element_type=F32)


def _deint(raw32, j, r0, gate=None):
    ev = raw32[pl.ds(r0 * 8 + j, 8, stride=16), :]
    od = raw32[pl.ds(r0 * 8 + j + 8, 8, stride=16), :]
    if gate is not None:
        ev = ev | gate
    lo = (ev & jnp.uint32(0xFFFF)) | (od << 16)
    hi = (ev >> 16) | (od & jnp.uint32(0xFFFF0000))
    return lo, hi


def _deint_block(raw32, nrows, store, chain):
    done = []
    for r0 in range(0, nrows, 16):
        for j in range(8):
            gate = _zero_after(done[-chain]) if 0 < chain <= len(done) else None
            lo, hi = _deint(raw32, j, r0, gate)
            store(2 * j, r0 // 2, lo)
            store(2 * j + 1, r0 // 2, hi)
            done.append(hi)


def _zero_after(x):
    return (pltpu.bitcast(x, U32) >> 16) >> 16


def _softmax_rows(sc, mask):
    sc = jnp.where(mask, sc, NEG)
    m = jnp.max(sc, axis=1, keepdims=True)
    p = jnp.exp(sc - m)
    l = jnp.sum(p, axis=1, keepdims=True)
    return p * (1.0 / l)


def _kernel(xa_hbm, mem0_ref, awq_hbm, awk_hbm, awv_hbm, awo_hbm,
            xb_hbm, c_hbm, bwq_hbm, bwuk_hbm, bwuv_hbm, bwo_hbm,
            out_hbm,
            xbt, xb, c, bwq_raw, bwuk_raw, bwuv_raw, bwot, bwq_d, wkv_d, q_all, kv, acct, s_buf0, s_buf1, p_buf0, p_buf1,
            xat, xa, a_raw, awot, aw_d, awo_d, mem, zq, zk, zv, ox, obuf,
            sems, osems,
            *, S, DM, H, E, DC, M, SEG):
    HE = H * E
    NSEG = S // SEG
    scale = E ** -0.5
    s_buf = (s_buf0, s_buf1)
    p_buf = (p_buf0, p_buf1)

    def halves(src, dst, s0):
        return [pltpu.make_async_copy(src.at[:, pl.ds(i * 128, 128)], dst.at[i], sems.at[s0 + i])
                for i in range(2)]

    cp_bwq = halves(bwq_hbm, bwq_raw, 0)
    cp_xb = pltpu.make_async_copy(xb_hbm, xbt, sems.at[2])
    cp_c = pltpu.make_async_copy(c_hbm, c, sems.at[3])
    cp_wuk = halves(bwuk_hbm, bwuk_raw, 4)
    cp_wuv = halves(bwuv_hbm, bwuv_raw, 6)
    cp_bwo = pltpu.make_async_copy(bwo_hbm, bwot, sems.at[8])
    cp_aw = [halves(w, a_raw.at[i], 9 + 2 * i) for i, w in enumerate((awq_hbm, awk_hbm, awv_hbm))]
    cp_aw = cp_aw[0] + cp_aw[1] + cp_aw[2]
    cp_xa = pltpu.make_async_copy(xa_hbm, xat, sems.at[15])
    cp_awo = pltpu.make_async_copy(awo_hbm, awot, sems.at[16])

    cp_xb.start()
    cp_bwq[0].start()
    cp_bwq[1].start()
    cp_xb.wait()

    def xb_t(i, carry):
        cc = pl.ds(pl.multiple_of(i * 256, 256), 256)
        xb[cc, :] = xbt[:, cc].T
        return carry

    lax.fori_loop(0, S // 256, xb_t, 0)
    for half in range(2):
        cp_bwq[half].wait()
        if half == 1:
            for cp in cp_wuk + cp_wuv + [cp_c, cp_bwo]:
                cp.start()

        def bwq_body(t, carry, half=half):
            r32 = bwq_raw.at[half].bitcast(U32).at[pl.ds(pl.multiple_of(t * 512, 512), 512)]
            dst = bwq_d.at[pl.ds(pl.multiple_of(t * 32, 32), 32)]

            def store(hd, r, v):
                dst[r:r + 8, hd * E + half * 128:hd * E + half * 128 + 128] = v

            _deint_block(r32, 64, store, 0)
            return carry

        lax.fori_loop(0, DM // 64, bwq_body, 0)

    TQP = 512
    PADL = 512 - DM
    ZR = 512 // 16
    scale2 = scale * 1.4426950408889634

    def q_step(t):
        i = lax.shift_right_logical(t, 2)
        n = lax.bitwise_and(t, 3)
        r0 = pl.multiple_of(i * TQP, TQP)
        c0 = pl.multiple_of(n * 4 * E, 4 * E)
        z = _dot(xb[pl.ds(r0, TQP), :], _bf(bwq_d[:, pl.ds(c0, 4 * E)])) * scale2
        z = _u32(z.astype(BF))
        rr = pl.ds(pl.multiple_of(i * (TQP // 2), TQP // 2), TQP // 2)
        for hh in range(4):
            q_all[n * 4 + hh, rr, :] = z[:, hh * E:(hh + 1) * E]
        acct[pl.ds(pl.multiple_of(t * ZR, ZR), ZR), :] = jnp.zeros((ZR, S), F32)

    DCH = int(os.environ.get('DCH', 1))

    def deint_kv(t):
        for w_i, raw in enumerate((bwuk_raw, bwuv_raw)):
            for half in range(2):
                r32 = raw.at[half].bitcast(U32).at[pl.ds(pl.multiple_of(t * 1024, 1024), 1024)]
                dst = wkv_d.at[:, pl.ds(pl.multiple_of(t * 64, 64), 64)]

                def store(hd, r, v, c0=w_i * E + half * 128, dst=dst):
                    dst[hd, r:r + 8, c0:c0 + 128] = v

                _deint_block(r32, 128, store, DCH)

    def q_plain(t, carry):
        q_step(t)
        return carry

    def q_kv(t, carry):
        q_step(t)
        deint_kv(t - 8)
        return carry

    lax.fori_loop(0, 8, q_plain, 0)
    for cp in cp_wuk + cp_wuv:
        cp.wait()
    for cp in cp_aw + [cp_xa, cp_awo]:
        cp.start()
    lax.fori_loop(8, 16, q_kv, 0)
    cp_c.wait()

    TQ = 256
    NQ = S // TQ
    HQ = TQ // 2

    def kv_chunk(h, slot, r0, nr):
        z = _dot(c[pl.ds(r0, nr), :], _bf(wkv_d[h]))
        kv[slot, pl.ds(r0 // 2, nr // 2), :] = _u32(z.astype(BF))

    KD = int(os.environ.get('KD', 512))
    kv_chunk(0, 0, 0, KD)
    cp_bwo.wait()
    for cp in cp_aw + [cp_xa, cp_awo]:
        cp.wait()

    RG = int(os.environ.get('RG', 8))
    CHL = [int(v) for v in os.environ.get('CH', '83222222')]

    def attention(h, slot, filler, CHS):
        wot_h = bwot[pl.ds(pl.multiple_of(h * DM, DM), DM), :]
        row = lax.broadcasted_iota(jnp.int32, (TQ, HQ), 0)
        col = lax.broadcasted_iota(jnp.int32, (TQ, HQ), 1)
        tri_main = row >= col
        tri_tail = tri_main[0:HQ]
        blocks = list(range(NQ))

        def scores(idx):
            i, b = blocks[idx], idx % 2
            n = (i + 1) * TQ
            nm = n - HQ
            nf = n - TQ
            q = _bf(q_all[h, pl.ds(i * TQ // 2, TQ // 2), :])
            if nf > 0:
                s_buf[b][:, 0:nf] = _dot_nt(q, _bf(kv[slot, pl.ds(0, nf // 2), 0:E]))
            s_mid = _dot_nt(q, _bf(kv[slot, pl.ds(nf // 2, HQ // 2), 0:E]))
            s_buf[b][:, nf:nm] = jnp.where(tri_main, s_mid, NEG)
            s_tail = _dot_nt(q[HQ:TQ], _bf(kv[slot, pl.ds(nm // 2, HQ // 2), 0:E]))
            s_buf[b][HQ:TQ, nm:n] = jnp.where(tri_tail, s_tail, NEG)

        def softmax(idx):
            i, b, CH = blocks[idx], idx % 2, CHS[idx]
            n = (i + 1) * TQ
            nm = n - HQ
            ls = []
            sms = []
            for g in range(TQ // RG):
                ne = nm if g * RG < HQ else n
                rows = slice(g * RG, (g + 1) * RG)
                mx = s_buf[b][rows, 0:128]
                if g >= CH:
                    mx = mx + sms[g - CH] * 0.0
                for t in range(1, ne // 128):
                    mx = jnp.maximum(mx, s_buf[b][rows, t * 128:(t + 1) * 128])
                m = jnp.broadcast_to(jnp.max(mx, axis=1, keepdims=True), (RG, 128))
                sm = None
                for t0 in range(0, ne, 256):
                    pgs = []
                    for t in range(t0, min(t0 + 256, ne), 128):
                        pg = jnp.exp2(s_buf[b][rows, t:t + 128] - m)
                        sm = pg if sm is None else sm + pg
                        pgs.append(pg)
                    p_buf[b][rows, t0:t0 + 128 * len(pgs)] = jnp.concatenate(pgs, axis=1).astype(BF)
                sms.append(sm)
                ls.append(jnp.sum(sm, axis=1, keepdims=True))
            return jnp.concatenate(ls, axis=0)

        def context(idx, l):
            i, b = blocks[idx], idx % 2
            n = (i + 1) * TQ
            nm = n - HQ
            ctx = _dot(p_buf[b][:, 0:nm], _bf(kv[slot, pl.ds(0, nm // 2), E:2 * E]))
            ctx_t = _dot(p_buf[b][HQ:TQ, nm:n], _bf(kv[slot, pl.ds(nm // 2, HQ // 2), E:2 * E]))
            ctx = jnp.concatenate([ctx[0:HQ], ctx[HQ:TQ] + ctx_t], axis=0)
            return (ctx * (1.0 / l)).astype(BF)

        def out_proj(idx, ctx):
            acct[PADL:PADL + DM, pl.ds(blocks[idx] * TQ, TQ)] += _dot_nt(wot_h, ctx)

        scores(0)
        ctx = None
        for idx in range(NQ):
            l = softmax(idx)
            filler(idx)
            if idx + 1 < NQ:
                scores(idx + 1)
            if ctx is not None:
                out_proj(idx - 1, ctx)
            ctx = context(idx, l)
        out_proj(NQ - 1, ctx)

    def deint_a(t):
        dst = aw_d.at[pl.ds(pl.multiple_of(t * 16, 16), 16)]
        for w_i in range(3):
            for half in range(2):
                r32 = a_raw.at[w_i, half].bitcast(U32).at[pl.ds(pl.multiple_of(t * 256, 256), 256)]

                def store(hd, r, v, c0=w_i * HE + half * 128):
                    dst[r:r + 8, c0 + hd * E:c0 + hd * E + 128] = v

                _deint_block(r32, 32, store, DCH)

    def prep_a(t):
        awo_d[pl.ds(pl.multiple_of(t * E, E), E), :] = awot[pl.ds(pl.multiple_of(t * DM, DM), DM), :].T
        cc = pl.ds(pl.multiple_of(t * 128, 128), 128)
        xa[cc, :] = xat[:, cc].T

    def head(h, carry):
        slot = lax.bitwise_and(h, 1)
        hn = jnp.minimum(h + 1, H - 1)

        def filler(idx):
            if KD == 256:
                if idx < NQ - 1:
                    kv_chunk(h, slot, (idx + 1) * TQ, TQ)
                else:
                    kv_chunk(hn, 1 - slot, 0, TQ)
            else:
                if 1 <= idx < NQ - 1:
                    kv_chunk(h, slot, (idx + 1) * TQ, TQ)
                elif idx == NQ - 1:
                    kv_chunk(hn, 1 - slot, 0, 2 * TQ)
            if idx == 2:
                deint_a(jnp.minimum(h, DM // 32 - 1))
            if idx == 3:
                prep_a(h)

        attention(h, slot, filler, CHL)
        return carry

    lax.fori_loop(0, H, head, 0)

    L = 48
    LV = M + SEG
    PR = 2 * SEG
    XA = 24
    NP = NSEG // 2

    zpad = jnp.zeros((4, L - LV, HE), BF)
    zk[:, LV:L, :] = zpad
    zv[:, LV:L, :] = zpad
    ox[1] = jnp.zeros(ox.shape[1:], BF)
    mem[...] = mem0_ref[...].astype(F32)

    def a_pro(t, carry):
        cols = pl.ds(pl.multiple_of(t * 1024, 1024), 1024)
        for w_i, dst in enumerate((zq, zk, zv)):
            z0 = _dot(xa[0:PR, :], _bf(aw_d[:, pl.ds(pl.multiple_of(w_i * HE + t * 1024, 1024), 1024)]))
            if w_i == 0:
                z0 = z0 * scale
            dst[0, 0:SEG, cols] = z0[0:SEG].astype(BF)
            dst[1, 0:SEG, cols] = z0[SEG:PR].astype(BF)
        return carry

    lax.fori_loop(0, HE // 1024, a_pro, 0)

    def bout(i, carry):
        r = pl.ds(pl.multiple_of(i * 256, 256), 256)
        obuf[r, DM - PADL:2 * DM] = acct[:, r].astype(BF).T
        return carry

    lax.fori_loop(0, S // 256, bout, 0)

    OC = 4
    NOC = NP // OC
    ORS = OC * PR

    def out_copy(k):
        r = pl.ds(pl.multiple_of(k * ORS, ORS), ORS)
        return pltpu.make_async_copy(obuf.at[r, :], out_hbm.at[r, :], osems.at[k])

    def substep(odd, cur, n0, n1, par, rn, rp, mask_m, mask_x):
        nx = PR - XA if odd else XA
        x0 = XA if odd else 0
        R = nx + M

        def scatter(dst, z):
            if odd:
                dst[n0, XA:SEG, :] = z[0:SEG - XA].astype(BF)
                dst[n1, 0:SEG, :] = z[SEG - XA:nx].astype(BF)
            else:
                dst[n0, 0:XA, :] = z[0:XA].astype(BF)

        lhs = jnp.concatenate([xa[pl.ds(rn + x0, nx), :].astype(F32), mem[...]], axis=0).astype(BF)
        zqk = _dot(lhs, _bf(aw_d[:, 0:2 * HE]))
        zqs = zqk[:, 0:HE] * scale
        scatter(zq, zqs)
        qm = zqs[nx:R].astype(BF)
        scatter(zk, zqk[:, HE:2 * HE])
        zk[cur, SEG:LV, :] = zqk[nx:R, HE:2 * HE].astype(BF)
        sm = jnp.concatenate(
            [_dot_nt(qm[:, h * E:(h + 1) * E], zk[cur, :, h * E:(h + 1) * E]) for h in range(H)], axis=0)
        zvv = _dot(lhs, _bf(aw_d[:, 2 * HE:3 * HE]))
        scatter(zv, zvv)
        zv[cur, SEG:LV, :] = zvv[nx:R].astype(BF)
        pm = _softmax_rows(sm, mask_m)
        o0 = XA + M if odd else 0
        for h in range(H):
            ox[1 - par, o0 + nx:o0 + R, h * E:(h + 1) * E] = _dot(
                pm[h * M:(h + 1) * M].astype(BF), zv[cur, :, h * E:(h + 1) * E]).astype(BF)
        sx = jnp.concatenate(
            [_dot_nt(zq[cur, :, h * E:(h + 1) * E], zk[cur, :, h * E:(h + 1) * E]) for h in range(H)], axis=0)
        o = _dot(ox[1 - par, o0:o0 + R, :], awo_d[...])
        obuf[pl.ds(rp + x0, nx), 0:DM] = o[0:nx].astype(BF)
        mem[...] = o[nx:R]
        px = _softmax_rows(sx, mask_x).astype(BF)
        for h in range(H):
            oh = _dot(px[h * SEG:(h + 1) * SEG], zv[cur, :, h * E:(h + 1) * E])
            cols = slice(h * E, (h + 1) * E)
            if odd:
                ox[par, XA + M + SEG - XA:XA + M + PR - XA, cols] = oh.astype(BF)
            else:
                ox[par, 0:XA, cols] = oh[0:XA].astype(BF)
                ox[par, XA + M:XA + M + SEG - XA, cols] = oh[XA:SEG].astype(BF)

    def pair(t, carry):
        colm = lax.broadcasted_iota(jnp.int32, (H * M, L), 1)
        mask_m = colm < LV
        rowx = lax.bitwise_and(lax.broadcasted_iota(jnp.int32, (H * SEG, L), 0), SEG - 1)
        colx = lax.broadcasted_iota(jnp.int32, (H * SEG, L), 1)
        mask_x = (colx < LV) & ((rowx >= colx) | (colx >= SEG))
        par = lax.bitwise_and(t, 1)
        c0 = 2 * par
        n0 = 2 - c0
        rn = pl.multiple_of(jnp.minimum(t + 1, NP - 1) * PR, PR)
        rp = pl.multiple_of(jnp.maximum(t - 1, 0) * PR, PR)
        substep(False, c0, n0, n0 + 1, par, rn, rp, mask_m, mask_x)
        substep(True, c0 + 1, n0, n0 + 1, par, rn, rp, mask_m, mask_x)

        @pl.when(jnp.logical_and(lax.bitwise_and(t, OC - 1) == 0, t > 0))
        def _():
            out_copy(lax.shift_right_logical(t, 2) - 1).start()

        return carry

    lax.fori_loop(0, NP, pair, 0)
    lp = (NP - 1) % 2
    oxl = jnp.concatenate([ox[lp, 0:XA, :].astype(F32), ox[lp, XA + M:XA + M + PR - XA, :].astype(F32)], axis=0)
    obuf[S - PR:S, 0:DM] = _dot(oxl.astype(BF), awo_d[...]).astype(BF)
    out_copy(NOC - 1).start()
    for k in range(NOC):
        out_copy(k).wait()


@functools.partial(jax.jit, static_argnames=("A_seg_len",))
def pallas_concat_heads__memory_aug_recurrent_mem_tr__compressed_kv_cla__prompt_kernel(
    A_x, A_mem0, A_Wq, A_Wk, A_Wv, A_Wo, A_seg_len,
    B_x, B_c_kv, B_w_q, B_w_uk, B_w_uv, B_w_o,
):
    _, S, DM = A_x.shape
    _, H, E = A_Wq.shape
    M = A_mem0.shape[1]
    DC = B_c_kv.shape[2]
    SEG = int(A_seg_len)
    assert (S, DM, H, E, M, DC, SEG) == (2048, 448, 16, 256, 8, 1024, 32)
    HE = H * E
    any_spec = pl.BlockSpec(memory_space=pl.ANY)
    vm = pltpu.VMEM
    scratch = [
        vm((DM, S), BF), vm((S, DM), BF), vm((S, DC), BF),
        vm((2, DM * H, 128), BF), vm((2, DC * H, 128), BF), vm((2, DC * H, 128), BF),
        vm((H * DM, E), BF),
        vm((DM // 2, HE), U32), vm((H, DC // 2, 2 * E), U32),
        vm((H, S // 2, E), U32), vm((2, S // 2, 2 * E), U32),
        vm((512, S), F32),
        vm((256, S), F32), vm((256, S), F32), vm((256, S), BF), vm((256, S), BF),
        vm((DM, S), BF), vm((S, DM), BF),
        vm((3, 2, DM * H, 128), BF), vm((H * DM, E), BF),
        vm((DM // 2, 3 * HE), U32), vm((HE, DM), BF),
        vm((M, DM), F32),
        vm((4, SEG, HE), BF), vm((4, 48, HE), BF), vm((4, 48, HE), BF),
        vm((2, 80, HE), BF),
        vm((S, 2 * DM), BF),
        pltpu.SemaphoreType.DMA((17,)), pltpu.SemaphoreType.DMA((8,)),
    ]
    out = pl.pallas_call(
        functools.partial(_kernel, S=S, DM=DM, H=H, E=E, DC=DC, M=M, SEG=SEG),
        out_shape=jax.ShapeDtypeStruct((S, 2 * DM), BF),
        in_specs=[any_spec, pl.BlockSpec(memory_space=pltpu.VMEM)] + [any_spec] * 10,
        out_specs=any_spec,
        scratch_shapes=scratch,
        compiler_params=pltpu.CompilerParams(vmem_limit_bytes=126 * 1024 * 1024),
    )(
        jnp.swapaxes(A_x, 1, 2).reshape(DM, S), A_mem0.reshape(M, DM),
        A_Wq.reshape(DM * H, E), A_Wk.reshape(DM * H, E), A_Wv.reshape(DM * H, E),
        jnp.swapaxes(A_Wo, 1, 2).reshape(H * DM, E),
        jnp.swapaxes(B_x, 1, 2).reshape(DM, S), B_c_kv.reshape(S, DC),
        B_w_q.reshape(DM * H, E), B_w_uk.reshape(DC * H, E), B_w_uv.reshape(DC * H, E),
        jnp.swapaxes(B_w_o, 1, 2).reshape(H * DM, E),
    )
    return out.reshape(1, S, 2 * DM)
```

```python
import functools
import os

import jax
import jax.numpy as jnp
from jax import lax
from jax.experimental import pallas as pl
from jax.experimental.pallas import tpu as pltpu

BF = jnp.bfloat16
F32 = jnp.float32
U32 = jnp.uint32
NT = (((1,), (1,)), ((), ()))
NEG = -1000000000.0


def _bf(x32):
    return pltpu.bitcast(x32, BF)


def _u32(xb):
    return pltpu.bitcast(xb, U32)


def _dot(a, b):
    return jnp.dot(a, b, preferred_element_type=F32)


def _dot_nt(a, b):
    return lax.dot_general(a, b, NT, preferred_element_type=F32)


def _deint(raw32, j, r0, gate=None):
    ev = raw32[pl.ds(r0 * 8 + j, 8, stride=16), :]
    od = raw32[pl.ds(r0 * 8 + j + 8, 8, stride=16), :]
    if gate is not None:
        ev = ev | gate
    lo = (ev & jnp.uint32(0xFFFF)) | (od << 16)
    hi = (ev >> 16) | (od & jnp.uint32(0xFFFF0000))
    return lo, hi


def _deint_block(raw32, nrows, store, chain):
    done = []
    for r0 in range(0, nrows, 16):
        for j in range(8):
            gate = _zero_after(done[-chain]) if 0 < chain <= len(done) else None
            lo, hi = _deint(raw32, j, r0, gate)
            store(2 * j, r0 // 2, lo)
            store(2 * j + 1, r0 // 2, hi)
            done.append(hi)


def _zero_after(x):
    return (pltpu.bitcast(x, U32) >> 16) >> 16


def _softmax_rows(sc, mask):
    sc = jnp.where(mask, sc, NEG)
    m = jnp.max(sc, axis=1, keepdims=True)
    p = jnp.exp(sc - m)
    l = jnp.sum(p, axis=1, keepdims=True)
    return p * (1.0 / l)


def _kernel(xa_hbm, mem0_ref, awq_hbm, awk_hbm, awv_hbm, awo_hbm,
            xb_hbm, c_hbm, bwq_hbm, bwuk_hbm, bwuv_hbm, bwo_hbm,
            out_hbm,
            xbt, xb, c, bwq_raw, bwuk_raw, bwuv_raw, bwot, bwq_d, wkv_d, q_all, kv, acct, s_buf0, s_buf1, p_buf0, p_buf1,
            xat, xa, a_raw, awot, aw_d, awo_d, mem, zq, zk, zv, ox, obuf,
            sems, osems,
            *, S, DM, H, E, DC, M, SEG):
    HE = H * E
    NSEG = S // SEG
    scale = E ** -0.5
    s_buf = (s_buf0, s_buf1)
    p_buf = (p_buf0, p_buf1)

    nsem = [0]

    def copy(src, dst):
        nsem[0] += 1
        return pltpu.make_async_copy(src, dst, sems.at[nsem[0] - 1])

    def slab(src, dst, part):
        nr = src.shape[0] // 2
        rows = pl.ds(part * nr, nr)
        return [copy(src.at[rows, pl.ds(i * 128, 128)], dst.at[i, rows]) for i in range(2)]

    def rows_half(src, dst, part):
        nr = src.shape[0] // 2
        return copy(src.at[pl.ds(part * nr, nr)], dst.at[pl.ds(part * nr, nr)])

    cp_bwq = [copy(bwq_hbm.at[:, pl.ds(i * 128, 128)], bwq_raw.at[i]) for i in range(2)]
    cp_xb = copy(xb_hbm, xbt)
    cp_c = copy(c_hbm, c)
    cp_xa = copy(xa_hbm, xat)
    cp_wkv = [slab(bwuk_hbm, bwuk_raw, p) + slab(bwuv_hbm, bwuv_raw, p) for p in range(2)]
    cp_late = [[rows_half(bwo_hbm, bwot, p), rows_half(awo_hbm, awot, p)]
               + slab(awq_hbm, a_raw.at[0], p) + slab(awk_hbm, a_raw.at[1], p) + slab(awv_hbm, a_raw.at[2], p)
               for p in range(2)]

    def start(cps):
        for cp in cps:
            cp.start()

    def wait(cps):
        for cp in cps:
            cp.wait()

    TQP = 512
    PADL = 512 - DM
    ZR = 512 // 16
    scale2 = scale * 1.4426950408889634

    def xb_t(i):
        cc = pl.ds(pl.multiple_of(i * 256, 256), 256)
        xb[cc, :] = xbt[:, cc].T

    def deint_bwq(half):
        def body(t, carry):
            r32 = bwq_raw.at[half].bitcast(U32).at[pl.ds(pl.multiple_of(t * 512, 512), 512)]
            dst = bwq_d.at[half, pl.ds(pl.multiple_of(t * 32, 32), 32)]

            def store(hd, r, v):
                dst[r:r + 8, hd * 128:(hd + 1) * 128] = v

            _deint_block(r32, 64, store, 0)
            return carry

        lax.fori_loop(0, DM // 64, body, 0)

    def q_step(half, t):
        i = lax.shift_right_logical(t, 1)
        n = lax.bitwise_and(t, 1)
        r0 = pl.multiple_of(i * TQP, TQP)
        c0 = pl.multiple_of(n * 1024, 1024)
        z = _dot(xb[pl.ds(r0, TQP), :], _bf(bwq_d[half, :, pl.ds(c0, 1024)])) * scale2
        z = _u32(z.astype(BF))
        rr = pl.ds(pl.multiple_of(i * (TQP // 2), TQP // 2), TQP // 2)
        for hh in range(8):
            q_all[n * 8 + hh, rr, half * 128:(half + 1) * 128] = z[:, hh * 128:(hh + 1) * 128]
        acct[pl.ds(pl.multiple_of((half * 8 + t) * ZR, ZR), ZR), :] = jnp.zeros((ZR, S), F32)

    start([cp_xb, cp_bwq[0]])
    cp_xb.wait()

    def xb_t0(i, carry):
        xb_t(i)
        return carry

    lax.fori_loop(0, 2, xb_t0, 0)
    cp_bwq[0].wait()
    start([cp_bwq[1]] + cp_wkv[0])
    deint_bwq(0)

    DCH = int(os.environ.get('DCH', 1))

    def deint_kv(t):
        for w_i, raw in enumerate((bwuk_raw, bwuv_raw)):
            for half in range(2):
                r32 = raw.at[half].bitcast(U32).at[pl.ds(pl.multiple_of(t * 1024, 1024), 1024)]
                dst = wkv_d.at[:, pl.ds(pl.multiple_of(t * 64, 64), 64)]

                def store(hd, r, v, c0=w_i * E + half * 128, dst=dst):
                    dst[hd, r:r + 8, c0:c0 + 128] = v

                _deint_block(r32, 128, store, DCH)

    W3 = int(os.environ.get('W3', 4))
    W4 = int(os.environ.get('W4', 2))

    def q_lo(t, carry):
        @pl.when(t == W3)
        def _():
            start(cp_wkv[1] + [cp_c])

        q_step(0, t)
        xb_t(jnp.minimum(t + 2, S // 256 - 1))
        return carry

    def q_hi(t, carry):
        @pl.when(t == W4)
        def _():
            start([cp_xa] + cp_late[0])

        @pl.when(t == 4)
        def _():
            wait(cp_wkv[1])

        q_step(1, t)
        deint_kv(t)
        return carry

    lax.fori_loop(0, 8, q_lo, 0)
    cp_bwq[1].wait()
    deint_bwq(1)
    wait(cp_wkv[0])
    lax.fori_loop(0, 8, q_hi, 0)
    cp_c.wait()

    TQ = 256
    NQ = S // TQ
    HQ = TQ // 2

    def kv_chunk(h, slot, r0, nr):
        z = _dot(c[pl.ds(r0, nr), :], _bf(wkv_d[h]))
        kv[slot, pl.ds(r0 // 2, nr // 2), :] = _u32(z.astype(BF))

    KD = int(os.environ.get('KD', 512))
    kv_chunk(0, 0, 0, KD)
    wait([cp_xa] + cp_late[0])
    start(cp_late[1])

    RG = int(os.environ.get('RG', 8))
    CHL = [int(v) for v in os.environ.get('CH', '83222222')]

    def attention(h, slot, filler, CHS):
        wot_h = bwot[pl.ds(pl.multiple_of(h * DM, DM), DM), :]
        row = lax.broadcasted_iota(jnp.int32, (TQ, HQ), 0)
        col = lax.broadcasted_iota(jnp.int32, (TQ, HQ), 1)
        tri_main = row >= col
        tri_tail = tri_main[0:HQ]
        blocks = list(range(NQ))

        def scores(idx):
            i, b = blocks[idx], idx % 2
            n = (i + 1) * TQ
            nm = n - HQ
            nf = n - TQ
            q = _bf(q_all[h, pl.ds(i * TQ // 2, TQ // 2), :])
            if nf > 0:
                s_buf[b][:, 0:nf] = _dot_nt(q, _bf(kv[slot, pl.ds(0, nf // 2), 0:E]))
            s_mid = _dot_nt(q, _bf(kv[slot, pl.ds(nf // 2, HQ // 2), 0:E]))
            s_buf[b][:, nf:nm] = jnp.where(tri_main, s_mid, NEG)
            s_tail = _dot_nt(q[HQ:TQ], _bf(kv[slot, pl.ds(nm // 2, HQ // 2), 0:E]))
            s_buf[b][HQ:TQ, nm:n] = jnp.where(tri_tail, s_tail, NEG)

        def softmax(idx):
            i, b, CH = blocks[idx], idx % 2, CHS[idx]
            n = (i + 1) * TQ
            nm = n - HQ
            ls = []
            sms = []
            for g in range(TQ // RG):
                ne = nm if g * RG < HQ else n
                rows = slice(g * RG, (g + 1) * RG)
                mx = s_buf[b][rows, 0:128]
                if g >= CH:
                    mx = mx + sms[g - CH] * 0.0
                for t in range(1, ne // 128):
                    mx = jnp.maximum(mx, s_buf[b][rows, t * 128:(t + 1) * 128])
                m = jnp.broadcast_to(jnp.max(mx, axis=1, keepdims=True), (RG, 128))
                sm = None
                for t0 in range(0, ne, 256):
                    pgs = []
                    for t in range(t0, min(t0 + 256, ne), 128):
                        pg = jnp.exp2(s_buf[b][rows, t:t + 128] - m)
                        sm = pg if sm is None else sm + pg
                        pgs.append(pg)
                    p_buf[b][rows, t0:t0 + 128 * len(pgs)] = jnp.concatenate(pgs, axis=1).astype(BF)
                sms.append(sm)
                ls.append(jnp.sum(sm, axis=1, keepdims=True))
            return jnp.concatenate(ls, axis=0)

        def context(idx, l):
            i, b = blocks[idx], idx % 2
            n = (i + 1) * TQ
            nm = n - HQ
            ctx = _dot(p_buf[b][:, 0:nm], _bf(kv[slot, pl.ds(0, nm // 2), E:2 * E]))
            ctx_t = _dot(p_buf[b][HQ:TQ, nm:n], _bf(kv[slot, pl.ds(nm // 2, HQ // 2), E:2 * E]))
            ctx = jnp.concatenate([ctx[0:HQ], ctx[HQ:TQ] + ctx_t], axis=0)
            return (ctx * (1.0 / l)).astype(BF)

        def out_proj(idx, ctx):
            acct[PADL:PADL + DM, pl.ds(blocks[idx] * TQ, TQ)] += _dot_nt(wot_h, ctx)

        scores(0)
        ctx = None
        for idx in range(NQ):
            l = softmax(idx)
            filler(idx)
            if idx + 1 < NQ:
                scores(idx + 1)
            if ctx is not None:
                out_proj(idx - 1, ctx)
            ctx = context(idx, l)
        out_proj(NQ - 1, ctx)

    def deint_a(t):
        dst = aw_d.at[pl.ds(pl.multiple_of(t * 16, 16), 16)]
        for w_i in range(3):
            for half in range(2):
                r32 = a_raw.at[w_i, half].bitcast(U32).at[pl.ds(pl.multiple_of(t * 256, 256), 256)]

                def store(hd, r, v, c0=w_i * HE + half * 128):
                    dst[r:r + 8, c0 + hd * E:c0 + hd * E + 128] = v

                _deint_block(r32, 32, store, DCH)

    def prep_a(t):
        awo_d[pl.ds(pl.multiple_of(t * E, E), E), :] = awot[pl.ds(pl.multiple_of(t * DM, DM), DM), :].T
        cc = pl.ds(pl.multiple_of(t * 128, 128), 128)
        xa[cc, :] = xat[:, cc].T

    def head(h, carry):
        slot = lax.bitwise_and(h, 1)
        hn = jnp.minimum(h + 1, H - 1)

        @pl.when(h == DM // 64)
        def _():
            wait(cp_late[1])

        def filler(idx):
            if KD == 256:
                if idx < NQ - 1:
                    kv_chunk(h, slot, (idx + 1) * TQ, TQ)
                else:
                    kv_chunk(hn, 1 - slot, 0, TQ)
            else:
                if 1 <= idx < NQ - 1:
                    kv_chunk(h, slot, (idx + 1) * TQ, TQ)
                elif idx == NQ - 1:
                    kv_chunk(hn, 1 - slot, 0, 2 * TQ)
            if idx == 2:
                deint_a(jnp.minimum(h, DM // 32 - 1))
            if idx == 3:
                prep_a(h)

        attention(h, slot, filler, CHL)
        return carry

    lax.fori_loop(0, H, head, 0)

    L = 48
    LV = M + SEG
    PR = 2 * SEG
    XA = 24
    NP = NSEG // 2

    zpad = jnp.zeros((4, L - LV, HE), BF)
    zk[:, LV:L, :] = zpad
    zv[:, LV:L, :] = zpad
    ox[1] = jnp.zeros(ox.shape[1:], BF)
    mem[...] = mem0_ref[...].astype(F32)

    def a_pro(t, carry):
        cols = pl.ds(pl.multiple_of(t * 1024, 1024), 1024)
        for w_i, dst in enumerate((zq, zk, zv)):
            z0 = _dot(xa[0:PR, :], _bf(aw_d[:, pl.ds(pl.multiple_of(w_i * HE + t * 1024, 1024), 1024)]))
            if w_i == 0:
                z0 = z0 * scale
            dst[0, 0:SEG, cols] = z0[0:SEG].astype(BF)
            dst[1, 0:SEG, cols] = z0[SEG:PR].astype(BF)
        return carry

    lax.fori_loop(0, HE // 1024, a_pro, 0)

    def bout(i, carry):
        r = pl.ds(pl.multiple_of(i * 256, 256), 256)
        obuf[r, DM - PADL:2 * DM] = acct[:, r].astype(BF).T
        return carry

    lax.fori_loop(0, S // 256, bout, 0)

    OC = 4
    NOC = NP // OC
    ORS = OC * PR

    def out_copy(k):
        r = pl.ds(pl.multiple_of(k * ORS, ORS), ORS)
        return pltpu.make_async_copy(obuf.at[r, :], out_hbm.at[r, :], osems.at[k])

    def substep(odd, cur, n0, n1, par, rn, rp, mask_m, mask_x):
        nx = PR - XA if odd else XA
        x0 = XA if odd else 0
        R = nx + M

        def scatter(dst, z):
            if odd:
                dst[n0, XA:SEG, :] = z[0:SEG - XA].astype(BF)
                dst[n1, 0:SEG, :] = z[SEG - XA:nx].astype(BF)
            else:
                dst[n0, 0:XA, :] = z[0:XA].astype(BF)

        lhs = jnp.concatenate([xa[pl.ds(rn + x0, nx), :].astype(F32), mem[...]], axis=0).astype(BF)
        zqk = _dot(lhs, _bf(aw_d[:, 0:2 * HE]))
        zqs = zqk[:, 0:HE] * scale
        scatter(zq, zqs)
        qm = zqs[nx:R].astype(BF)
        scatter(zk, zqk[:, HE:2 * HE])
        zk[cur, SEG:LV, :] = zqk[nx:R, HE:2 * HE].astype(BF)
        sm = jnp.concatenate(
            [_dot_nt(qm[:, h * E:(h + 1) * E], zk[cur, :, h * E:(h + 1) * E]) for h in range(H)], axis=0)
        zvv = _dot(lhs, _bf(aw_d[:, 2 * HE:3 * HE]))
        scatter(zv, zvv)
        zv[cur, SEG:LV, :] = zvv[nx:R].astype(BF)
        pm = _softmax_rows(sm, mask_m)
        o0 = XA + M if odd else 0
        for h in range(H):
            ox[1 - par, o0 + nx:o0 + R, h * E:(h + 1) * E] = _dot(
                pm[h * M:(h + 1) * M].astype(BF), zv[cur, :, h * E:(h + 1) * E]).astype(BF)
        sx = jnp.concatenate(
            [_dot_nt(zq[cur, :, h * E:(h + 1) * E], zk[cur, :, h * E:(h + 1) * E]) for h in range(H)], axis=0)
        o = _dot(ox[1 - par, o0:o0 + R, :], awo_d[...])
        obuf[pl.ds(rp + x0, nx), 0:DM] = o[0:nx].astype(BF)
        mem[...] = o[nx:R]
        px = _softmax_rows(sx, mask_x).astype(BF)
        for h in range(H):
            oh = _dot(px[h * SEG:(h + 1) * SEG], zv[cur, :, h * E:(h + 1) * E])
            cols = slice(h * E, (h + 1) * E)
            if odd:
                ox[par, XA + M + SEG - XA:XA + M + PR - XA, cols] = oh.astype(BF)
            else:
                ox[par, 0:XA, cols] = oh[0:XA].astype(BF)
                ox[par, XA + M:XA + M + SEG - XA, cols] = oh[XA:SEG].astype(BF)

    def pair(t, carry):
        colm = lax.broadcasted_iota(jnp.int32, (H * M, L), 1)
        mask_m = colm < LV
        rowx = lax.bitwise_and(lax.broadcasted_iota(jnp.int32, (H * SEG, L), 0), SEG - 1)
        colx = lax.broadcasted_iota(jnp.int32, (H * SEG, L), 1)
        mask_x = (colx < LV) & ((rowx >= colx) | (colx >= SEG))
        par = lax.bitwise_and(t, 1)
        c0 = 2 * par
        n0 = 2 - c0
        rn = pl.multiple_of(jnp.minimum(t + 1, NP - 1) * PR, PR)
        rp = pl.multiple_of(jnp.maximum(t - 1, 0) * PR, PR)
        substep(False, c0, n0, n0 + 1, par, rn, rp, mask_m, mask_x)
        substep(True, c0 + 1, n0, n0 + 1, par, rn, rp, mask_m, mask_x)

        @pl.when(jnp.logical_and(lax.bitwise_and(t, OC - 1) == 0, t > 0))
        def _():
            out_copy(lax.shift_right_logical(t, 2) - 1).start()

        return carry

    lax.fori_loop(0, NP, pair, 0)
    lp = (NP - 1) % 2
    oxl = jnp.concatenate([ox[lp, 0:XA, :].astype(F32), ox[lp, XA + M:XA + M + PR - XA, :].astype(F32)], axis=0)
    obuf[S - PR:S, 0:DM] = _dot(oxl.astype(BF), awo_d[...]).astype(BF)
    out_copy(NOC - 1).start()
    for k in range(NOC):
        out_copy(k).wait()


@functools.partial(jax.jit, static_argnames=("A_seg_len",))
def pallas_concat_heads__memory_aug_recurrent_mem_tr__compressed_kv_cla__prompt_kernel(
    A_x, A_mem0, A_Wq, A_Wk, A_Wv, A_Wo, A_seg_len,
    B_x, B_c_kv, B_w_q, B_w_uk, B_w_uv, B_w_o,
):
    _, S, DM = A_x.shape
    _, H, E = A_Wq.shape
    M = A_mem0.shape[1]
    DC = B_c_kv.shape[2]
    SEG = int(A_seg_len)
    assert (S, DM, H, E, M, DC, SEG) == (2048, 448, 16, 256, 8, 1024, 32)
    HE = H * E
    any_spec = pl.BlockSpec(memory_space=pl.ANY)
    vm = pltpu.VMEM
    scratch = [
        vm((DM, S), BF), vm((S, DM), BF), vm((S, DC), BF),
        vm((2, DM * H, 128), BF), vm((2, DC * H, 128), BF), vm((2, DC * H, 128), BF),
        vm((H * DM, E), BF),
        vm((2, DM // 2, HE // 2), U32), vm((H, DC // 2, 2 * E), U32),
        vm((H, S // 2, E), U32), vm((2, S // 2, 2 * E), U32),
        vm((512, S), F32),
        vm((256, S), F32), vm((256, S), F32), vm((256, S), BF), vm((256, S), BF),
        vm((DM, S), BF), vm((S, DM), BF),
        vm((3, 2, DM * H, 128), BF), vm((H * DM, E), BF),
        vm((DM // 2, 3 * HE), U32), vm((HE, DM), BF),
        vm((M, DM), F32),
        vm((4, SEG, HE), BF), vm((4, 48, HE), BF), vm((4, 48, HE), BF),
        vm((2, 80, HE), BF),
        vm((S, 2 * DM), BF),
        pltpu.SemaphoreType.DMA((29,)), pltpu.SemaphoreType.DMA((8,)),
    ]
    out = pl.pallas_call(
        functools.partial(_kernel, S=S, DM=DM, H=H, E=E, DC=DC, M=M, SEG=SEG),
        out_shape=jax.ShapeDtypeStruct((S, 2 * DM), BF),
        in_specs=[any_spec, pl.BlockSpec(memory_space=pltpu.VMEM)] + [any_spec] * 10,
        out_specs=any_spec,
        scratch_shapes=scratch,
        compiler_params=pltpu.CompilerParams(vmem_limit_bytes=126 * 1024 * 1024),
    )(
        jnp.swapaxes(A_x, 1, 2).reshape(DM, S), A_mem0.reshape(M, DM),
        A_Wq.reshape(DM * H, E), A_Wk.reshape(DM * H, E), A_Wv.reshape(DM * H, E),
        jnp.swapaxes(A_Wo, 1, 2).reshape(H * DM, E),
        jnp.swapaxes(B_x, 1, 2).reshape(DM, S), B_c_kv.reshape(S, DC),
        B_w_q.reshape(DM * H, E), B_w_uk.reshape(DC * H, E), B_w_uv.reshape(DC * H, E),
        jnp.swapaxes(B_w_o, 1, 2).reshape(H * DM, E),
    )
    return out.reshape(1, S, 2 * DM)
```

```python
import functools
import os

import jax
import jax.numpy as jnp
from jax import lax
from jax.experimental import pallas as pl
from jax.experimental.pallas import tpu as pltpu

BF = jnp.bfloat16
F32 = jnp.float32
U32 = jnp.uint32
NT = (((1,), (1,)), ((), ()))
NEG = -1000000000.0


def _bf(x32):
    return pltpu.bitcast(x32, BF)


def _u32(xb):
    return pltpu.bitcast(xb, U32)


def _dot(a, b):
    return jnp.dot(a, b, preferred_element_type=F32)


def _dot_nt(a, b):
    return lax.dot_general(a, b, NT, preferred_element_type=F32)


def _deint(raw32, j, r0, gate=None):
    ev = raw32[pl.ds(r0 * 8 + j, 8, stride=16), :]
    od = raw32[pl.ds(r0 * 8 + j + 8, 8, stride=16), :]
    if gate is not None:
        ev = ev | gate
    lo = (ev & jnp.uint32(0xFFFF)) | (od << 16)
    hi = (ev >> 16) | (od & jnp.uint32(0xFFFF0000))
    return lo, hi


def _deint_block(raw32, nrows, store, chain):
    done = []
    for r0 in range(0, nrows, 16):
        for j in range(8):
            gate = _zero_after(done[-chain]) if 0 < chain <= len(done) else None
            lo, hi = _deint(raw32, j, r0, gate)
            store(2 * j, r0 // 2, lo)
            store(2 * j + 1, r0 // 2, hi)
            done.append(hi)


def _zero_after(x):
    return (pltpu.bitcast(x, U32) >> 16) >> 16


def _softmax_rows(sc, mask):
    sc = jnp.where(mask, sc, NEG)
    m = jnp.max(sc, axis=1, keepdims=True)
    p = jnp.exp(sc - m)
    l = jnp.sum(p, axis=1, keepdims=True)
    return p * (1.0 / l)


def _kernel(xa_hbm, mem0_ref, awq_hbm, awk_hbm, awv_hbm, awo_hbm,
            xb_hbm, c_hbm, bwq_hbm, bwuk_hbm, bwuv_hbm, bwo_hbm,
            out_hbm,
            xbt, xb, c, bwq_raw, bwuk_raw, bwuv_raw, bwot, bwq_d, wkv_d, q_all, kv, acct, s_buf0, s_buf1, p_buf0, p_buf1,
            xat, xa, a_raw, awot, aw_d, awo_d, mem, zq, zk, zv, oxe, oxo, obuf,
            sems, osems,
            *, S, DM, H, E, DC, M, SEG):
    HE = H * E
    NSEG = S // SEG
    scale = E ** -0.5
    s_buf = (s_buf0, s_buf1)
    p_buf = (p_buf0, p_buf1)

    nsem = [0]

    def copy(src, dst):
        nsem[0] += 1
        return pltpu.make_async_copy(src, dst, sems.at[nsem[0] - 1])

    def slab(src, dst, part):
        nr = src.shape[0] // 2
        rows = pl.ds(part * nr, nr)
        return [copy(src.at[rows, pl.ds(i * 128, 128)], dst.at[i, rows]) for i in range(2)]

    def rows_half(src, dst, part):
        nr = src.shape[0] // 2
        return copy(src.at[pl.ds(part * nr, nr)], dst.at[pl.ds(part * nr, nr)])

    cp_bwq = [copy(bwq_hbm.at[:, pl.ds(i * 128, 128)], bwq_raw.at[i]) for i in range(2)]
    cp_xb = copy(xb_hbm, xbt)
    cp_c = copy(c_hbm, c)
    cp_xa = copy(xa_hbm, xat)
    cp_wkv = [slab(bwuk_hbm, bwuk_raw, p) + slab(bwuv_hbm, bwuv_raw, p) for p in range(2)]
    cp_late = [[rows_half(bwo_hbm, bwot, p), rows_half(awo_hbm, awot, p)]
               + slab(awq_hbm, a_raw.at[0], p) + slab(awk_hbm, a_raw.at[1], p) + slab(awv_hbm, a_raw.at[2], p)
               for p in range(2)]

    def start(cps):
        for cp in cps:
            cp.start()

    def wait(cps):
        for cp in cps:
            cp.wait()

    TQP = 512
    PADL = 512 - DM
    ZR = 512 // 16
    scale2 = scale * 1.4426950408889634

    def xb_t(i):
        cc = pl.ds(pl.multiple_of(i * 256, 256), 256)
        xb[cc, :] = xbt[:, cc].T

    def deint_bwq(half):
        def body(t, carry):
            r32 = bwq_raw.at[half].bitcast(U32).at[pl.ds(pl.multiple_of(t * 512, 512), 512)]
            dst = bwq_d.at[half, pl.ds(pl.multiple_of(t * 32, 32), 32)]

            def store(hd, r, v):
                dst[r:r + 8, hd * 128:(hd + 1) * 128] = v

            _deint_block(r32, 64, store, 0)
            return carry

        lax.fori_loop(0, DM // 64, body, 0)

    def q_step(half, t):
        i = lax.shift_right_logical(t, 1)
        n = lax.bitwise_and(t, 1)
        r0 = pl.multiple_of(i * TQP, TQP)
        c0 = pl.multiple_of(n * 1024, 1024)
        z = _dot(xb[pl.ds(r0, TQP), :], _bf(bwq_d[half, :, pl.ds(c0, 1024)])) * scale2
        z = _u32(z.astype(BF))
        rr = pl.ds(pl.multiple_of(i * (TQP // 2), TQP // 2), TQP // 2)
        for hh in range(8):
            q_all[n * 8 + hh, rr, half * 128:(half + 1) * 128] = z[:, hh * 128:(hh + 1) * 128]
        acct[pl.ds(pl.multiple_of((half * 8 + t) * ZR, ZR), ZR), :] = jnp.zeros((ZR, S), F32)

    start([cp_xb, cp_bwq[0]])
    cp_xb.wait()

    def xb_t0(i, carry):
        xb_t(i)
        return carry

    lax.fori_loop(0, 2, xb_t0, 0)
    cp_bwq[0].wait()
    start([cp_bwq[1]] + cp_wkv[0])
    deint_bwq(0)

    DCH = int(os.environ.get('DCH', 1))

    def deint_kv(t):
        for w_i, raw in enumerate((bwuk_raw, bwuv_raw)):
            for half in range(2):
                r32 = raw.at[half].bitcast(U32).at[pl.ds(pl.multiple_of(t * 1024, 1024), 1024)]
                dst = wkv_d.at[:, pl.ds(pl.multiple_of(t * 64, 64), 64)]

                def store(hd, r, v, c0=w_i * E + half * 128, dst=dst):
                    dst[hd, r:r + 8, c0:c0 + 128] = v

                _deint_block(r32, 128, store, DCH)

    W3 = int(os.environ.get('W3', 4))
    W4 = int(os.environ.get('W4', 2))

    def q_lo(t, carry):
        @pl.when(t == W3)
        def _():
            start(cp_wkv[1] + [cp_c])

        q_step(0, t)
        xb_t(jnp.minimum(t + 2, S // 256 - 1))
        return carry

    def q_hi(t, carry):
        @pl.when(t == W4)
        def _():
            start([cp_xa] + cp_late[0])

        @pl.when(t == 4)
        def _():
            wait(cp_wkv[1])

        q_step(1, t)
        deint_kv(t)
        return carry

    lax.fori_loop(0, 8, q_lo, 0)
    cp_bwq[1].wait()
    deint_bwq(1)
    wait(cp_wkv[0])
    lax.fori_loop(0, 8, q_hi, 0)
    cp_c.wait()

    TQ = 256
    NQ = S // TQ
    HQ = TQ // 2

    def kv_chunk(h, slot, r0, nr):
        z = _dot(c[pl.ds(r0, nr), :], _bf(wkv_d[h]))
        kv[slot, pl.ds(r0 // 2, nr // 2), :] = _u32(z.astype(BF))

    KD = int(os.environ.get('KD', 256))
    kv_chunk(0, 0, 0, KD)
    wait([cp_xa] + cp_late[0])
    start(cp_late[1])

    RG = int(os.environ.get('RG', 8))
    CHL = [int(v) for v in os.environ.get('CH', '43222223')]

    def attention(h, slot, filler, CHS):
        wot_h = bwot[pl.ds(pl.multiple_of(h * DM, DM), DM), :]
        row = lax.broadcasted_iota(jnp.int32, (TQ, HQ), 0)
        col = lax.broadcasted_iota(jnp.int32, (TQ, HQ), 1)
        tri_main = row >= col
        tri_tail = tri_main[0:HQ]
        blocks = list(range(NQ))

        def scores(idx):
            i, b = blocks[idx], idx % 2
            n = (i + 1) * TQ
            nm = n - HQ
            nf = n - TQ
            q = _bf(q_all[h, pl.ds(i * TQ // 2, TQ // 2), :])
            if nf > 0:
                s_buf[b][:, 0:nf] = _dot_nt(q, _bf(kv[slot, pl.ds(0, nf // 2), 0:E]))
            s_mid = _dot_nt(q, _bf(kv[slot, pl.ds(nf // 2, HQ // 2), 0:E]))
            s_buf[b][:, nf:nm] = jnp.where(tri_main, s_mid, NEG)
            s_tail = _dot_nt(q[HQ:TQ], _bf(kv[slot, pl.ds(nm // 2, HQ // 2), 0:E]))
            s_buf[b][HQ:TQ, nm:n] = jnp.where(tri_tail, s_tail, NEG)

        def softmax(idx):
            i, b, CH = blocks[idx], idx % 2, CHS[idx]
            n = (i + 1) * TQ
            nm = n - HQ
            ls = []
            sms = []
            for g in range(TQ // RG):
                ne = nm if g * RG < HQ else n
                rows = slice(g * RG, (g + 1) * RG)
                mx = s_buf[b][rows, 0:128]
                if g >= CH:
                    mx = mx + sms[g - CH] * 0.0
                for t in range(1, ne // 128):
                    mx = jnp.maximum(mx, s_buf[b][rows, t * 128:(t + 1) * 128])
                m = jnp.broadcast_to(jnp.max(mx, axis=1, keepdims=True), (RG, 128))
                sm = None
                for t0 in range(0, ne, 256):
                    pgs = []
                    for t in range(t0, min(t0 + 256, ne), 128):
                        pg = jnp.exp2(s_buf[b][rows, t:t + 128] - m)
                        sm = pg if sm is None else sm + pg
                        pgs.append(pg)
                    p_buf[b][rows, t0:t0 + 128 * len(pgs)] = jnp.concatenate(pgs, axis=1).astype(BF)
                sms.append(sm)
                ls.append(jnp.sum(sm, axis=1, keepdims=True))
            return jnp.concatenate(ls, axis=0)

        def context(idx, l):
            i, b = blocks[idx], idx % 2
            n = (i + 1) * TQ
            nm = n - HQ
            ctx = _dot(p_buf[b][:, 0:nm], _bf(kv[slot, pl.ds(0, nm // 2), E:2 * E]))
            ctx_t = _dot(p_buf[b][HQ:TQ, nm:n], _bf(kv[slot, pl.ds(nm // 2, HQ // 2), E:2 * E]))
            ctx = jnp.concatenate([ctx[0:HQ], ctx[HQ:TQ] + ctx_t], axis=0)
            return (ctx * (1.0 / l)).astype(BF)

        def out_proj(idx, ctx):
            acct[PADL:PADL + DM, pl.ds(blocks[idx] * TQ, TQ)] += _dot_nt(wot_h, ctx)

        scores(0)
        ctx = None
        for idx in range(NQ):
            l = softmax(idx)
            filler(idx)
            if idx + 1 < NQ:
                scores(idx + 1)
            if ctx is not None:
                out_proj(idx - 1, ctx)
            ctx = context(idx, l)
        out_proj(NQ - 1, ctx)

    def deint_a(t):
        dst = aw_d.at[pl.ds(pl.multiple_of(t * 16, 16), 16)]
        for w_i in range(3):
            for half in range(2):
                r32 = a_raw.at[w_i, half].bitcast(U32).at[pl.ds(pl.multiple_of(t * 256, 256), 256)]

                def store(hd, r, v, c0=w_i * HE + half * 128):
                    dst[r:r + 8, c0 + hd * E:c0 + hd * E + 128] = v

                _deint_block(r32, 32, store, DCH)

    def prep_a(t):
        awo_d[pl.ds(pl.multiple_of(t * (E // 2), E // 2), E // 2), :] = _u32(
            awot[pl.ds(pl.multiple_of(t * DM, DM), DM), :].T)
        cc = pl.ds(pl.multiple_of(t * 128, 128), 128)
        xa[cc, :] = xat[:, cc].T

    def head(h, carry):
        slot = lax.bitwise_and(h, 1)
        hn = jnp.minimum(h + 1, H - 1)

        @pl.when(h == DM // 64)
        def _():
            wait(cp_late[1])

        def filler(idx):
            if KD == 256:
                if idx < NQ - 1:
                    kv_chunk(h, slot, (idx + 1) * TQ, TQ)
                else:
                    kv_chunk(hn, 1 - slot, 0, TQ)
            else:
                if 1 <= idx < NQ - 1:
                    kv_chunk(h, slot, (idx + 1) * TQ, TQ)
                elif idx == NQ - 1:
                    kv_chunk(hn, 1 - slot, 0, 2 * TQ)
            if idx == 2:
                deint_a(jnp.minimum(h, DM // 32 - 1))
            if idx == 3:
                prep_a(h)

        attention(h, slot, filler, CHL)
        return carry

    lax.fori_loop(0, H, head, 0)

    L = 48
    LV = M + SEG
    PR = 2 * SEG
    XE = 40
    XO = PR - XE
    NP = NSEG // 2
    OC = 4
    NOC = NP // OC
    ORS = OC * PR

    zpad = jnp.zeros((2, L - LV, HE), BF)
    zk[:, LV:L, :] = zpad
    zv[:, LV:L, :] = zpad
    oxe[...] = jnp.zeros(oxe.shape, BF)
    mem[...] = mem0_ref[...].astype(F32)

    def out_copy(k):
        r = pl.ds(pl.multiple_of(k * ORS, ORS), ORS)
        return pltpu.make_async_copy(obuf.at[r, :], out_hbm.at[r, :], osems.at[k])

    def b_out(j):
        r = pl.ds(pl.multiple_of(j * 128, 128), 128)
        obuf[r, DM:2 * DM] = acct[:, r].astype(BF).T[:, PADL:]

    def substep(odd, r0, ro, mask_m, mask_x, filler):
        cur = int(odd)
        nx = XO if odd else XE
        x0 = XE if odd else 0
        R = nx + M
        oxo_lhs = oxo if odd else oxe

        def scatter(dst, z):
            if odd:
                dst[1, XE - SEG:SEG, :] = z[0:XO].astype(BF)
            else:
                dst[0, 0:SEG, :] = z[0:SEG].astype(BF)
                dst[1, 0:XE - SEG, :] = z[SEG:XE].astype(BF)

        lhs = jnp.concatenate([xa[pl.ds(r0 + x0, nx), :].astype(F32), mem[...]], axis=0).astype(BF)
        zqk = _dot(lhs, _bf(aw_d[:, 0:2 * HE]))
        zqs = zqk[:, 0:HE] * scale
        scatter(zq, zqs)
        qm = zqs[nx:R].astype(BF)
        scatter(zk, zqk[:, HE:2 * HE])
        zk[cur, SEG:LV, :] = zqk[nx:R, HE:2 * HE].astype(BF)
        sm = jnp.concatenate(
            [_dot_nt(qm[:, h * E:(h + 1) * E], zk[cur, :, h * E:(h + 1) * E]) for h in range(H)], axis=0)
        zvv = _dot(lhs, _bf(aw_d[:, 2 * HE:3 * HE]))
        scatter(zv, zvv)
        zv[cur, SEG:LV, :] = zvv[nx:R].astype(BF)
        pm = _softmax_rows(sm, mask_m)
        for h in range(H):
            oxo_lhs[nx:R, h * E:(h + 1) * E] = _dot(
                pm[h * M:(h + 1) * M].astype(BF), zv[cur, :, h * E:(h + 1) * E]).astype(BF)
        sx = jnp.concatenate(
            [_dot_nt(zq[cur, :, h * E:(h + 1) * E], zk[cur, :, h * E:(h + 1) * E]) for h in range(H)], axis=0)
        filler()
        o = _dot(oxo_lhs[...], _bf(awo_d[...]))
        obuf[pl.ds(ro, nx), 0:DM] = o[0:nx].astype(BF)
        mem[...] = o[nx:R]
        px = _softmax_rows(sx, mask_x).astype(BF)
        for h in range(H):
            oh = _dot(px[h * SEG:(h + 1) * SEG], zv[cur, :, h * E:(h + 1) * E])
            cols = slice(h * E, (h + 1) * E)
            if odd:
                oxe[XE - SEG:XE, cols] = oh.astype(BF)
            else:
                oxo[0:XO, cols] = oh[0:XO].astype(BF)
                oxe[0:XE - SEG, cols] = oh[XO:SEG].astype(BF)

    def pair(t, carry):
        colm = lax.broadcasted_iota(jnp.int32, (H * M, L), 1)
        mask_m = colm < LV
        rowx = lax.bitwise_and(lax.broadcasted_iota(jnp.int32, (H * SEG, L), 0), SEG - 1)
        colx = lax.broadcasted_iota(jnp.int32, (H * SEG, L), 1)
        mask_x = (colx < LV) & ((rowx >= colx) | (colx >= SEG))
        r0 = pl.multiple_of(t * PR, PR)
        re = pl.multiple_of(jnp.maximum(r0 - XE, XO), 8)
        substep(False, r0, re, mask_m, mask_x, lambda: b_out(lax.shift_right_logical(t, 1)))
        substep(True, r0, r0, mask_m, mask_x, lambda: None)

        @pl.when(jnp.logical_and(lax.bitwise_and(t, OC - 1) == 0, t > 0))
        def _():
            out_copy(lax.shift_right_logical(t, 2) - 1).start()

        return carry

    lax.fori_loop(0, NP, pair, 0)
    obuf[S - XE:S, 0:DM] = _dot(oxe[...], _bf(awo_d[...]))[0:XE].astype(BF)
    out_copy(NOC - 1).start()
    for k in range(NOC):
        out_copy(k).wait()


@functools.partial(jax.jit, static_argnames=("A_seg_len",))
def pallas_concat_heads__memory_aug_recurrent_mem_tr__compressed_kv_cla__prompt_kernel(
    A_x, A_mem0, A_Wq, A_Wk, A_Wv, A_Wo, A_seg_len,
    B_x, B_c_kv, B_w_q, B_w_uk, B_w_uv, B_w_o,
):
    _, S, DM = A_x.shape
    _, H, E = A_Wq.shape
    M = A_mem0.shape[1]
    DC = B_c_kv.shape[2]
    SEG = int(A_seg_len)
    assert (S, DM, H, E, M, DC, SEG) == (2048, 448, 16, 256, 8, 1024, 32)
    HE = H * E
    any_spec = pl.BlockSpec(memory_space=pl.ANY)
    vm = pltpu.VMEM
    scratch = [
        vm((DM, S), BF), vm((S, DM), BF), vm((S, DC), BF),
        vm((2, DM * H, 128), BF), vm((2, DC * H, 128), BF), vm((2, DC * H, 128), BF),
        vm((H * DM, E), BF),
        vm((2, DM // 2, HE // 2), U32), vm((H, DC // 2, 2 * E), U32),
        vm((H, S // 2, E), U32), vm((2, S // 2, 2 * E), U32),
        vm((512, S), F32),
        vm((256, S), F32), vm((256, S), F32), vm((256, S), BF), vm((256, S), BF),
        vm((DM, S), BF), vm((S, DM), BF),
        vm((3, 2, DM * H, 128), BF), vm((H * DM, E), BF),
        vm((DM // 2, 3 * HE), U32), vm((HE // 2, DM), U32),
        vm((M, DM), F32),
        vm((2, SEG, HE), BF), vm((2, 48, HE), BF), vm((2, 48, HE), BF),
        vm((48, HE), BF), vm((32, HE), BF),
        vm((S, 2 * DM), BF),
        pltpu.SemaphoreType.DMA((29,)), pltpu.SemaphoreType.DMA((8,)),
    ]
    out = pl.pallas_call(
        functools.partial(_kernel, S=S, DM=DM, H=H, E=E, DC=DC, M=M, SEG=SEG),
        out_shape=jax.ShapeDtypeStruct((S, 2 * DM), BF),
        in_specs=[any_spec, pl.BlockSpec(memory_space=pltpu.VMEM)] + [any_spec] * 10,
        out_specs=any_spec,
        scratch_shapes=scratch,
        compiler_params=pltpu.CompilerParams(vmem_limit_bytes=126 * 1024 * 1024),
    )(
        jnp.swapaxes(A_x, 1, 2).reshape(DM, S), A_mem0.reshape(M, DM),
        A_Wq.reshape(DM * H, E), A_Wk.reshape(DM * H, E), A_Wv.reshape(DM * H, E),
        jnp.swapaxes(A_Wo, 1, 2).reshape(H * DM, E),
        jnp.swapaxes(B_x, 1, 2).reshape(DM, S), B_c_kv.reshape(S, DC),
        B_w_q.reshape(DM * H, E), B_w_uk.reshape(DC * H, E), B_w_uv.reshape(DC * H, E),
        jnp.swapaxes(B_w_o, 1, 2).reshape(H * DM, E),
    )
    return out.reshape(1, S, 2 * DM)
```

```python
import functools
import os

import jax
import jax.numpy as jnp
from jax import lax
from jax.experimental import pallas as pl
from jax.experimental.pallas import tpu as pltpu

BF = jnp.bfloat16
F32 = jnp.float32
U32 = jnp.uint32
NT = (((1,), (1,)), ((), ()))
NEG = -1000000000.0


def _bf(x32):
    return pltpu.bitcast(x32, BF)


def _u32(xb):
    return pltpu.bitcast(xb, U32)


def _dot(a, b):
    return jnp.dot(a, b, preferred_element_type=F32)


def _dot_nt(a, b):
    return lax.dot_general(a, b, NT, preferred_element_type=F32)


def _deint(raw32, j, r0, gate=None):
    ev = raw32[pl.ds(r0 * 8 + j, 8, stride=16), :]
    od = raw32[pl.ds(r0 * 8 + j + 8, 8, stride=16), :]
    if gate is not None:
        ev = ev | gate
    lo = (ev & jnp.uint32(0xFFFF)) | (od << 16)
    hi = (ev >> 16) | (od & jnp.uint32(0xFFFF0000))
    return lo, hi


def _deint_block(raw32, nrows, store, chain):
    done = []
    for r0 in range(0, nrows, 16):
        for j in range(8):
            gate = _zero_after(done[-chain]) if 0 < chain <= len(done) else None
            lo, hi = _deint(raw32, j, r0, gate)
            store(2 * j, r0 // 2, lo)
            store(2 * j + 1, r0 // 2, hi)
            done.append(hi)


def _zero_after(x):
    return (pltpu.bitcast(x, U32) >> 16) >> 16


def _softmax_rows(sc, mask):
    sc = jnp.where(mask, sc, NEG)
    m = jnp.max(sc, axis=1, keepdims=True)
    p = jnp.exp(sc - m)
    l = jnp.sum(p, axis=1, keepdims=True)
    return p * (1.0 / l)


def _kernel(xa_hbm, mem0_ref, awq_hbm, awk_hbm, awv_hbm, awo_hbm,
            xb_hbm, c_hbm, bwq_hbm, bwuk_hbm, bwuv_hbm, bwo_hbm,
            out_hbm,
            xbt, xb, c, bwq_raw, bwuk_raw, bwuv_raw, bwot, bwq_d, wkv_d, q_all, kv, acct, s_buf0, s_buf1, p_buf0, p_buf1,
            xat, xa, a_raw, awot, aw_d, awo_d, mem, zq, zk, zv, oxe, oxo, obuf,
            sems, osems,
            *, S, DM, H, E, DC, M, SEG):
    HE = H * E
    NSEG = S // SEG
    scale = E ** -0.5
    s_buf = (s_buf0, s_buf1)
    p_buf = (p_buf0, p_buf1)

    nsem = [0]

    def copy(src, dst):
        nsem[0] += 1
        return pltpu.make_async_copy(src, dst, sems.at[nsem[0] - 1])

    def slab(src, dst, part):
        nr = src.shape[0] // 2
        rows = pl.ds(part * nr, nr)
        return [copy(src.at[rows, pl.ds(i * 128, 128)], dst.at[i, rows]) for i in range(2)]

    def rows_half(src, dst, part):
        nr = src.shape[0] // 2
        return copy(src.at[pl.ds(part * nr, nr)], dst.at[pl.ds(part * nr, nr)])

    cp_bwq = [copy(bwq_hbm.at[:, pl.ds(i * 128, 128)], bwq_raw.at[i]) for i in range(2)]
    cp_xb = copy(xb_hbm, xbt)
    cp_c = copy(c_hbm, c)
    cp_xa = copy(xa_hbm, xat)
    cp_wkv = [slab(bwuk_hbm, bwuk_raw, p) + slab(bwuv_hbm, bwuv_raw, p) for p in range(2)]
    cp_late = [[rows_half(bwo_hbm, bwot, p), rows_half(awo_hbm, awot, p)]
               + slab(awq_hbm, a_raw.at[0], p) + slab(awk_hbm, a_raw.at[1], p) + slab(awv_hbm, a_raw.at[2], p)
               for p in range(2)]

    def start(cps):
        for cp in cps:
            cp.start()

    def wait(cps):
        for cp in cps:
            cp.wait()

    TQP = 512
    PADL = 512 - DM
    ZR = 512 // 16
    scale2 = scale * 1.4426950408889634

    def xb_t(i):
        cc = pl.ds(pl.multiple_of(i * 256, 256), 256)
        xb[cc, :] = xbt[:, cc].T

    def deint_bwq(half):
        def body(t, carry):
            r32 = bwq_raw.at[half].bitcast(U32).at[pl.ds(pl.multiple_of(t * 512, 512), 512)]
            dst = bwq_d.at[half, pl.ds(pl.multiple_of(t * 32, 32), 32)]

            def store(hd, r, v):
                dst[r:r + 8, hd * 128:(hd + 1) * 128] = v

            _deint_block(r32, 64, store, 0)
            return carry

        lax.fori_loop(0, DM // 64, body, 0)

    def q_step(half, t):
        i = lax.shift_right_logical(t, 1)
        n = lax.bitwise_and(t, 1)
        r0 = pl.multiple_of(i * TQP, TQP)
        c0 = pl.multiple_of(n * 1024, 1024)
        z = _dot(xb[pl.ds(r0, TQP), :], _bf(bwq_d[half, :, pl.ds(c0, 1024)])) * scale2
        z = _u32(z.astype(BF))
        rr = pl.ds(pl.multiple_of(i * (TQP // 2), TQP // 2), TQP // 2)
        for hh in range(8):
            q_all[n * 8 + hh, rr, half * 128:(half + 1) * 128] = z[:, hh * 128:(hh + 1) * 128]
        acct[pl.ds(pl.multiple_of((half * 8 + t) * ZR, ZR), ZR), :] = jnp.zeros((ZR, S), F32)

    start([cp_xb, cp_bwq[0]])
    cp_xb.wait()

    def xb_t0(i, carry):
        xb_t(i)
        return carry

    lax.fori_loop(0, 2, xb_t0, 0)
    cp_bwq[0].wait()
    start([cp_bwq[1]] + cp_wkv[0])
    deint_bwq(0)

    DCH = int(os.environ.get('DCH', 1))

    def deint_kv(t):
        for w_i, raw in enumerate((bwuk_raw, bwuv_raw)):
            for half in range(2):
                r32 = raw.at[half].bitcast(U32).at[pl.ds(pl.multiple_of(t * 1024, 1024), 1024)]
                dst = wkv_d.at[:, pl.ds(pl.multiple_of(t * 64, 64), 64)]

                def store(hd, r, v, c0=w_i * E + half * 128, dst=dst):
                    dst[hd, r:r + 8, c0:c0 + 128] = v

                _deint_block(r32, 128, store, DCH)

    W3 = int(os.environ.get('W3', 4))
    W4 = int(os.environ.get('W4', 2))

    def q_lo(t, carry):
        @pl.when(t == W3)
        def _():
            start(cp_wkv[1] + [cp_c])

        q_step(0, t)
        xb_t(jnp.minimum(t + 2, S // 256 - 1))
        return carry

    def q_hi(t, carry):
        @pl.when(t == W4)
        def _():
            start([cp_xa] + cp_late[0])

        @pl.when(t == 4)
        def _():
            wait(cp_wkv[1])

        q_step(1, t)
        deint_kv(t)
        return carry

    lax.fori_loop(0, 8, q_lo, 0)
    cp_bwq[1].wait()
    deint_bwq(1)
    wait(cp_wkv[0])
    lax.fori_loop(0, 8, q_hi, 0)
    cp_c.wait()

    TQ = 256
    NQ = S // TQ
    HQ = TQ // 2

    def kv_chunk(h, slot, r0, nr):
        z = _dot(c[pl.ds(r0, nr), :], _bf(wkv_d[h]))
        kv[slot, pl.ds(r0 // 2, nr // 2), :] = _u32(z.astype(BF))

    KD = int(os.environ.get('KD', 256))
    kv_chunk(0, 0, 0, KD)
    wait([cp_xa] + cp_late[0])
    start(cp_late[1])

    RG = int(os.environ.get('RG', 8))
    CHL = [int(v) for v in os.environ.get('CH', '43222223')]

    def attention(h, slot, filler, CHS):
        wot_h = bwot[pl.ds(pl.multiple_of(h * DM, DM), DM), :]
        row = lax.broadcasted_iota(jnp.int32, (TQ, HQ), 0)
        col = lax.broadcasted_iota(jnp.int32, (TQ, HQ), 1)
        tri_main = row >= col
        tri_tail = tri_main[0:HQ]
        blocks = list(range(NQ))

        def scores(idx):
            i, b = blocks[idx], idx % 2
            n = (i + 1) * TQ
            nm = n - HQ
            nf = n - TQ
            q = _bf(q_all[h, pl.ds(i * TQ // 2, TQ // 2), :])
            if nf > 0:
                s_buf[b][:, 0:nf] = _dot_nt(q, _bf(kv[slot, pl.ds(0, nf // 2), 0:E]))
            s_mid = _dot_nt(q, _bf(kv[slot, pl.ds(nf // 2, HQ // 2), 0:E]))
            s_buf[b][:, nf:nm] = jnp.where(tri_main, s_mid, NEG)
            s_tail = _dot_nt(q[HQ:TQ], _bf(kv[slot, pl.ds(nm // 2, HQ // 2), 0:E]))
            s_buf[b][HQ:TQ, nm:n] = jnp.where(tri_tail, s_tail, NEG)

        def softmax(idx):
            i, b, CH = blocks[idx], idx % 2, CHS[idx]
            n = (i + 1) * TQ
            nm = n - HQ
            ls = []
            sms = []
            for g in range(TQ // RG):
                ne = nm if g * RG < HQ else n
                rows = slice(g * RG, (g + 1) * RG)
                mx = s_buf[b][rows, 0:128]
                if g >= CH:
                    mx = mx + sms[g - CH] * 0.0
                for t in range(1, ne // 128):
                    mx = jnp.maximum(mx, s_buf[b][rows, t * 128:(t + 1) * 128])
                m = jnp.broadcast_to(jnp.max(mx, axis=1, keepdims=True), (RG, 128))
                sm = None
                for t0 in range(0, ne, 256):
                    pgs = []
                    for t in range(t0, min(t0 + 256, ne), 128):
                        pg = jnp.exp2(s_buf[b][rows, t:t + 128] - m)
                        sm = pg if sm is None else sm + pg
                        pgs.append(pg)
                    p_buf[b][rows, t0:t0 + 128 * len(pgs)] = jnp.concatenate(pgs, axis=1).astype(BF)
                sms.append(sm)
                ls.append(jnp.sum(sm, axis=1, keepdims=True))
            return jnp.concatenate(ls, axis=0)

        def context(idx, l):
            i, b = blocks[idx], idx % 2
            n = (i + 1) * TQ
            nm = n - HQ
            ctx = _dot(p_buf[b][:, 0:nm], _bf(kv[slot, pl.ds(0, nm // 2), E:2 * E]))
            ctx_t = _dot(p_buf[b][HQ:TQ, nm:n], _bf(kv[slot, pl.ds(nm // 2, HQ // 2), E:2 * E]))
            ctx = jnp.concatenate([ctx[0:HQ], ctx[HQ:TQ] + ctx_t], axis=0)
            return (ctx * (1.0 / l)).astype(BF)

        def out_proj(idx, ctx):
            acct[PADL:PADL + DM, pl.ds(blocks[idx] * TQ, TQ)] += _dot_nt(wot_h, ctx)

        scores(0)
        ctx = None
        for idx in range(NQ):
            l = softmax(idx)
            filler(idx)
            if idx + 1 < NQ:
                scores(idx + 1)
            if ctx is not None:
                out_proj(idx - 1, ctx)
            ctx = context(idx, l)
        out_proj(NQ - 1, ctx)

    def deint_a(t):
        dst = aw_d.at[pl.ds(pl.multiple_of(t * 16, 16), 16)]
        for w_i in range(3):
            for half in range(2):
                r32 = a_raw.at[w_i, half].bitcast(U32).at[pl.ds(pl.multiple_of(t * 256, 256), 256)]

                def store(hd, r, v, c0=w_i * HE + half * 128):
                    dst[r:r + 8, c0 + hd * E:c0 + hd * E + 128] = v

                _deint_block(r32, 32, store, DCH)

    def prep_a(t):
        awo_d[pl.ds(pl.multiple_of(t * (E // 2), E // 2), E // 2), :] = _u32(
            awot[pl.ds(pl.multiple_of(t * DM, DM), DM), :].T)
        cc = pl.ds(pl.multiple_of(t * 128, 128), 128)
        xa[cc, :] = xat[:, cc].T

    def head(h, carry):
        slot = lax.bitwise_and(h, 1)
        hn = jnp.minimum(h + 1, H - 1)

        @pl.when(h == DM // 64)
        def _():
            wait(cp_late[1])

        def filler(idx):
            if KD == 256:
                if idx < NQ - 1:
                    kv_chunk(h, slot, (idx + 1) * TQ, TQ)
                else:
                    kv_chunk(hn, 1 - slot, 0, TQ)
            else:
                if 1 <= idx < NQ - 1:
                    kv_chunk(h, slot, (idx + 1) * TQ, TQ)
                elif idx == NQ - 1:
                    kv_chunk(hn, 1 - slot, 0, 2 * TQ)
            if idx == 2:
                deint_a(jnp.minimum(h, DM // 32 - 1))
            if idx == 3:
                prep_a(h)

        attention(h, slot, filler, CHL)
        return carry

    lax.fori_loop(0, H, head, 0)

    L = 48
    LV = M + SEG
    PR = 2 * SEG
    XE = 40
    XO = PR - XE
    NP = NSEG // 2
    OC = 4
    NOC = NP // OC
    ORS = OC * PR

    zpad = jnp.zeros((2, L - LV, HE), BF)
    zq[:, LV:L, :] = zpad
    zk[:, LV:L, :] = zpad
    zv[:, LV:L, :] = zpad
    oxe[...] = jnp.zeros(oxe.shape, BF)
    mem[...] = mem0_ref[...].astype(F32)

    def out_copy(k):
        r = pl.ds(pl.multiple_of(k * ORS, ORS), ORS)
        return pltpu.make_async_copy(obuf.at[r, :], out_hbm.at[r, :], osems.at[k])

    def b_out(j):
        r = pl.ds(pl.multiple_of(j * 128, 128), 128)
        obuf[r, DM:2 * DM] = acct[:, r].astype(BF).T[:, PADL:]

    def substep(odd, r0, ro, mask_m, mask_x, filler):
        cur = int(odd)
        nx = XO if odd else XE
        x0 = XE if odd else 0
        R = nx + M
        oxo_lhs = oxo if odd else oxe

        def scatter(dst, z):
            if odd:
                dst[1, XE - SEG:SEG, :] = z[0:XO].astype(BF)
            else:
                dst[0, 0:SEG, :] = z[0:SEG].astype(BF)
                dst[1, 0:XE - SEG, :] = z[SEG:XE].astype(BF)

        lhs = jnp.concatenate([xa[pl.ds(r0 + x0, nx), :].astype(F32), mem[...]], axis=0).astype(BF)
        zqk = _dot(lhs, _bf(aw_d[:, 0:2 * HE]))
        zqs = zqk[:, 0:HE] * scale
        scatter(zq, zqs)
        zq[cur, SEG:LV, :] = zqs[nx:R].astype(BF)
        scatter(zk, zqk[:, HE:2 * HE])
        zk[cur, SEG:LV, :] = zqk[nx:R, HE:2 * HE].astype(BF)
        sc = [_dot_nt(zq[cur, :, h * E:(h + 1) * E], zk[cur, :, h * E:(h + 1) * E]) for h in range(H)]
        zvv = _dot(lhs, _bf(aw_d[:, 2 * HE:3 * HE]))
        scatter(zv, zvv)
        zv[cur, SEG:LV, :] = zvv[nx:R].astype(BF)
        pm = _softmax_rows(jnp.concatenate([a[SEG:LV] for a in sc], axis=0), mask_m)
        px = _softmax_rows(jnp.concatenate([a[0:SEG] for a in sc], axis=0), mask_x).astype(BF)
        for h in range(H):
            oxo_lhs[nx:R, h * E:(h + 1) * E] = _dot(
                pm[h * M:(h + 1) * M].astype(BF), zv[cur, :, h * E:(h + 1) * E]).astype(BF)

        def x_pv(h):
            oh = _dot(px[h * SEG:(h + 1) * SEG], zv[cur, :, h * E:(h + 1) * E])
            cols = slice(h * E, (h + 1) * E)
            if odd:
                oxe[XE - SEG:XE, cols] = oh.astype(BF)
            else:
                oxo[0:XO, cols] = oh[0:XO].astype(BF)
                return oh[XO:SEG].astype(BF)

        filler()
        NE = int(os.environ.get('NE', 4))
        early = [x_pv(h) for h in range(NE)]
        o = _dot(oxo_lhs[...], _bf(awo_d[...]))
        obuf[pl.ds(ro, nx), 0:DM] = o[0:nx].astype(BF)
        mem[...] = o[nx:R]
        late = [x_pv(h) for h in range(NE, H)]
        if not odd:
            for h, v in enumerate(early + late):
                oxe[0:XE - SEG, h * E:(h + 1) * E] = v

    def pair(t, carry):
        colm = lax.broadcasted_iota(jnp.int32, (H * M, L), 1)
        mask_m = colm < LV
        rowx = lax.bitwise_and(lax.broadcasted_iota(jnp.int32, (H * SEG, L), 0), SEG - 1)
        colx = lax.broadcasted_iota(jnp.int32, (H * SEG, L), 1)
        mask_x = (colx < LV) & ((rowx >= colx) | (colx >= SEG))
        r0 = pl.multiple_of(t * PR, PR)
        re = pl.multiple_of(jnp.maximum(r0 - XE, XO), 8)
        substep(False, r0, re, mask_m, mask_x, lambda: b_out(lax.shift_right_logical(t, 1)))
        substep(True, r0, r0, mask_m, mask_x, lambda: None)

        @pl.when(jnp.logical_and(lax.bitwise_and(t, OC - 1) == 0, t > 0))
        def _():
            out_copy(lax.shift_right_logical(t, 2) - 1).start()

        return carry

    lax.fori_loop(0, NP, pair, 0)
    obuf[S - XE:S, 0:DM] = _dot(oxe[...], _bf(awo_d[...]))[0:XE].astype(BF)
    out_copy(NOC - 1).start()
    for k in range(NOC):
        out_copy(k).wait()


@functools.partial(jax.jit, static_argnames=("A_seg_len",))
def pallas_concat_heads__memory_aug_recurrent_mem_tr__compressed_kv_cla__prompt_kernel(
    A_x, A_mem0, A_Wq, A_Wk, A_Wv, A_Wo, A_seg_len,
    B_x, B_c_kv, B_w_q, B_w_uk, B_w_uv, B_w_o,
):
    _, S, DM = A_x.shape
    _, H, E = A_Wq.shape
    M = A_mem0.shape[1]
    DC = B_c_kv.shape[2]
    SEG = int(A_seg_len)
    assert (S, DM, H, E, M, DC, SEG) == (2048, 448, 16, 256, 8, 1024, 32)
    HE = H * E
    any_spec = pl.BlockSpec(memory_space=pl.ANY)
    vm = pltpu.VMEM
    scratch = [
        vm((DM, S), BF), vm((S, DM), BF), vm((S, DC), BF),
        vm((2, DM * H, 128), BF), vm((2, DC * H, 128), BF), vm((2, DC * H, 128), BF),
        vm((H * DM, E), BF),
        vm((2, DM // 2, HE // 2), U32), vm((H, DC // 2, 2 * E), U32),
        vm((H, S // 2, E), U32), vm((2, S // 2, 2 * E), U32),
        vm((512, S), F32),
        vm((256, S), F32), vm((256, S), F32), vm((256, S), BF), vm((256, S), BF),
        vm((DM, S), BF), vm((S, DM), BF),
        vm((3, 2, DM * H, 128), BF), vm((H * DM, E), BF),
        vm((DM // 2, 3 * HE), U32), vm((HE // 2, DM), U32),
        vm((M, DM), F32),
        vm((2, 48, HE), BF), vm((2, 48, HE), BF), vm((2, 48, HE), BF),
        vm((48, HE), BF), vm((32, HE), BF),
        vm((S, 2 * DM), BF),
        pltpu.SemaphoreType.DMA((29,)), pltpu.SemaphoreType.DMA((8,)),
    ]
    out = pl.pallas_call(
        functools.partial(_kernel, S=S, DM=DM, H=H, E=E, DC=DC, M=M, SEG=SEG),
        out_shape=jax.ShapeDtypeStruct((S, 2 * DM), BF),
        in_specs=[any_spec, pl.BlockSpec(memory_space=pltpu.VMEM)] + [any_spec] * 10,
        out_specs=any_spec,
        scratch_shapes=scratch,
        compiler_params=pltpu.CompilerParams(vmem_limit_bytes=126 * 1024 * 1024),
    )(
        jnp.swapaxes(A_x, 1, 2).reshape(DM, S), A_mem0.reshape(M, DM),
        A_Wq.reshape(DM * H, E), A_Wk.reshape(DM * H, E), A_Wv.reshape(DM * H, E),
        jnp.swapaxes(A_Wo, 1, 2).reshape(H * DM, E),
        jnp.swapaxes(B_x, 1, 2).reshape(DM, S), B_c_kv.reshape(S, DC),
        B_w_q.reshape(DM * H, E), B_w_uk.reshape(DC * H, E), B_w_uv.reshape(DC * H, E),
        jnp.swapaxes(B_w_o, 1, 2).reshape(H * DM, E),
    )
    return out.reshape(1, S, 2 * DM)
```

```python
import functools
import os

import jax
import jax.numpy as jnp
from jax import lax
from jax.experimental import pallas as pl
from jax.experimental.pallas import tpu as pltpu

BF = jnp.bfloat16
F32 = jnp.float32
U32 = jnp.uint32
NT = (((1,), (1,)), ((), ()))
NEG = -1000000000.0


def _bf(x32):
    return pltpu.bitcast(x32, BF)


def _u32(xb):
    return pltpu.bitcast(xb, U32)


def _dot(a, b):
    return jnp.dot(a, b, preferred_element_type=F32)


def _dot_nt(a, b):
    return lax.dot_general(a, b, NT, preferred_element_type=F32)


def _deint(raw32, j, r0, gate=None):
    ev = raw32[pl.ds(r0 * 8 + j, 8, stride=16), :]
    od = raw32[pl.ds(r0 * 8 + j + 8, 8, stride=16), :]
    if gate is not None:
        ev = ev | gate
    lo = (ev & jnp.uint32(0xFFFF)) | (od << 16)
    hi = (ev >> 16) | (od & jnp.uint32(0xFFFF0000))
    return lo, hi


def _deint_block(raw32, nrows, store, chain):
    done = []
    for r0 in range(0, nrows, 16):
        for j in range(8):
            gate = _zero_after(done[-chain]) if 0 < chain <= len(done) else None
            lo, hi = _deint(raw32, j, r0, gate)
            store(2 * j, r0 // 2, lo)
            store(2 * j + 1, r0 // 2, hi)
            done.append(hi)


def _zero_after(x):
    return (pltpu.bitcast(x, U32) >> 16) >> 16


def _softmax_rows(sc, mask):
    sc = jnp.where(mask, sc, NEG)
    m = jnp.max(sc, axis=1, keepdims=True)
    p = jnp.exp(sc - m)
    l = jnp.sum(p, axis=1, keepdims=True)
    return p * (1.0 / l)


def _kernel(xa_hbm, mem0_ref, awq_hbm, awk_hbm, awv_hbm, awo_hbm,
            xb_hbm, c_hbm, bwq_hbm, bwuk_hbm, bwuv_hbm, bwo_hbm,
            out_hbm,
            xbt, xb, c, bwq_raw, bwuk_raw, bwuv_raw, bwot, bwq_d, wkv_d, q_all, kv, acct, s_buf0, s_buf1, p_buf0, p_buf1, ctx_last,
            xat, xa, a_raw, awot, aw_d, awo_d, mem, zq, zk, zv, oxe, oxo, obuf,
            sems, osems,
            *, S, DM, H, E, DC, M, SEG):
    HE = H * E
    NSEG = S // SEG
    scale = E ** -0.5
    s_buf = (s_buf0, s_buf1)
    p_buf = (p_buf0, p_buf1)

    nsem = [0]

    def copy(src, dst):
        nsem[0] += 1
        return pltpu.make_async_copy(src, dst, sems.at[nsem[0] - 1])

    def slab(src, dst, part):
        nr = src.shape[0] // 2
        rows = pl.ds(part * nr, nr)
        return [copy(src.at[rows, pl.ds(i * 128, 128)], dst.at[i, rows]) for i in range(2)]

    def rows_half(src, dst, part):
        nr = src.shape[0] // 2
        return copy(src.at[pl.ds(part * nr, nr)], dst.at[pl.ds(part * nr, nr)])

    cp_bwq = [copy(bwq_hbm.at[:, pl.ds(i * 128, 128)], bwq_raw.at[i]) for i in range(2)]
    cp_xb = copy(xb_hbm, xbt)
    cp_c = copy(c_hbm, c)
    cp_xa = copy(xa_hbm, xat)
    cp_wkv = [slab(bwuk_hbm, bwuk_raw, p) + slab(bwuv_hbm, bwuv_raw, p) for p in range(2)]
    cp_late = [[rows_half(bwo_hbm, bwot, p), rows_half(awo_hbm, awot, p)]
               + slab(awq_hbm, a_raw.at[0], p) + slab(awk_hbm, a_raw.at[1], p) + slab(awv_hbm, a_raw.at[2], p)
               for p in range(2)]

    def start(cps):
        for cp in cps:
            cp.start()

    def wait(cps):
        for cp in cps:
            cp.wait()

    TQP = 512
    PADL = 512 - DM
    ZR = 512 // 16
    scale2 = scale * 1.4426950408889634

    def xb_t(i):
        cc = pl.ds(pl.multiple_of(i * 256, 256), 256)
        xb[cc, :] = xbt[:, cc].T

    def deint_bwq(half):
        def body(t, carry):
            r32 = bwq_raw.at[half].bitcast(U32).at[pl.ds(pl.multiple_of(t * 512, 512), 512)]
            dst = bwq_d.at[half, pl.ds(pl.multiple_of(t * 32, 32), 32)]

            def store(hd, r, v):
                dst[r:r + 8, hd * 128:(hd + 1) * 128] = v

            _deint_block(r32, 64, store, 0)
            return carry

        lax.fori_loop(0, DM // 64, body, 0)

    def q_step(half, t):
        i = lax.shift_right_logical(t, 1)
        n = lax.bitwise_and(t, 1)
        r0 = pl.multiple_of(i * TQP, TQP)
        c0 = pl.multiple_of(n * 1024, 1024)
        z = _dot(xb[pl.ds(r0, TQP), :], _bf(bwq_d[half, :, pl.ds(c0, 1024)])) * scale2
        z = _u32(z.astype(BF))
        rr = pl.ds(pl.multiple_of(i * (TQP // 2), TQP // 2), TQP // 2)
        for hh in range(8):
            q_all[n * 8 + hh, rr, half * 128:(half + 1) * 128] = z[:, hh * 128:(hh + 1) * 128]
        acct[pl.ds(pl.multiple_of((half * 8 + t) * ZR, ZR), ZR), :] = jnp.zeros((ZR, S), F32)

    start([cp_xb, cp_bwq[0]])
    cp_xb.wait()

    def xb_t0(i, carry):
        xb_t(i)
        return carry

    lax.fori_loop(0, 2, xb_t0, 0)
    cp_bwq[0].wait()
    start([cp_bwq[1]] + cp_wkv[0])
    deint_bwq(0)

    DCH = int(os.environ.get('DCH', 1))

    def deint_kv(t):
        for w_i, raw in enumerate((bwuk_raw, bwuv_raw)):
            for half in range(2):
                r32 = raw.at[half].bitcast(U32).at[pl.ds(pl.multiple_of(t * 1024, 1024), 1024)]
                dst = wkv_d.at[:, pl.ds(pl.multiple_of(t * 64, 64), 64)]

                def store(hd, r, v, c0=w_i * E + half * 128, dst=dst):
                    dst[hd, r:r + 8, c0:c0 + 128] = v

                _deint_block(r32, 128, store, DCH)

    W3 = int(os.environ.get('W3', 4))
    W4 = int(os.environ.get('W4', 2))

    def q_lo(t, carry):
        @pl.when(t == W3)
        def _():
            start(cp_wkv[1] + [cp_c])

        q_step(0, t)
        xb_t(jnp.minimum(t + 2, S // 256 - 1))
        return carry

    def q_hi(t, carry):
        @pl.when(t == W4)
        def _():
            start([cp_xa] + cp_late[0])

        @pl.when(t == 4)
        def _():
            wait(cp_wkv[1])

        q_step(1, t)
        deint_kv(t)
        return carry

    lax.fori_loop(0, 8, q_lo, 0)
    cp_bwq[1].wait()
    deint_bwq(1)
    wait(cp_wkv[0])
    lax.fori_loop(0, 8, q_hi, 0)
    cp_c.wait()

    TQ = 256
    NQ = S // TQ
    HQ = TQ // 2

    def kv_chunk(h, slot, r0, nr):
        z = _dot(c[pl.ds(r0, nr), :], _bf(wkv_d[h]))
        kv[slot, pl.ds(r0 // 2, nr // 2), :] = _u32(z.astype(BF))

    KD = int(os.environ.get('KD', 256))
    kv_chunk(0, 0, 0, KD)
    wait([cp_xa] + cp_late[0])
    start(cp_late[1])

    RG = int(os.environ.get('RG', 8))
    CHL = [int(v) for v in os.environ.get('CH', '43222223')]

    def attention(h, slot, filler, CHS):
        wot_h = bwot[pl.ds(pl.multiple_of(h * DM, DM), DM), :]
        row = lax.broadcasted_iota(jnp.int32, (TQ, HQ), 0)
        col = lax.broadcasted_iota(jnp.int32, (TQ, HQ), 1)
        tri_main = row >= col
        tri_tail = tri_main[0:HQ]
        blocks = list(range(NQ))

        def scores(idx):
            i, b = blocks[idx], idx % 2
            n = (i + 1) * TQ
            nm = n - HQ
            nf = n - TQ
            q = _bf(q_all[h, pl.ds(i * TQ // 2, TQ // 2), :])
            if nf > 0:
                s_buf[b][:, 0:nf] = _dot_nt(q, _bf(kv[slot, pl.ds(0, nf // 2), 0:E]))
            s_mid = _dot_nt(q, _bf(kv[slot, pl.ds(nf // 2, HQ // 2), 0:E]))
            s_buf[b][:, nf:nm] = jnp.where(tri_main, s_mid, NEG)
            s_tail = _dot_nt(q[HQ:TQ], _bf(kv[slot, pl.ds(nm // 2, HQ // 2), 0:E]))
            s_buf[b][HQ:TQ, nm:n] = jnp.where(tri_tail, s_tail, NEG)

        def softmax(idx):
            i, b, CH = blocks[idx], idx % 2, CHS[idx]
            n = (i + 1) * TQ
            nm = n - HQ
            ls = []
            sms = []
            for g in range(TQ // RG):
                ne = nm if g * RG < HQ else n
                rows = slice(g * RG, (g + 1) * RG)
                mx = s_buf[b][rows, 0:128]
                if g >= CH:
                    mx = mx + sms[g - CH] * 0.0
                for t in range(1, ne // 128):
                    mx = jnp.maximum(mx, s_buf[b][rows, t * 128:(t + 1) * 128])
                m = jnp.broadcast_to(jnp.max(mx, axis=1, keepdims=True), (RG, 128))
                sm = None
                for t0 in range(0, ne, 256):
                    pgs = []
                    for t in range(t0, min(t0 + 256, ne), 128):
                        pg = jnp.exp2(s_buf[b][rows, t:t + 128] - m)
                        sm = pg if sm is None else sm + pg
                        pgs.append(pg)
                    p_buf[b][rows, t0:t0 + 128 * len(pgs)] = jnp.concatenate(pgs, axis=1).astype(BF)
                sms.append(sm)
                ls.append(jnp.sum(sm, axis=1, keepdims=True))
            return jnp.concatenate(ls, axis=0)

        def context(idx, l):
            i, b = blocks[idx], idx % 2
            n = (i + 1) * TQ
            nm = n - HQ
            ctx = _dot(p_buf[b][:, 0:nm], _bf(kv[slot, pl.ds(0, nm // 2), E:2 * E]))
            ctx_t = _dot(p_buf[b][HQ:TQ, nm:n], _bf(kv[slot, pl.ds(nm // 2, HQ // 2), E:2 * E]))
            ctx = jnp.concatenate([ctx[0:HQ], ctx[HQ:TQ] + ctx_t], axis=0)
            return (ctx * (1.0 / l)).astype(BF)

        def out_proj(idx, ctx):
            acct[PADL:PADL + DM, pl.ds(blocks[idx] * TQ, TQ)] += _dot_nt(wot_h, ctx)

        scores(0)
        hp = jnp.maximum(h - 1, 0)
        acct[PADL:PADL + DM, pl.ds(S - TQ, TQ)] += _dot_nt(
            bwot[pl.ds(pl.multiple_of(hp * DM, DM), DM), :], ctx_last[...])
        ctx = None
        for idx in range(NQ):
            l = softmax(idx)
            filler(idx)
            if idx + 1 < NQ:
                scores(idx + 1)
            if ctx is not None:
                out_proj(idx - 1, ctx)
            ctx = context(idx, l)
        ctx_last[...] = ctx

    def deint_a(t):
        dst = aw_d.at[pl.ds(pl.multiple_of(t * 16, 16), 16)]
        for w_i in range(3):
            for half in range(2):
                r32 = a_raw.at[w_i, half].bitcast(U32).at[pl.ds(pl.multiple_of(t * 256, 256), 256)]

                def store(hd, r, v, c0=w_i * HE + half * 128):
                    dst[r:r + 8, c0 + hd * E:c0 + hd * E + 128] = v

                _deint_block(r32, 32, store, DCH)

    def prep_a(t):
        awo_d[pl.ds(pl.multiple_of(t * (E // 2), E // 2), E // 2), :] = _u32(
            awot[pl.ds(pl.multiple_of(t * DM, DM), DM), :].T)
        cc = pl.ds(pl.multiple_of(t * 128, 128), 128)
        xa[cc, :] = xat[:, cc].T

    def head(h, carry):
        slot = lax.bitwise_and(h, 1)
        hn = jnp.minimum(h + 1, H - 1)

        @pl.when(h == DM // 64)
        def _():
            wait(cp_late[1])

        def filler(idx):
            if KD == 256:
                if idx < NQ - 1:
                    kv_chunk(h, slot, (idx + 1) * TQ, TQ)
                else:
                    kv_chunk(hn, 1 - slot, 0, TQ)
            else:
                if 1 <= idx < NQ - 1:
                    kv_chunk(h, slot, (idx + 1) * TQ, TQ)
                elif idx == NQ - 1:
                    kv_chunk(hn, 1 - slot, 0, 2 * TQ)
            if idx == 2:
                deint_a(jnp.minimum(h, DM // 32 - 1))
            if idx == 3:
                prep_a(h)

        attention(h, slot, filler, CHL)
        return carry

    ctx_last[...] = jnp.zeros(ctx_last.shape, BF)
    lax.fori_loop(0, H, head, 0)
    acct[PADL:PADL + DM, S - TQ:S] += _dot_nt(bwot[(H - 1) * DM:H * DM, :], ctx_last[...])

    L = 48
    LV = M + SEG
    PR = 2 * SEG
    XE = 40
    XO = PR - XE
    NP = NSEG // 2
    OC = 4
    NOC = NP // OC
    ORS = OC * PR

    zpad = jnp.zeros((2, L - LV, HE), BF)
    zq[:, LV:L, :] = zpad
    zk[:, LV:L, :] = zpad
    zv[:, LV:L, :] = zpad
    oxe[...] = jnp.zeros(oxe.shape, BF)
    mem[...] = mem0_ref[...].astype(F32)

    def out_copy(k):
        r = pl.ds(pl.multiple_of(k * ORS, ORS), ORS)
        return pltpu.make_async_copy(obuf.at[r, :], out_hbm.at[r, :], osems.at[k])

    def b_out(t):
        r = pl.ds(pl.multiple_of(lax.shift_right_logical(t, 1) * 128, 128), 128)
        f0 = pl.multiple_of(lax.bitwise_and(t, 1) * 256, 256)
        obuf[r, pl.ds(pl.multiple_of(DM - PADL + f0, 128), 256)] = acct[pl.ds(f0, 256), r].astype(BF).T

    def substep(odd, r0, ro, mask_m, mask_x, filler):
        cur = int(odd)
        nx = XO if odd else XE
        x0 = XE if odd else 0
        R = nx + M
        oxo_lhs = oxo if odd else oxe

        def scatter(dst, z):
            if odd:
                dst[1, XE - SEG:SEG, :] = z[0:XO].astype(BF)
            else:
                dst[0, 0:SEG, :] = z[0:SEG].astype(BF)
                dst[1, 0:XE - SEG, :] = z[SEG:XE].astype(BF)

        lhs = jnp.concatenate([xa[pl.ds(r0 + x0, nx), :].astype(F32), mem[...]], axis=0).astype(BF)
        zqk = _dot(lhs, _bf(aw_d[:, 0:2 * HE]))
        zqs = zqk[:, 0:HE] * scale
        scatter(zq, zqs)
        zq[cur, SEG:LV, :] = zqs[nx:R].astype(BF)
        scatter(zk, zqk[:, HE:2 * HE])
        zk[cur, SEG:LV, :] = zqk[nx:R, HE:2 * HE].astype(BF)
        sc = [_dot_nt(zq[cur, :, h * E:(h + 1) * E], zk[cur, :, h * E:(h + 1) * E]) for h in range(H)]
        zvv = _dot(lhs, _bf(aw_d[:, 2 * HE:3 * HE]))
        scatter(zv, zvv)
        zv[cur, SEG:LV, :] = zvv[nx:R].astype(BF)
        pm = _softmax_rows(jnp.concatenate([a[SEG:LV] for a in sc], axis=0), mask_m)
        px = _softmax_rows(jnp.concatenate([a[0:SEG] for a in sc], axis=0), mask_x).astype(BF)
        for h in range(H):
            oxo_lhs[nx:R, h * E:(h + 1) * E] = _dot(
                pm[h * M:(h + 1) * M].astype(BF), zv[cur, :, h * E:(h + 1) * E]).astype(BF)

        def x_pv(h):
            oh = _dot(px[h * SEG:(h + 1) * SEG], zv[cur, :, h * E:(h + 1) * E])
            cols = slice(h * E, (h + 1) * E)
            if odd:
                oxe[XE - SEG:XE, cols] = oh.astype(BF)
            else:
                oxo[0:XO, cols] = oh[0:XO].astype(BF)
                return oh[XO:SEG].astype(BF)

        filler()
        NE = int(os.environ.get('NE', 4))
        early = [x_pv(h) for h in range(NE)]
        o = _dot(oxo_lhs[...], _bf(awo_d[...]))
        obuf[pl.ds(ro, nx), 0:DM] = o[0:nx].astype(BF)
        mem[...] = o[nx:R]
        late = [x_pv(h) for h in range(NE, H)]
        if not odd:
            for h, v in enumerate(early + late):
                oxe[0:XE - SEG, h * E:(h + 1) * E] = v

    def pair(t, carry):
        colm = lax.broadcasted_iota(jnp.int32, (H * M, L), 1)
        mask_m = colm < LV
        rowx = lax.bitwise_and(lax.broadcasted_iota(jnp.int32, (H * SEG, L), 0), SEG - 1)
        colx = lax.broadcasted_iota(jnp.int32, (H * SEG, L), 1)
        mask_x = (colx < LV) & ((rowx >= colx) | (colx >= SEG))
        r0 = pl.multiple_of(t * PR, PR)
        re = pl.multiple_of(jnp.maximum(r0 - XE, XO), 8)
        substep(False, r0, re, mask_m, mask_x, lambda: b_out(t))
        substep(True, r0, r0, mask_m, mask_x, lambda: None)

        @pl.when(jnp.logical_and(lax.bitwise_and(t, OC - 1) == 0, t > 0))
        def _():
            out_copy(lax.shift_right_logical(t, 2) - 1).start()

        return carry

    lax.fori_loop(0, NP, pair, 0)
    obuf[S - XE:S, 0:DM] = _dot(oxe[...], _bf(awo_d[...]))[0:XE].astype(BF)
    out_copy(NOC - 1).start()
    for k in range(NOC):
        out_copy(k).wait()


@functools.partial(jax.jit, static_argnames=("A_seg_len",))
def pallas_concat_heads__memory_aug_recurrent_mem_tr__compressed_kv_cla__prompt_kernel(
    A_x, A_mem0, A_Wq, A_Wk, A_Wv, A_Wo, A_seg_len,
    B_x, B_c_kv, B_w_q, B_w_uk, B_w_uv, B_w_o,
):
    _, S, DM = A_x.shape
    _, H, E = A_Wq.shape
    M = A_mem0.shape[1]
    DC = B_c_kv.shape[2]
    SEG = int(A_seg_len)
    assert (S, DM, H, E, M, DC, SEG) == (2048, 448, 16, 256, 8, 1024, 32)
    HE = H * E
    any_spec = pl.BlockSpec(memory_space=pl.ANY)
    vm = pltpu.VMEM
    scratch = [
        vm((DM, S), BF), vm((S, DM), BF), vm((S, DC), BF),
        vm((2, DM * H, 128), BF), vm((2, DC * H, 128), BF), vm((2, DC * H, 128), BF),
        vm((H * DM, E), BF),
        vm((2, DM // 2, HE // 2), U32), vm((H, DC // 2, 2 * E), U32),
        vm((H, S // 2, E), U32), vm((2, S // 2, 2 * E), U32),
        vm((512, S), F32),
        vm((256, S), F32), vm((256, S), F32), vm((256, S), BF), vm((256, S), BF), vm((256, E), BF),
        vm((DM, S), BF), vm((S, DM), BF),
        vm((3, 2, DM * H, 128), BF), vm((H * DM, E), BF),
        vm((DM // 2, 3 * HE), U32), vm((HE // 2, DM), U32),
        vm((M, DM), F32),
        vm((2, 48, HE), BF), vm((2, 48, HE), BF), vm((2, 48, HE), BF),
        vm((48, HE), BF), vm((32, HE), BF),
        vm((S, 2 * DM), BF),
        pltpu.SemaphoreType.DMA((29,)), pltpu.SemaphoreType.DMA((8,)),
    ]
    out = pl.pallas_call(
        functools.partial(_kernel, S=S, DM=DM, H=H, E=E, DC=DC, M=M, SEG=SEG),
        out_shape=jax.ShapeDtypeStruct((S, 2 * DM), BF),
        in_specs=[any_spec, pl.BlockSpec(memory_space=pltpu.VMEM)] + [any_spec] * 10,
        out_specs=any_spec,
        scratch_shapes=scratch,
        compiler_params=pltpu.CompilerParams(vmem_limit_bytes=126 * 1024 * 1024),
    )(
        jnp.swapaxes(A_x, 1, 2).reshape(DM, S), A_mem0.reshape(M, DM),
        A_Wq.reshape(DM * H, E), A_Wk.reshape(DM * H, E), A_Wv.reshape(DM * H, E),
        jnp.swapaxes(A_Wo, 1, 2).reshape(H * DM, E),
        jnp.swapaxes(B_x, 1, 2).reshape(DM, S), B_c_kv.reshape(S, DC),
        B_w_q.reshape(DM * H, E), B_w_uk.reshape(DC * H, E), B_w_uv.reshape(DC * H, E),
        jnp.swapaxes(B_w_o, 1, 2).reshape(H * DM, E),
    )
    return out.reshape(1, S, 2 * DM)
```

```python
import functools
import os

import jax
import jax.numpy as jnp
from jax import lax
from jax.experimental import pallas as pl
from jax.experimental.pallas import tpu as pltpu

BF = jnp.bfloat16
F32 = jnp.float32
U32 = jnp.uint32
NT = (((1,), (1,)), ((), ()))
NEG = -1000000000.0


def _bf(x32):
    return pltpu.bitcast(x32, BF)


def _u32(xb):
    return pltpu.bitcast(xb, U32)


def _dot(a, b):
    return jnp.dot(a, b, preferred_element_type=F32)


def _dot_nt(a, b):
    return lax.dot_general(a, b, NT, preferred_element_type=F32)


def _deint(raw32, j, r0, gate=None):
    ev = raw32[pl.ds(r0 * 8 + j, 8, stride=16), :]
    od = raw32[pl.ds(r0 * 8 + j + 8, 8, stride=16), :]
    if gate is not None:
        ev = ev | gate
    lo = (ev & jnp.uint32(0xFFFF)) | (od << 16)
    hi = (ev >> 16) | (od & jnp.uint32(0xFFFF0000))
    return lo, hi


def _deint_block(raw32, nrows, store, chain):
    done = []
    for r0 in range(0, nrows, 16):
        for j in range(8):
            gate = _zero_after(done[-chain]) if 0 < chain <= len(done) else None
            lo, hi = _deint(raw32, j, r0, gate)
            store(2 * j, r0 // 2, lo)
            store(2 * j + 1, r0 // 2, hi)
            done.append(hi)


def _zero_after(x):
    return (pltpu.bitcast(x, U32) >> 16) >> 16


def _softmax_rows(sc, mask):
    sc = jnp.where(mask, sc, NEG)
    m = jnp.max(sc, axis=1, keepdims=True)
    p = jnp.exp(sc - m)
    l = jnp.sum(p, axis=1, keepdims=True)
    return p * (1.0 / l)


def _kernel(xa_hbm, mem0_ref, awq_hbm, awk_hbm, awv_hbm, awo_hbm,
            xb_hbm, c_hbm, bwq_hbm, bwuk_hbm, bwuv_hbm, bwo_hbm,
            out_hbm,
            xbt, xb, c, bwq_raw, bwuk_raw, bwuv_raw, bwot, bwq_d, wkv_d, q_all, kv, acct, s_buf0, s_buf1, p_buf0, p_buf1, ctx_last,
            xat, xa, a_raw, awot, aw_d, awo_d, mem, zq, zk, zv, oxe, oxo, obuf,
            sems, osems,
            *, S, DM, H, E, DC, M, SEG):
    HE = H * E
    NSEG = S // SEG
    scale = E ** -0.5
    s_buf = (s_buf0, s_buf1)
    p_buf = (p_buf0, p_buf1)

    nsem = [0]

    def copy(src, dst):
        nsem[0] += 1
        return pltpu.make_async_copy(src, dst, sems.at[nsem[0] - 1])

    def slab(src, dst, part):
        nr = src.shape[0] // 2
        rows = pl.ds(part * nr, nr)
        return [copy(src.at[rows, pl.ds(i * 128, 128)], dst.at[i, rows]) for i in range(2)]

    def rows_half(src, dst, part):
        nr = src.shape[0] // 2
        return copy(src.at[pl.ds(part * nr, nr)], dst.at[pl.ds(part * nr, nr)])

    cp_bwq = [copy(bwq_hbm.at[:, pl.ds(i * 128, 128)], bwq_raw.at[i]) for i in range(2)]
    cp_xb = [copy(xb_hbm.at[:, 0:512], xbt.at[:, 0:512]), copy(xb_hbm.at[:, 512:S], xbt.at[:, 512:S])]
    cp_c = copy(c_hbm, c)
    cp_xa = copy(xa_hbm, xat)
    cp_wkv = [slab(bwuk_hbm, bwuk_raw, p) + slab(bwuv_hbm, bwuv_raw, p) for p in range(2)]
    cp_late = [[rows_half(bwo_hbm, bwot, p), rows_half(awo_hbm, awot, p)]
               + slab(awq_hbm, a_raw.at[0], p) + slab(awk_hbm, a_raw.at[1], p) + slab(awv_hbm, a_raw.at[2], p)
               for p in range(2)]

    def start(cps):
        for cp in cps:
            cp.start()

    def wait(cps):
        for cp in cps:
            cp.wait()

    TQP = 512
    PADL = 512 - DM
    ZR = 512 // 16
    scale2 = scale * 1.4426950408889634

    def xb_t(i):
        cc = pl.ds(pl.multiple_of(i * 256, 256), 256)
        xb[cc, :] = xbt[:, cc].T

    def deint_bwq(half):
        def body(t, carry):
            r32 = bwq_raw.at[half].bitcast(U32).at[pl.ds(pl.multiple_of(t * 512, 512), 512)]
            dst = bwq_d.at[half, pl.ds(pl.multiple_of(t * 32, 32), 32)]

            def store(hd, r, v):
                dst[r:r + 8, hd * 128:(hd + 1) * 128] = v

            _deint_block(r32, 64, store, 0)
            return carry

        lax.fori_loop(0, DM // 64, body, 0)

    def q_step(half, t):
        i = lax.shift_right_logical(t, 1)
        n = lax.bitwise_and(t, 1)
        r0 = pl.multiple_of(i * TQP, TQP)
        c0 = pl.multiple_of(n * 1024, 1024)
        z = _dot(xb[pl.ds(r0, TQP), :], _bf(bwq_d[half, :, pl.ds(c0, 1024)])) * scale2
        z = _u32(z.astype(BF))
        rr = pl.ds(pl.multiple_of(i * (TQP // 2), TQP // 2), TQP // 2)
        for hh in range(8):
            q_all[n * 8 + hh, rr, half * 128:(half + 1) * 128] = z[:, hh * 128:(hh + 1) * 128]
        acct[pl.ds(pl.multiple_of((half * 8 + t) * ZR, ZR), ZR), :] = jnp.zeros((ZR, S), F32)

    start([cp_xb[0], cp_bwq[0]])
    cp_xb[0].wait()

    def xb_t0(i, carry):
        xb_t(i)
        return carry

    lax.fori_loop(0, 2, xb_t0, 0)
    cp_bwq[0].wait()
    cp_xb[1].start()
    deint_bwq(0)
    start([cp_bwq[1]] + cp_wkv[0])

    DCH = int(os.environ.get('DCH', 1))

    def deint_kv(t):
        for w_i, raw in enumerate((bwuk_raw, bwuv_raw)):
            for half in range(2):
                r32 = raw.at[half].bitcast(U32).at[pl.ds(pl.multiple_of(t * 1024, 1024), 1024)]
                dst = wkv_d.at[:, pl.ds(pl.multiple_of(t * 64, 64), 64)]

                def store(hd, r, v, c0=w_i * E + half * 128, dst=dst):
                    dst[hd, r:r + 8, c0:c0 + 128] = v

                _deint_block(r32, 128, store, DCH)

    W3 = int(os.environ.get('W3', 4))
    W4 = int(os.environ.get('W4', 2))

    def q_lo(t, carry):
        @pl.when(t == W3)
        def _():
            start(cp_wkv[1] + [cp_c])

        @pl.when(t == 1)
        def _():
            cp_xb[1].wait()

        q_step(0, t)
        j = jnp.minimum(lax.shift_right_logical(t + 1, 1), S // 512 - 1)
        xb_t(2 * j)
        xb_t(2 * j + 1)
        return carry

    def q_hi(t, carry):
        @pl.when(t == W4)
        def _():
            start([cp_xa] + cp_late[0])

        @pl.when(t == 4)
        def _():
            wait(cp_wkv[1])

        q_step(1, t)
        deint_kv(t)
        return carry

    lax.fori_loop(0, 8, q_lo, 0)
    cp_bwq[1].wait()
    deint_bwq(1)
    wait(cp_wkv[0])
    lax.fori_loop(0, 8, q_hi, 0)
    cp_c.wait()

    TQ = 256
    NQ = S // TQ
    HQ = TQ // 2

    def kv_chunk(h, slot, r0, nr):
        z = _dot(c[pl.ds(r0, nr), :], _bf(wkv_d[h]))
        kv[slot, pl.ds(r0 // 2, nr // 2), :] = _u32(z.astype(BF))

    KD = int(os.environ.get('KD', 256))
    kv_chunk(0, 0, 0, KD)
    wait([cp_xa] + cp_late[0])
    start(cp_late[1])

    RG = int(os.environ.get('RG', 8))
    CHL = [int(v) for v in os.environ.get('CH', '43222223')]

    def attention(h, slot, filler, CHS):
        wot_h = bwot[pl.ds(pl.multiple_of(h * DM, DM), DM), :]
        row = lax.broadcasted_iota(jnp.int32, (TQ, HQ), 0)
        col = lax.broadcasted_iota(jnp.int32, (TQ, HQ), 1)
        tri_main = row >= col
        tri_tail = tri_main[0:HQ]
        blocks = list(range(NQ))

        def scores(idx):
            i, b = blocks[idx], idx % 2
            n = (i + 1) * TQ
            nm = n - HQ
            nf = n - TQ
            q = _bf(q_all[h, pl.ds(i * TQ // 2, TQ // 2), :])
            if nf > 0:
                s_buf[b][:, 0:nf] = _dot_nt(q, _bf(kv[slot, pl.ds(0, nf // 2), 0:E]))
            s_mid = _dot_nt(q, _bf(kv[slot, pl.ds(nf // 2, HQ // 2), 0:E]))
            s_buf[b][:, nf:nm] = jnp.where(tri_main, s_mid, NEG)
            s_tail = _dot_nt(q[HQ:TQ], _bf(kv[slot, pl.ds(nm // 2, HQ // 2), 0:E]))
            s_buf[b][HQ:TQ, nm:n] = jnp.where(tri_tail, s_tail, NEG)

        def softmax(idx):
            i, b, CH = blocks[idx], idx % 2, CHS[idx]
            n = (i + 1) * TQ
            nm = n - HQ
            ls = []
            sms = []
            for g in range(TQ // RG):
                ne = nm if g * RG < HQ else n
                rows = slice(g * RG, (g + 1) * RG)
                mx = s_buf[b][rows, 0:128]
                if g >= CH:
                    mx = mx + sms[g - CH] * 0.0
                for t in range(1, ne // 128):
                    mx = jnp.maximum(mx, s_buf[b][rows, t * 128:(t + 1) * 128])
                m = jnp.broadcast_to(jnp.max(mx, axis=1, keepdims=True), (RG, 128))
                sm = None
                for t0 in range(0, ne, 256):
                    pgs = []
                    for t in range(t0, min(t0 + 256, ne), 128):
                        pg = jnp.exp2(s_buf[b][rows, t:t + 128] - m)
                        sm = pg if sm is None else sm + pg
                        pgs.append(pg)
                    p_buf[b][rows, t0:t0 + 128 * len(pgs)] = jnp.concatenate(pgs, axis=1).astype(BF)
                sms.append(sm)
                ls.append(jnp.sum(sm, axis=1, keepdims=True))
            return jnp.concatenate(ls, axis=0)

        def context(idx, l):
            i, b = blocks[idx], idx % 2
            n = (i + 1) * TQ
            nm = n - HQ
            ctx = _dot(p_buf[b][:, 0:nm], _bf(kv[slot, pl.ds(0, nm // 2), E:2 * E]))
            ctx_t = _dot(p_buf[b][HQ:TQ, nm:n], _bf(kv[slot, pl.ds(nm // 2, HQ // 2), E:2 * E]))
            ctx = jnp.concatenate([ctx[0:HQ], ctx[HQ:TQ] + ctx_t], axis=0)
            return (ctx * (1.0 / l)).astype(BF)

        def out_proj(idx, ctx):
            acct[PADL:PADL + DM, pl.ds(blocks[idx] * TQ, TQ)] += _dot_nt(wot_h, ctx)

        scores(0)
        hp = jnp.maximum(h - 1, 0)
        acct[PADL:PADL + DM, pl.ds(S - TQ, TQ)] += _dot_nt(
            bwot[pl.ds(pl.multiple_of(hp * DM, DM), DM), :], ctx_last[...])
        ctx = None
        for idx in range(NQ):
            l = softmax(idx)
            filler(idx)
            if idx + 1 < NQ:
                scores(idx + 1)
            if ctx is not None:
                out_proj(idx - 1, ctx)
            ctx = context(idx, l)
        ctx_last[...] = ctx

    def deint_a(t):
        dst = aw_d.at[pl.ds(pl.multiple_of(t * 16, 16), 16)]
        for w_i in range(3):
            for half in range(2):
                r32 = a_raw.at[w_i, half].bitcast(U32).at[pl.ds(pl.multiple_of(t * 256, 256), 256)]

                def store(hd, r, v, c0=w_i * HE + half * 128):
                    dst[r:r + 8, c0 + hd * E:c0 + hd * E + 128] = v

                _deint_block(r32, 32, store, DCH)

    def prep_a(t):
        awo_d[pl.ds(pl.multiple_of(t * (E // 2), E // 2), E // 2), :] = _u32(
            awot[pl.ds(pl.multiple_of(t * DM, DM), DM), :].T)
        cc = pl.ds(pl.multiple_of(t * 128, 128), 128)
        xa[cc, :] = xat[:, cc].T

    def head(h, carry):
        slot = lax.bitwise_and(h, 1)
        hn = jnp.minimum(h + 1, H - 1)

        @pl.when(h == DM // 64)
        def _():
            wait(cp_late[1])

        def filler(idx):
            if KD == 256:
                if idx < NQ - 1:
                    kv_chunk(h, slot, (idx + 1) * TQ, TQ)
                else:
                    kv_chunk(hn, 1 - slot, 0, TQ)
            else:
                if 1 <= idx < NQ - 1:
                    kv_chunk(h, slot, (idx + 1) * TQ, TQ)
                elif idx == NQ - 1:
                    kv_chunk(hn, 1 - slot, 0, 2 * TQ)
            if idx == 2:
                deint_a(jnp.minimum(h, DM // 32 - 1))
            if idx == 3:
                prep_a(h)

        attention(h, slot, filler, CHL)
        return carry

    ctx_last[...] = jnp.zeros(ctx_last.shape, BF)
    lax.fori_loop(0, H, head, 0)
    acct[PADL:PADL + DM, S - TQ:S] += _dot_nt(bwot[(H - 1) * DM:H * DM, :], ctx_last[...])

    L = 48
    LV = M + SEG
    PR = 2 * SEG
    XE = 40
    XO = PR - XE
    NP = NSEG // 2
    OC = 4
    NOC = NP // OC
    ORS = OC * PR

    zpad = jnp.zeros((2, L - LV, HE), BF)
    zq[:, LV:L, :] = zpad
    zk[:, LV:L, :] = zpad
    zv[:, LV:L, :] = zpad
    oxe[...] = jnp.zeros(oxe.shape, BF)
    mem[...] = mem0_ref[...].astype(F32)

    def out_copy(k):
        r = pl.ds(pl.multiple_of(k * ORS, ORS), ORS)
        return pltpu.make_async_copy(obuf.at[r, :], out_hbm.at[r, :], osems.at[k])

    def b_out(t):
        r = pl.ds(pl.multiple_of(lax.shift_right_logical(t, 1) * 128, 128), 128)
        f0 = pl.multiple_of(lax.bitwise_and(t, 1) * 256, 256)
        blk = acct[pl.ds(f0, 256), r].astype(BF)
        if os.environ.get('BO', 'xlu') == 'mxu':
            eye = (lax.broadcasted_iota(jnp.int32, (128, 128), 0)
                   == lax.broadcasted_iota(jnp.int32, (128, 128), 1)).astype(BF)
            blk_t = _dot_nt(eye, blk).astype(BF)
        else:
            blk_t = blk.T
        obuf[r, pl.ds(pl.multiple_of(DM - PADL + f0, 128), 256)] = blk_t

    def substep(odd, r0, ro, mask_m, mask_x, filler):
        cur = int(odd)
        nx = XO if odd else XE
        x0 = XE if odd else 0
        R = nx + M
        oxo_lhs = oxo if odd else oxe

        def scatter(dst, z):
            if odd:
                dst[1, XE - SEG:SEG, :] = z[0:XO].astype(BF)
            else:
                dst[0, 0:SEG, :] = z[0:SEG].astype(BF)
                dst[1, 0:XE - SEG, :] = z[SEG:XE].astype(BF)

        lhs = jnp.concatenate([xa[pl.ds(r0 + x0, nx), :].astype(F32), mem[...]], axis=0).astype(BF)
        zqk = _dot(lhs, _bf(aw_d[:, 0:2 * HE]))
        zqs = zqk[:, 0:HE] * scale
        scatter(zq, zqs)
        zq[cur, SEG:LV, :] = zqs[nx:R].astype(BF)
        scatter(zk, zqk[:, HE:2 * HE])
        zk[cur, SEG:LV, :] = zqk[nx:R, HE:2 * HE].astype(BF)
        sc = [_dot_nt(zq[cur, :, h * E:(h + 1) * E], zk[cur, :, h * E:(h + 1) * E]) for h in range(H)]
        zvv = _dot(lhs, _bf(aw_d[:, 2 * HE:3 * HE]))
        scatter(zv, zvv)
        zv[cur, SEG:LV, :] = zvv[nx:R].astype(BF)
        pm = _softmax_rows(jnp.concatenate([a[SEG:LV] for a in sc], axis=0), mask_m)
        px = _softmax_rows(jnp.concatenate([a[0:SEG] for a in sc], axis=0), mask_x).astype(BF)
        for h in range(H):
            oxo_lhs[nx:R, h * E:(h + 1) * E] = _dot(
                pm[h * M:(h + 1) * M].astype(BF), zv[cur, :, h * E:(h + 1) * E]).astype(BF)

        def x_pv(h):
            oh = _dot(px[h * SEG:(h + 1) * SEG], zv[cur, :, h * E:(h + 1) * E])
            cols = slice(h * E, (h + 1) * E)
            if odd:
                oxe[XE - SEG:XE, cols] = oh.astype(BF)
            else:
                oxo[0:XO, cols] = oh[0:XO].astype(BF)
                return oh[XO:SEG].astype(BF)

        filler()
        NE = int(os.environ.get('NE', 4))
        early = [x_pv(h) for h in range(NE)]
        o = _dot(oxo_lhs[...], _bf(awo_d[...]))
        obuf[pl.ds(ro, nx), 0:DM] = o[0:nx].astype(BF)
        mem[...] = o[nx:R]
        late = [x_pv(h) for h in range(NE, H)]
        if not odd:
            for h, v in enumerate(early + late):
                oxe[0:XE - SEG, h * E:(h + 1) * E] = v

    def pair(t, carry):
        colm = lax.broadcasted_iota(jnp.int32, (H * M, L), 1)
        mask_m = colm < LV
        rowx = lax.bitwise_and(lax.broadcasted_iota(jnp.int32, (H * SEG, L), 0), SEG - 1)
        colx = lax.broadcasted_iota(jnp.int32, (H * SEG, L), 1)
        mask_x = (colx < LV) & ((rowx >= colx) | (colx >= SEG))
        r0 = pl.multiple_of(t * PR, PR)
        re = pl.multiple_of(jnp.maximum(r0 - XE, XO), 8)
        substep(False, r0, re, mask_m, mask_x, lambda: b_out(t))
        substep(True, r0, r0, mask_m, mask_x, lambda: None)

        @pl.when(jnp.logical_and(lax.bitwise_and(t, OC - 1) == 0, t > 0))
        def _():
            out_copy(lax.shift_right_logical(t, 2) - 1).start()

        return carry

    lax.fori_loop(0, NP, pair, 0)
    TL = 48
    tail = [pltpu.make_async_copy(obuf.at[a:b, :], out_hbm.at[a:b, :], osems.at[k])
            for a, b, k in ((S - ORS, S - TL, NOC - 1), (S - TL, S, NOC))]
    tail[0].start()
    obuf[S - XE:S, 0:DM] = _dot(oxe[...], _bf(awo_d[...]))[0:XE].astype(BF)
    tail[1].start()
    for k in range(NOC - 1):
        out_copy(k).wait()
    wait(tail)


@functools.partial(jax.jit, static_argnames=("A_seg_len",))
def pallas_concat_heads__memory_aug_recurrent_mem_tr__compressed_kv_cla__prompt_kernel(
    A_x, A_mem0, A_Wq, A_Wk, A_Wv, A_Wo, A_seg_len,
    B_x, B_c_kv, B_w_q, B_w_uk, B_w_uv, B_w_o,
):
    _, S, DM = A_x.shape
    _, H, E = A_Wq.shape
    M = A_mem0.shape[1]
    DC = B_c_kv.shape[2]
    SEG = int(A_seg_len)
    assert (S, DM, H, E, M, DC, SEG) == (2048, 448, 16, 256, 8, 1024, 32)
    HE = H * E
    any_spec = pl.BlockSpec(memory_space=pl.ANY)
    vm = pltpu.VMEM
    scratch = [
        vm((DM, S), BF), vm((S, DM), BF), vm((S, DC), BF),
        vm((2, DM * H, 128), BF), vm((2, DC * H, 128), BF), vm((2, DC * H, 128), BF),
        vm((H * DM, E), BF),
        vm((2, DM // 2, HE // 2), U32), vm((H, DC // 2, 2 * E), U32),
        vm((H, S // 2, E), U32), vm((2, S // 2, 2 * E), U32),
        vm((512, S), F32),
        vm((256, S), F32), vm((256, S), F32), vm((256, S), BF), vm((256, S), BF), vm((256, E), BF),
        vm((DM, S), BF), vm((S, DM), BF),
        vm((3, 2, DM * H, 128), BF), vm((H * DM, E), BF),
        vm((DM // 2, 3 * HE), U32), vm((HE // 2, DM), U32),
        vm((M, DM), F32),
        vm((2, 48, HE), BF), vm((2, 48, HE), BF), vm((2, 48, HE), BF),
        vm((48, HE), BF), vm((32, HE), BF),
        vm((S, 2 * DM), BF),
        pltpu.SemaphoreType.DMA((30,)), pltpu.SemaphoreType.DMA((9,)),
    ]
    out = pl.pallas_call(
        functools.partial(_kernel, S=S, DM=DM, H=H, E=E, DC=DC, M=M, SEG=SEG),
        out_shape=jax.ShapeDtypeStruct((S, 2 * DM), BF),
        in_specs=[any_spec, pl.BlockSpec(memory_space=pltpu.VMEM)] + [any_spec] * 10,
        out_specs=any_spec,
        scratch_shapes=scratch,
        compiler_params=pltpu.CompilerParams(vmem_limit_bytes=126 * 1024 * 1024),
    )(
        jnp.swapaxes(A_x, 1, 2).reshape(DM, S), A_mem0.reshape(M, DM),
        A_Wq.reshape(DM * H, E), A_Wk.reshape(DM * H, E), A_Wv.reshape(DM * H, E),
        jnp.swapaxes(A_Wo, 1, 2).reshape(H * DM, E),
        jnp.swapaxes(B_x, 1, 2).reshape(DM, S), B_c_kv.reshape(S, DC),
        B_w_q.reshape(DM * H, E), B_w_uk.reshape(DC * H, E), B_w_uv.reshape(DC * H, E),
        jnp.swapaxes(B_w_o, 1, 2).reshape(H * DM, E),
    )
    return out.reshape(1, S, 2 * DM)
```

```python
import functools

import jax
import jax.numpy as jnp
from jax import lax
from jax.experimental import pallas as pl
from jax.experimental.pallas import tpu as pltpu

BF = jnp.bfloat16
F32 = jnp.float32
U32 = jnp.uint32
NT = (((1,), (1,)), ((), ()))
NEG = -1000000000.0


def _bf(x32):
    return pltpu.bitcast(x32, BF)


def _u32(xb):
    return pltpu.bitcast(xb, U32)


def _dot(a, b):
    return jnp.dot(a, b, preferred_element_type=F32)


def _dot_nt(a, b):
    return lax.dot_general(a, b, NT, preferred_element_type=F32)


def _deint(raw32, j, r0, gate=None):
    ev = raw32[pl.ds(r0 * 8 + j, 8, stride=16), :]
    od = raw32[pl.ds(r0 * 8 + j + 8, 8, stride=16), :]
    if gate is not None:
        ev = ev | gate
    lo = (ev & jnp.uint32(0xFFFF)) | (od << 16)
    hi = (ev >> 16) | (od & jnp.uint32(0xFFFF0000))
    return lo, hi


def _deint_block(raw32, nrows, store, chain):
    done = []
    for r0 in range(0, nrows, 16):
        for j in range(8):
            gate = _zero_after(done[-chain]) if 0 < chain <= len(done) else None
            lo, hi = _deint(raw32, j, r0, gate)
            store(2 * j, r0 // 2, lo)
            store(2 * j + 1, r0 // 2, hi)
            done.append(hi)


def _zero_after(x):
    return (pltpu.bitcast(x, U32) >> 16) >> 16


def _softmax_rows(sc, mask):
    sc = jnp.where(mask, sc, NEG)
    m = jnp.max(sc, axis=1, keepdims=True)
    p = jnp.exp(sc - m)
    l = jnp.sum(p, axis=1, keepdims=True)
    return p * (1.0 / l)


def _kernel(xa_hbm, mem0_ref, awq_hbm, awk_hbm, awv_hbm, awo_hbm,
            xb_hbm, c_hbm, bwq_hbm, bwuk_hbm, bwuv_hbm, bwo_hbm,
            out_hbm,
            xbt, xb, c, bwq_raw, bwuk_raw, bwuv_raw, bwot, bwq_d, wkv_d, q_all, kv, acct, s_buf0, s_buf1, p_buf0, p_buf1, ctx_last,
            xat, xa, a_raw, awot, aw_d, awo_d, mem, zq, zk, zv, oxe, oxo, obuf,
            sems, osems,
            *, S, DM, H, E, DC, M, SEG):
    HE = H * E
    NSEG = S // SEG
    scale = E ** -0.5
    s_buf = (s_buf0, s_buf1)
    p_buf = (p_buf0, p_buf1)

    nsem = [0]

    def copy(src, dst):
        nsem[0] += 1
        return pltpu.make_async_copy(src, dst, sems.at[nsem[0] - 1])

    def slab(src, dst, part):
        nr = src.shape[0] // 2
        rows = pl.ds(part * nr, nr)
        return [copy(src.at[rows, pl.ds(i * 128, 128)], dst.at[i, rows]) for i in range(2)]

    def rows_half(src, dst, part):
        nr = src.shape[0] // 2
        return copy(src.at[pl.ds(part * nr, nr)], dst.at[pl.ds(part * nr, nr)])

    cp_bwq = [copy(bwq_hbm.at[:, pl.ds(i * 128, 128)], bwq_raw.at[i]) for i in range(2)]
    cp_xb = [copy(xb_hbm.at[:, 0:512], xbt.at[:, 0:512]), copy(xb_hbm.at[:, 512:S], xbt.at[:, 512:S])]
    cp_c = copy(c_hbm, c)
    cp_xa = copy(xa_hbm, xat)
    cp_wkv = [slab(bwuk_hbm, bwuk_raw, p) + slab(bwuv_hbm, bwuv_raw, p) for p in range(2)]
    cp_late = [[rows_half(bwo_hbm, bwot, p), rows_half(awo_hbm, awot, p)]
               + slab(awq_hbm, a_raw.at[0], p) + slab(awk_hbm, a_raw.at[1], p) + slab(awv_hbm, a_raw.at[2], p)
               for p in range(2)]

    def start(cps):
        for cp in cps:
            cp.start()

    def wait(cps):
        for cp in cps:
            cp.wait()

    TQP = 512
    PADL = 512 - DM
    ZR = 512 // 16
    scale2 = scale * 1.4426950408889634

    def xb_t(i):
        cc = pl.ds(pl.multiple_of(i * 256, 256), 256)
        xb[cc, :] = xbt[:, cc].T

    def deint_bwq(half):
        def body(t, carry):
            r32 = bwq_raw.at[half].bitcast(U32).at[pl.ds(pl.multiple_of(t * 512, 512), 512)]
            dst = bwq_d.at[half, pl.ds(pl.multiple_of(t * 32, 32), 32)]

            def store(hd, r, v):
                dst[r:r + 8, hd * 128:(hd + 1) * 128] = v

            _deint_block(r32, 64, store, 0)
            return carry

        lax.fori_loop(0, DM // 64, body, 0)

    def q_step(half, t):
        i = lax.shift_right_logical(t, 1)
        n = lax.bitwise_and(t, 1)
        r0 = pl.multiple_of(i * TQP, TQP)
        c0 = pl.multiple_of(n * 1024, 1024)
        z = _dot(xb[pl.ds(r0, TQP), :], _bf(bwq_d[half, :, pl.ds(c0, 1024)])) * scale2
        z = _u32(z.astype(BF))
        rr = pl.ds(pl.multiple_of(i * (TQP // 2), TQP // 2), TQP // 2)
        for hh in range(8):
            q_all[n * 8 + hh, rr, half * 128:(half + 1) * 128] = z[:, hh * 128:(hh + 1) * 128]
        acct[pl.ds(pl.multiple_of((half * 8 + t) * ZR, ZR), ZR), :] = jnp.zeros((ZR, S), F32)

    start([cp_xb[0], cp_bwq[0]])
    cp_xb[0].wait()

    def xb_t0(i, carry):
        xb_t(i)
        return carry

    lax.fori_loop(0, 2, xb_t0, 0)
    cp_bwq[0].wait()
    cp_xb[1].start()
    deint_bwq(0)
    start([cp_bwq[1]] + cp_wkv[0])

    DCH = 1

    def deint_kv(t):
        for w_i, raw in enumerate((bwuk_raw, bwuv_raw)):
            for half in range(2):
                r32 = raw.at[half].bitcast(U32).at[pl.ds(pl.multiple_of(t * 1024, 1024), 1024)]
                dst = wkv_d.at[:, pl.ds(pl.multiple_of(t * 64, 64), 64)]

                def store(hd, r, v, c0=w_i * E + half * 128, dst=dst):
                    dst[hd, r:r + 8, c0:c0 + 128] = v

                _deint_block(r32, 128, store, DCH)

    W3, W4 = 4, 2

    def q_lo(t, carry):
        @pl.when(t == W3)
        def _():
            start(cp_wkv[1] + [cp_c])

        @pl.when(t == 1)
        def _():
            cp_xb[1].wait()

        q_step(0, t)
        j = jnp.minimum(lax.shift_right_logical(t + 1, 1), S // 512 - 1)
        xb_t(2 * j)
        xb_t(2 * j + 1)
        return carry

    def q_hi(t, carry):
        @pl.when(t == W4)
        def _():
            start([cp_xa] + cp_late[0])

        @pl.when(t == 4)
        def _():
            wait(cp_wkv[1])

        q_step(1, t)
        deint_kv(t)
        return carry

    lax.fori_loop(0, 8, q_lo, 0)
    cp_bwq[1].wait()
    deint_bwq(1)
    wait(cp_wkv[0])
    lax.fori_loop(0, 8, q_hi, 0)
    cp_c.wait()

    TQ = 256
    NQ = S // TQ
    HQ = TQ // 2

    def kv_chunk(h, slot, r0, nr):
        z = _dot(c[pl.ds(r0, nr), :], _bf(wkv_d[h]))
        kv[slot, pl.ds(r0 // 2, nr // 2), :] = _u32(z.astype(BF))

    kv_chunk(0, 0, 0, TQ)
    wait([cp_xa] + cp_late[0])
    start(cp_late[1])

    RG = 8
    CHL = [4, 3, 2, 2, 2, 2, 2, 3]

    def attention(h, slot, filler, CHS):
        wot_h = bwot[pl.ds(pl.multiple_of(h * DM, DM), DM), :]
        row = lax.broadcasted_iota(jnp.int32, (TQ, HQ), 0)
        col = lax.broadcasted_iota(jnp.int32, (TQ, HQ), 1)
        tri_main = row >= col
        tri_tail = tri_main[0:HQ]
        blocks = list(range(NQ))

        def scores(idx):
            i, b = blocks[idx], idx % 2
            n = (i + 1) * TQ
            nm = n - HQ
            nf = n - TQ
            q = _bf(q_all[h, pl.ds(i * TQ // 2, TQ // 2), :])
            if nf > 0:
                s_buf[b][:, 0:nf] = _dot_nt(q, _bf(kv[slot, pl.ds(0, nf // 2), 0:E]))
            s_mid = _dot_nt(q, _bf(kv[slot, pl.ds(nf // 2, HQ // 2), 0:E]))
            s_buf[b][:, nf:nm] = jnp.where(tri_main, s_mid, NEG)
            s_tail = _dot_nt(q[HQ:TQ], _bf(kv[slot, pl.ds(nm // 2, HQ // 2), 0:E]))
            s_buf[b][HQ:TQ, nm:n] = jnp.where(tri_tail, s_tail, NEG)

        def softmax(idx):
            i, b, CH = blocks[idx], idx % 2, CHS[idx]
            n = (i + 1) * TQ
            nm = n - HQ
            ls = []
            sms = []
            for g in range(TQ // RG):
                ne = nm if g * RG < HQ else n
                rows = slice(g * RG, (g + 1) * RG)
                mx = s_buf[b][rows, 0:128]
                if g >= CH:
                    mx = pltpu.bitcast(_u32(mx) | _zero_after(sms[g - CH]), F32)
                for t in range(1, ne // 128):
                    mx = jnp.maximum(mx, s_buf[b][rows, t * 128:(t + 1) * 128])
                m = jnp.broadcast_to(jnp.max(mx, axis=1, keepdims=True), (RG, 128))
                sm = None
                for t0 in range(0, ne, 256):
                    pgs = []
                    for t in range(t0, min(t0 + 256, ne), 128):
                        pg = jnp.exp2(s_buf[b][rows, t:t + 128] - m)
                        sm = pg if sm is None else sm + pg
                        pgs.append(pg)
                    p_buf[b][rows, t0:t0 + 128 * len(pgs)] = jnp.concatenate(pgs, axis=1).astype(BF)
                sms.append(sm)
                ls.append(jnp.sum(sm, axis=1, keepdims=True))
            return jnp.concatenate(ls, axis=0)

        def context(idx, l):
            i, b = blocks[idx], idx % 2
            n = (i + 1) * TQ
            nm = n - HQ
            ctx = _dot(p_buf[b][:, 0:nm], _bf(kv[slot, pl.ds(0, nm // 2), E:2 * E]))
            ctx_t = _dot(p_buf[b][HQ:TQ, nm:n], _bf(kv[slot, pl.ds(nm // 2, HQ // 2), E:2 * E]))
            ctx = jnp.concatenate([ctx[0:HQ], ctx[HQ:TQ] + ctx_t], axis=0)
            return (ctx * (1.0 / l)).astype(BF)

        def out_proj(idx, ctx):
            acct[PADL:PADL + DM, pl.ds(blocks[idx] * TQ, TQ)] += _dot_nt(wot_h, ctx)

        scores(0)
        hp = jnp.maximum(h - 1, 0)
        acct[PADL:PADL + DM, pl.ds(S - TQ, TQ)] += _dot_nt(
            bwot[pl.ds(pl.multiple_of(hp * DM, DM), DM), :], ctx_last[...])
        ctx = None
        for idx in range(NQ):
            l = softmax(idx)
            filler(idx)
            if idx + 1 < NQ:
                scores(idx + 1)
            if ctx is not None:
                out_proj(idx - 1, ctx)
            ctx = context(idx, l)
        ctx_last[...] = ctx

    def deint_a(t):
        dst = aw_d.at[pl.ds(pl.multiple_of(t * 16, 16), 16)]
        for w_i in range(3):
            for half in range(2):
                r32 = a_raw.at[w_i, half].bitcast(U32).at[pl.ds(pl.multiple_of(t * 256, 256), 256)]

                def store(hd, r, v, c0=w_i * HE + half * 128):
                    dst[r:r + 8, c0 + hd * E:c0 + hd * E + 128] = v

                _deint_block(r32, 32, store, DCH)

    def prep_a(t):
        awo_d[pl.ds(pl.multiple_of(t * (E // 2), E // 2), E // 2), :] = _u32(
            awot[pl.ds(pl.multiple_of(t * DM, DM), DM), :].T)
        cc = pl.ds(pl.multiple_of(t * 128, 128), 128)
        xa[cc, :] = xat[:, cc].T

    def head(h, carry):
        slot = lax.bitwise_and(h, 1)
        hn = jnp.minimum(h + 1, H - 1)

        @pl.when(h == DM // 64)
        def _():
            wait(cp_late[1])

        def filler(idx):
            if idx < NQ - 1:
                kv_chunk(h, slot, (idx + 1) * TQ, TQ)
            else:
                kv_chunk(hn, 1 - slot, 0, TQ)
            if idx == 2:
                deint_a(jnp.minimum(h, DM // 32 - 1))
            if idx == 3:
                prep_a(h)

        attention(h, slot, filler, CHL)
        return carry

    ctx_last[...] = jnp.zeros(ctx_last.shape, BF)
    lax.fori_loop(0, H, head, 0)
    acct[PADL:PADL + DM, S - TQ:S] += _dot_nt(bwot[(H - 1) * DM:H * DM, :], ctx_last[...])

    L = 48
    LV = M + SEG
    PR = 2 * SEG
    XE = 40
    XO = PR - XE
    NP = NSEG // 2
    OC = 4
    NOC = NP // OC
    ORS = OC * PR

    zpad = jnp.zeros((2, L - LV, HE), BF)
    zq[:, LV:L, :] = zpad
    zk[:, LV:L, :] = zpad
    zv[:, LV:L, :] = zpad
    oxe[...] = jnp.zeros(oxe.shape, BF)
    mem[...] = mem0_ref[...].astype(F32)

    def out_copy(k):
        r = pl.ds(pl.multiple_of(k * ORS, ORS), ORS)
        return pltpu.make_async_copy(obuf.at[r, :], out_hbm.at[r, :], osems.at[k])

    def b_out(t):
        r = pl.ds(pl.multiple_of(lax.shift_right_logical(t, 1) * 128, 128), 128)
        f0 = pl.multiple_of(lax.bitwise_and(t, 1) * 256, 256)
        blk = acct[pl.ds(f0, 256), r].astype(BF)
        obuf[r, pl.ds(pl.multiple_of(DM - PADL + f0, 128), 256)] = blk.T

    def substep(odd, r0, ro, mask_m, mask_x, filler):
        cur = int(odd)
        nx = XO if odd else XE
        x0 = XE if odd else 0
        R = nx + M
        oxo_lhs = oxo if odd else oxe

        def scatter(dst, z):
            if odd:
                dst[1, XE - SEG:SEG, :] = z[0:XO].astype(BF)
            else:
                dst[0, 0:SEG, :] = z[0:SEG].astype(BF)
                dst[1, 0:XE - SEG, :] = z[SEG:XE].astype(BF)

        lhs = jnp.concatenate([xa[pl.ds(r0 + x0, nx), :].astype(F32), mem[...]], axis=0).astype(BF)
        zqk = _dot(lhs, _bf(aw_d[:, 0:2 * HE]))
        zqs = zqk[:, 0:HE] * scale
        scatter(zq, zqs)
        zq[cur, SEG:LV, :] = zqs[nx:R].astype(BF)
        scatter(zk, zqk[:, HE:2 * HE])
        zk[cur, SEG:LV, :] = zqk[nx:R, HE:2 * HE].astype(BF)
        sc = [_dot_nt(zq[cur, :, h * E:(h + 1) * E], zk[cur, :, h * E:(h + 1) * E]) for h in range(H)]
        zvv = _dot(lhs, _bf(aw_d[:, 2 * HE:3 * HE]))
        scatter(zv, zvv)
        zv[cur, SEG:LV, :] = zvv[nx:R].astype(BF)
        pm = _softmax_rows(jnp.concatenate([a[SEG:LV] for a in sc], axis=0), mask_m)
        px = _softmax_rows(jnp.concatenate([a[0:SEG] for a in sc], axis=0), mask_x).astype(BF)
        for h in range(H):
            oxo_lhs[nx:R, h * E:(h + 1) * E] = _dot(
                pm[h * M:(h + 1) * M].astype(BF), zv[cur, :, h * E:(h + 1) * E]).astype(BF)

        def x_pv(h):
            oh = _dot(px[h * SEG:(h + 1) * SEG], zv[cur, :, h * E:(h + 1) * E])
            cols = slice(h * E, (h + 1) * E)
            if odd:
                oxe[XE - SEG:XE, cols] = oh.astype(BF)
            else:
                oxo[0:XO, cols] = oh[0:XO].astype(BF)
                return oh[XO:SEG].astype(BF)

        filler()
        NE = 4
        early = [x_pv(h) for h in range(NE)]
        o = _dot(oxo_lhs[...], _bf(awo_d[...]))
        obuf[pl.ds(ro, nx), 0:DM] = o[0:nx].astype(BF)
        mem[...] = o[nx:R]
        late = [x_pv(h) for h in range(NE, H)]
        if not odd:
            for h, v in enumerate(early + late):
                oxe[0:XE - SEG, h * E:(h + 1) * E] = v

    def pair(t, carry):
        colm = lax.broadcasted_iota(jnp.int32, (H * M, L), 1)
        mask_m = colm < LV
        rowx = lax.bitwise_and(lax.broadcasted_iota(jnp.int32, (H * SEG, L), 0), SEG - 1)
        colx = lax.broadcasted_iota(jnp.int32, (H * SEG, L), 1)
        mask_x = (colx < LV) & ((rowx >= colx) | (colx >= SEG))
        r0 = pl.multiple_of(t * PR, PR)
        re = pl.multiple_of(jnp.maximum(r0 - XE, XO), 8)
        substep(False, r0, re, mask_m, mask_x, lambda: b_out(t))
        substep(True, r0, r0, mask_m, mask_x, lambda: None)

        @pl.when(jnp.logical_and(lax.bitwise_and(t, OC - 1) == 0, t > 0))
        def _():
            out_copy(lax.shift_right_logical(t, 2) - 1).start()

        return carry

    lax.fori_loop(0, NP, pair, 0)
    TL = 48
    tail = [pltpu.make_async_copy(obuf.at[a:b, :], out_hbm.at[a:b, :], osems.at[k])
            for a, b, k in ((S - ORS, S - TL, NOC - 1), (S - TL, S, NOC))]
    tail[0].start()
    obuf[S - XE:S, 0:DM] = _dot(oxe[...], _bf(awo_d[...]))[0:XE].astype(BF)
    tail[1].start()
    for k in range(NOC - 1):
        out_copy(k).wait()
    wait(tail)


@functools.partial(jax.jit, static_argnames=("A_seg_len",))
def pallas_concat_heads__memory_aug_recurrent_mem_tr__compressed_kv_cla__prompt_kernel(
    A_x, A_mem0, A_Wq, A_Wk, A_Wv, A_Wo, A_seg_len,
    B_x, B_c_kv, B_w_q, B_w_uk, B_w_uv, B_w_o,
):
    _, S, DM = A_x.shape
    _, H, E = A_Wq.shape
    M = A_mem0.shape[1]
    DC = B_c_kv.shape[2]
    SEG = int(A_seg_len)
    assert (S, DM, H, E, M, DC, SEG) == (2048, 448, 16, 256, 8, 1024, 32)
    HE = H * E
    any_spec = pl.BlockSpec(memory_space=pl.ANY)
    vm = pltpu.VMEM
    scratch = [
        vm((DM, S), BF), vm((S, DM), BF), vm((S, DC), BF),
        vm((2, DM * H, 128), BF), vm((2, DC * H, 128), BF), vm((2, DC * H, 128), BF),
        vm((H * DM, E), BF),
        vm((2, DM // 2, HE // 2), U32), vm((H, DC // 2, 2 * E), U32),
        vm((H, S // 2, E), U32), vm((2, S // 2, 2 * E), U32),
        vm((512, S), F32),
        vm((256, S), F32), vm((256, S), F32), vm((256, S), BF), vm((256, S), BF), vm((256, E), BF),
        vm((DM, S), BF), vm((S, DM), BF),
        vm((3, 2, DM * H, 128), BF), vm((H * DM, E), BF),
        vm((DM // 2, 3 * HE), U32), vm((HE // 2, DM), U32),
        vm((M, DM), F32),
        vm((2, 48, HE), BF), vm((2, 48, HE), BF), vm((2, 48, HE), BF),
        vm((48, HE), BF), vm((32, HE), BF),
        vm((S, 2 * DM), BF),
        pltpu.SemaphoreType.DMA((30,)), pltpu.SemaphoreType.DMA((9,)),
    ]
    out = pl.pallas_call(
        functools.partial(_kernel, S=S, DM=DM, H=H, E=E, DC=DC, M=M, SEG=SEG),
        out_shape=jax.ShapeDtypeStruct((S, 2 * DM), BF),
        in_specs=[any_spec, pl.BlockSpec(memory_space=pltpu.VMEM)] + [any_spec] * 10,
        out_specs=any_spec,
        scratch_shapes=scratch,
        compiler_params=pltpu.CompilerParams(vmem_limit_bytes=126 * 1024 * 1024),
    )(
        jnp.swapaxes(A_x, 1, 2).reshape(DM, S), A_mem0.reshape(M, DM),
        A_Wq.reshape(DM * H, E), A_Wk.reshape(DM * H, E), A_Wv.reshape(DM * H, E),
        jnp.swapaxes(A_Wo, 1, 2).reshape(H * DM, E),
        jnp.swapaxes(B_x, 1, 2).reshape(DM, S), B_c_kv.reshape(S, DC),
        B_w_q.reshape(DM * H, E), B_w_uk.reshape(DC * H, E), B_w_uv.reshape(DC * H, E),
        jnp.swapaxes(B_w_o, 1, 2).reshape(H * DM, E),
    )
    return out.reshape(1, S, 2 * DM)
```

```python
import functools

import jax
import jax.numpy as jnp
from jax import lax
from jax.experimental import pallas as pl
from jax.experimental.pallas import tpu as pltpu

BF = jnp.bfloat16
F32 = jnp.float32
U32 = jnp.uint32
NT = (((1,), (1,)), ((), ()))
NEG = -1000000000.0


def _bf(x32):
    return pltpu.bitcast(x32, BF)


def _u32(xb):
    return pltpu.bitcast(xb, U32)


def _dot(a, b):
    return jnp.dot(a, b, preferred_element_type=F32)


def _dot_nt(a, b):
    return lax.dot_general(a, b, NT, preferred_element_type=F32)


def _deint(raw32, j, r0, gate=None):
    ev = raw32[pl.ds(r0 * 8 + j, 8, stride=16), :]
    od = raw32[pl.ds(r0 * 8 + j + 8, 8, stride=16), :]
    if gate is not None:
        ev = ev | gate
    lo = (ev & jnp.uint32(0xFFFF)) | (od << 16)
    hi = (ev >> 16) | (od & jnp.uint32(0xFFFF0000))
    return lo, hi


def _deint_block(raw32, nrows, store, chain):
    done = []
    for r0 in range(0, nrows, 16):
        for j in range(8):
            gate = _zero_after(done[-chain]) if 0 < chain <= len(done) else None
            lo, hi = _deint(raw32, j, r0, gate)
            store(2 * j, r0 // 2, lo)
            store(2 * j + 1, r0 // 2, hi)
            done.append(hi)


def _zero_after(x):
    return (pltpu.bitcast(x, U32) >> 16) >> 16


def _softmax_rows(sc, mask):
    sc = jnp.where(mask, sc, NEG)
    m = jnp.max(sc, axis=1, keepdims=True)
    p = jnp.exp(sc - m)
    l = jnp.sum(p, axis=1, keepdims=True)
    return p * (1.0 / l)


def _kernel(xa_hbm, mem0_ref, awq_hbm, awk_hbm, awv_hbm, awo_hbm,
            xb_hbm, c_hbm, bwq_hbm, bwuk_hbm, bwuv_hbm, bwo_hbm,
            out_hbm,
            xbt, xb, c, bwq_raw, bwuk_raw, bwuv_raw, bwot, bwq_d0, bwq_d1, wkv_d, q_all, kv, acct, s_buf0, s_buf1, p_buf0, p_buf1, ctx_last,
            xat, xa, a_raw, awot, aw_d, awo_d, mem, zq, zk, zv, oxe, oxo, obuf,
            sems, osems,
            *, S, DM, H, E, DC, M, SEG):
    HE = H * E
    NSEG = S // SEG
    scale = E ** -0.5
    s_buf = (s_buf0, s_buf1)
    p_buf = (p_buf0, p_buf1)
    bwq_d = (bwq_d0, bwq_d1)

    nsem = [0]

    def copy(src, dst):
        nsem[0] += 1
        return pltpu.make_async_copy(src, dst, sems.at[nsem[0] - 1])

    def slab(src, dst, part):
        nr = src.shape[0] // 2
        rows = pl.ds(part * nr, nr)
        return [copy(src.at[rows, pl.ds(i * 128, 128)], dst.at[i, rows]) for i in range(2)]

    def rows_half(src, dst, part):
        nr = src.shape[0] // 2
        return copy(src.at[pl.ds(part * nr, nr)], dst.at[pl.ds(part * nr, nr)])

    SP = 5
    cp_bwq0 = [copy(bwq_hbm.at[rows, pl.ds(0, 128)], bwq_raw.at[0, rows])
               for rows in (pl.ds(0, SP * 64 * H), pl.ds(SP * 64 * H, (DM - SP * 64) * H))]
    cp_bwq1 = copy(bwq_hbm.at[:, pl.ds(128, 128)], bwq_raw.at[1])
    cp_xb = [copy(xb_hbm.at[:, 0:512], xbt.at[:, 0:512]), copy(xb_hbm.at[:, 512:S], xbt.at[:, 512:S])]
    cp_c = copy(c_hbm, c)
    cp_xa = copy(xa_hbm, xat)
    cp_wkv = [slab(bwuk_hbm, bwuk_raw, p) + slab(bwuv_hbm, bwuv_raw, p) for p in range(2)]
    cp_late = [[rows_half(bwo_hbm, bwot, p), rows_half(awo_hbm, awot, p)]
               + slab(awq_hbm, a_raw.at[0], p) + slab(awk_hbm, a_raw.at[1], p) + slab(awv_hbm, a_raw.at[2], p)
               for p in range(2)]

    def start(cps):
        for cp in cps:
            cp.start()

    def wait(cps):
        for cp in cps:
            cp.wait()

    TQP = 512
    PADL = 512 - DM
    ZR = 512 // 16
    scale2 = scale * 1.4426950408889634

    def xb_t(i):
        cc = pl.ds(pl.multiple_of(i * 256, 256), 256)
        xb[cc, :] = xbt[:, cc].T

    def deint_bwq(src, half, t, nr, chain):
        r32 = bwq_raw.at[src].bitcast(U32).at[pl.ds(pl.multiple_of(t * nr * 8, 128), nr * 8)]
        dst = bwq_d[half].at[pl.ds(pl.multiple_of(t * (nr // 2), 8), nr // 2)]

        def store(hd, r, v):
            dst[r:r + 8, hd * 128:(hd + 1) * 128] = v

        _deint_block(r32, nr, store, chain)

    def q_step(half, t):
        i = lax.shift_right_logical(t, 1)
        n = lax.bitwise_and(t, 1)
        r0 = pl.multiple_of(i * TQP, TQP)
        c0 = pl.multiple_of(n * 1024, 1024)
        z = _dot(xb[pl.ds(r0, TQP), :], _bf(bwq_d[half][:, pl.ds(c0, 1024)])) * scale2
        z = _u32(z.astype(BF))
        rr = pl.ds(pl.multiple_of(i * (TQP // 2), TQP // 2), TQP // 2)
        for hh in range(8):
            q_all[n * 8 + hh, rr, half * 128:(half + 1) * 128] = z[:, hh * 128:(hh + 1) * 128]
        acct[pl.ds(pl.multiple_of((half * 8 + t) * ZR, ZR), ZR), :] = jnp.zeros((ZR, S), F32)

    def xb_t0(i, carry):
        xb_t(i)
        return carry

    def deint_bwq0(t, carry):
        @pl.when(t == SP)
        def _():
            cp_bwq0[1].wait()
            cp_xb[1].start()

        deint_bwq(0, 0, t, 64, 0)
        return carry

    start([cp_xb[0]] + cp_bwq0)
    cp_xb[0].wait()
    lax.fori_loop(0, 2, xb_t0, 0)
    cp_bwq0[0].wait()
    lax.fori_loop(0, DM // 64, deint_bwq0, 0)
    start([cp_bwq1] + cp_wkv[0])

    DCH = 1

    def deint_kv(t):
        for w_i, raw in enumerate((bwuk_raw, bwuv_raw)):
            for half in range(2):
                r32 = raw.at[half].bitcast(U32).at[pl.ds(pl.multiple_of(t * 1024, 1024), 1024)]
                dst = wkv_d.at[:, pl.ds(pl.multiple_of(t * 64, 64), 64)]

                def store(hd, r, v, c0=w_i * E + half * 128, dst=dst):
                    dst[hd, r:r + 8, c0:c0 + 128] = v

                _deint_block(r32, 128, store, DCH)

    W3, W4 = 4, 2

    def q_lo(t, carry):
        @pl.when(t == W3)
        def _():
            start(cp_wkv[1] + [cp_c])

        @pl.when(t == 1)
        def _():
            cp_xb[1].wait()

        @pl.when(t == 4)
        def _():
            cp_bwq1.wait()

        q_step(0, t)
        deint_bwq(lax.shift_right_logical(t, 2), 1, lax.bitwise_and(t, 3), DM // 4, DCH)
        j = jnp.minimum(lax.shift_right_logical(t + 1, 1), S // 512 - 1)
        xb_t(2 * j)
        xb_t(2 * j + 1)
        return carry

    def q_hi(t, carry):
        @pl.when(t == W4)
        def _():
            start([cp_xa] + cp_late[0])

        @pl.when(t == 4)
        def _():
            wait(cp_wkv[1])

        q_step(1, t)
        deint_kv(t)
        return carry

    lax.fori_loop(0, 8, q_lo, 0)
    wait(cp_wkv[0])
    lax.fori_loop(0, 8, q_hi, 0)
    cp_c.wait()

    TQ = 256
    NQ = S // TQ
    HQ = TQ // 2

    def kv_chunk(h, slot, r0, nr):
        z = _dot(c[pl.ds(r0, nr), :], _bf(wkv_d[h]))
        kv[slot, pl.ds(r0 // 2, nr // 2), :] = _u32(z.astype(BF))

    kv_chunk(0, 0, 0, TQ)
    wait([cp_xa] + cp_late[0])
    start(cp_late[1])

    RG = 8
    CHL = [4, 3, 2, 2, 2, 2, 2, 3]

    def attention(h, slot, filler, CHS):
        wot_h = bwot[pl.ds(pl.multiple_of(h * DM, DM), DM), :]
        row = lax.broadcasted_iota(jnp.int32, (TQ, HQ), 0)
        col = lax.broadcasted_iota(jnp.int32, (TQ, HQ), 1)
        tri_main = row >= col
        tri_tail = tri_main[0:HQ]
        blocks = list(range(NQ))

        def scores(idx):
            i, b = blocks[idx], idx % 2
            n = (i + 1) * TQ
            nm = n - HQ
            nf = n - TQ
            q = _bf(q_all[h, pl.ds(i * TQ // 2, TQ // 2), :])
            if nf > 0:
                s_buf[b][:, 0:nf] = _dot_nt(q, _bf(kv[slot, pl.ds(0, nf // 2), 0:E]))
            s_mid = _dot_nt(q, _bf(kv[slot, pl.ds(nf // 2, HQ // 2), 0:E]))
            s_buf[b][:, nf:nm] = jnp.where(tri_main, s_mid, NEG)
            s_tail = _dot_nt(q[HQ:TQ], _bf(kv[slot, pl.ds(nm // 2, HQ // 2), 0:E]))
            s_buf[b][HQ:TQ, nm:n] = jnp.where(tri_tail, s_tail, NEG)

        def softmax(idx):
            i, b, CH = blocks[idx], idx % 2, CHS[idx]
            n = (i + 1) * TQ
            nm = n - HQ
            ls = []
            sms = []
            for g in range(TQ // RG):
                ne = nm if g * RG < HQ else n
                rows = slice(g * RG, (g + 1) * RG)
                mx = s_buf[b][rows, 0:128]
                if g >= CH:
                    mx = pltpu.bitcast(_u32(mx) | _zero_after(sms[g - CH]), F32)
                for t in range(1, ne // 128):
                    mx = jnp.maximum(mx, s_buf[b][rows, t * 128:(t + 1) * 128])
                m = jnp.broadcast_to(jnp.max(mx, axis=1, keepdims=True), (RG, 128))
                sm = None
                for t0 in range(0, ne, 256):
                    pgs = []
                    for t in range(t0, min(t0 + 256, ne), 128):
                        pg = jnp.exp2(s_buf[b][rows, t:t + 128] - m)
                        sm = pg if sm is None else sm + pg
                        pgs.append(pg)
                    p_buf[b][rows, t0:t0 + 128 * len(pgs)] = jnp.concatenate(pgs, axis=1).astype(BF)
                sms.append(sm)
                ls.append(jnp.sum(sm, axis=1, keepdims=True))
            return jnp.concatenate(ls, axis=0)

        def context(idx, l):
            i, b = blocks[idx], idx % 2
            n = (i + 1) * TQ
            nm = n - HQ
            ctx = _dot(p_buf[b][:, 0:nm], _bf(kv[slot, pl.ds(0, nm // 2), E:2 * E]))
            ctx_t = _dot(p_buf[b][HQ:TQ, nm:n], _bf(kv[slot, pl.ds(nm // 2, HQ // 2), E:2 * E]))
            ctx = jnp.concatenate([ctx[0:HQ], ctx[HQ:TQ] + ctx_t], axis=0)
            return (ctx * (1.0 / l)).astype(BF)

        def out_proj(idx, ctx):
            acct[PADL:PADL + DM, pl.ds(blocks[idx] * TQ, TQ)] += _dot_nt(wot_h, ctx)

        scores(0)
        hp = jnp.maximum(h - 1, 0)
        acct[PADL:PADL + DM, pl.ds(S - TQ, TQ)] += _dot_nt(
            bwot[pl.ds(pl.multiple_of(hp * DM, DM), DM), :], ctx_last[...])
        ctx = None
        for idx in range(NQ):
            l = softmax(idx)
            filler(idx)
            if idx + 1 < NQ:
                scores(idx + 1)
            if ctx is not None:
                out_proj(idx - 1, ctx)
            ctx = context(idx, l)
        ctx_last[...] = ctx

    def deint_a(t):
        dst = aw_d.at[pl.ds(pl.multiple_of(t * 16, 16), 16)]
        for w_i in range(3):
            for half in range(2):
                r32 = a_raw.at[w_i, half].bitcast(U32).at[pl.ds(pl.multiple_of(t * 256, 256), 256)]

                def store(hd, r, v, c0=w_i * HE + half * 128):
                    dst[r:r + 8, c0 + hd * E:c0 + hd * E + 128] = v

                _deint_block(r32, 32, store, DCH)

    def prep_a(t):
        awo_d[pl.ds(pl.multiple_of(t * (E // 2), E // 2), E // 2), :] = _u32(
            awot[pl.ds(pl.multiple_of(t * DM, DM), DM), :].T)
        cc = pl.ds(pl.multiple_of(t * 128, 128), 128)
        xa[cc, :] = xat[:, cc].T

    def head(h, carry):
        slot = lax.bitwise_and(h, 1)
        hn = jnp.minimum(h + 1, H - 1)

        @pl.when(h == DM // 64)
        def _():
            wait(cp_late[1])

        def filler(idx):
            if idx < NQ - 1:
                kv_chunk(h, slot, (idx + 1) * TQ, TQ)
            else:
                kv_chunk(hn, 1 - slot, 0, TQ)
            if idx == 2:
                deint_a(jnp.minimum(h, DM // 32 - 1))
            if idx == 3:
                prep_a(h)

        attention(h, slot, filler, CHL)
        return carry

    ctx_last[...] = jnp.zeros(ctx_last.shape, BF)
    lax.fori_loop(0, H, head, 0)
    acct[PADL:PADL + DM, S - TQ:S] += _dot_nt(bwot[(H - 1) * DM:H * DM, :], ctx_last[...])

    L = 48
    LV = M + SEG
    PR = 2 * SEG
    XE = 40
    XO = PR - XE
    NP = NSEG // 2
    OC = 4
    NOC = NP // OC
    ORS = OC * PR

    zpad = jnp.zeros((2, L - LV, HE), BF)
    zq[:, LV:L, :] = zpad
    zk[:, LV:L, :] = zpad
    zv[:, LV:L, :] = zpad
    oxe[...] = jnp.zeros(oxe.shape, BF)
    mem[...] = mem0_ref[...].astype(F32)

    def out_copy(k):
        r = pl.ds(pl.multiple_of(k * ORS, ORS), ORS)
        return pltpu.make_async_copy(obuf.at[r, :], out_hbm.at[r, :], osems.at[k])

    def b_out(t):
        r = pl.ds(pl.multiple_of(lax.shift_right_logical(t, 1) * 128, 128), 128)
        f0 = pl.multiple_of(lax.bitwise_and(t, 1) * 256, 256)
        blk = acct[pl.ds(f0, 256), r].astype(BF)
        obuf[r, pl.ds(pl.multiple_of(DM - PADL + f0, 128), 256)] = blk.T

    def substep(odd, r0, ro, mask_m, mask_x, filler):
        cur = int(odd)
        nx = XO if odd else XE
        x0 = XE if odd else 0
        R = nx + M
        oxo_lhs = oxo if odd else oxe

        def scatter(dst, z):
            if odd:
                dst[1, XE - SEG:SEG, :] = z[0:XO].astype(BF)
            else:
                dst[0, 0:SEG, :] = z[0:SEG].astype(BF)
                dst[1, 0:XE - SEG, :] = z[SEG:XE].astype(BF)

        lhs = jnp.concatenate([xa[pl.ds(r0 + x0, nx), :].astype(F32), mem[...]], axis=0).astype(BF)
        zqk = _dot(lhs, _bf(aw_d[:, 0:2 * HE]))
        zqs = zqk[:, 0:HE] * scale
        scatter(zq, zqs)
        zq[cur, SEG:LV, :] = zqs[nx:R].astype(BF)
        scatter(zk, zqk[:, HE:2 * HE])
        zk[cur, SEG:LV, :] = zqk[nx:R, HE:2 * HE].astype(BF)
        sc = [_dot_nt(zq[cur, :, h * E:(h + 1) * E], zk[cur, :, h * E:(h + 1) * E]) for h in range(H)]
        zvv = _dot(lhs, _bf(aw_d[:, 2 * HE:3 * HE]))
        scatter(zv, zvv)
        zv[cur, SEG:LV, :] = zvv[nx:R].astype(BF)
        pm = _softmax_rows(jnp.concatenate([a[SEG:LV] for a in sc], axis=0), mask_m)
        px = _softmax_rows(jnp.concatenate([a[0:SEG] for a in sc], axis=0), mask_x).astype(BF)
        for h in range(H):
            oxo_lhs[nx:R, h * E:(h + 1) * E] = _dot(
                pm[h * M:(h + 1) * M].astype(BF), zv[cur, :, h * E:(h + 1) * E]).astype(BF)

        def x_pv(h):
            oh = _dot(px[h * SEG:(h + 1) * SEG], zv[cur, :, h * E:(h + 1) * E])
            cols = slice(h * E, (h + 1) * E)
            if odd:
                oxe[XE - SEG:XE, cols] = oh.astype(BF)
            else:
                oxo[0:XO, cols] = oh[0:XO].astype(BF)
                return oh[XO:SEG].astype(BF)

        filler()
        NE = 6 if odd else 3
        early = [x_pv(h) for h in range(NE)]
        o = _dot(oxo_lhs[...], _bf(awo_d[...]))
        obuf[pl.ds(ro, nx), 0:DM] = o[0:nx].astype(BF)
        mem[...] = o[nx:R]
        late = [x_pv(h) for h in range(NE, H)]
        if not odd:
            for h, v in enumerate(early + late):
                oxe[0:XE - SEG, h * E:(h + 1) * E] = v

    def pair(t, carry):
        colm = lax.broadcasted_iota(jnp.int32, (H * M, L), 1)
        mask_m = colm < LV
        rowx = lax.bitwise_and(lax.broadcasted_iota(jnp.int32, (H * SEG, L), 0), SEG - 1)
        colx = lax.broadcasted_iota(jnp.int32, (H * SEG, L), 1)
        mask_x = (colx < LV) & ((rowx >= colx) | (colx >= SEG))
        r0 = pl.multiple_of(t * PR, PR)
        re = pl.multiple_of(jnp.maximum(r0 - XE, XO), 8)
        substep(False, r0, re, mask_m, mask_x, lambda: b_out(t))
        substep(True, r0, r0, mask_m, mask_x, lambda: None)

        @pl.when(jnp.logical_and(lax.bitwise_and(t, OC - 1) == 0, t > 0))
        def _():
            out_copy(lax.shift_right_logical(t, 2) - 1).start()

        return carry

    lax.fori_loop(0, NP, pair, 0)
    TL = 48
    tail = [pltpu.make_async_copy(obuf.at[a:b, :], out_hbm.at[a:b, :], osems.at[k])
            for a, b, k in ((S - ORS, S - TL, NOC - 1), (S - TL, S, NOC))]
    tail[0].start()
    obuf[S - XE:S, 0:DM] = _dot(oxe[...], _bf(awo_d[...]))[0:XE].astype(BF)
    tail[1].start()
    for k in range(NOC - 1):
        out_copy(k).wait()
    wait(tail)


@functools.partial(jax.jit, static_argnames=("A_seg_len",))
def pallas_concat_heads__memory_aug_recurrent_mem_tr__compressed_kv_cla__prompt_kernel(
    A_x, A_mem0, A_Wq, A_Wk, A_Wv, A_Wo, A_seg_len,
    B_x, B_c_kv, B_w_q, B_w_uk, B_w_uv, B_w_o,
):
    _, S, DM = A_x.shape
    _, H, E = A_Wq.shape
    M = A_mem0.shape[1]
    DC = B_c_kv.shape[2]
    SEG = int(A_seg_len)
    assert (S, DM, H, E, M, DC, SEG) == (2048, 448, 16, 256, 8, 1024, 32)
    HE = H * E
    any_spec = pl.BlockSpec(memory_space=pl.ANY)
    vm = pltpu.VMEM
    scratch = [
        vm((DM, S), BF), vm((S, DM), BF), vm((S, DC), BF),
        vm((2, DM * H, 128), BF), vm((2, DC * H, 128), BF), vm((2, DC * H, 128), BF),
        vm((H * DM, E), BF),
        vm((DM // 2, HE // 2), U32), vm((DM // 2, HE // 2), U32),
        vm((H, DC // 2, 2 * E), U32),
        vm((H, S // 2, E), U32), vm((2, S // 2, 2 * E), U32),
        vm((512, S), F32),
        vm((256, S), F32), vm((256, S), F32), vm((256, S), BF), vm((256, S), BF), vm((256, E), BF),
        vm((DM, S), BF), vm((S, DM), BF),
        vm((3, 2, DM * H, 128), BF), vm((H * DM, E), BF),
        vm((DM // 2, 3 * HE), U32), vm((HE // 2, DM), U32),
        vm((M, DM), F32),
        vm((2, 48, HE), BF), vm((2, 48, HE), BF), vm((2, 48, HE), BF),
        vm((48, HE), BF), vm((32, HE), BF),
        vm((S, 2 * DM), BF),
        pltpu.SemaphoreType.DMA((31,)), pltpu.SemaphoreType.DMA((9,)),
    ]
    out = pl.pallas_call(
        functools.partial(_kernel, S=S, DM=DM, H=H, E=E, DC=DC, M=M, SEG=SEG),
        out_shape=jax.ShapeDtypeStruct((S, 2 * DM), BF),
        in_specs=[any_spec, pl.BlockSpec(memory_space=pltpu.VMEM)] + [any_spec] * 10,
        out_specs=any_spec,
        scratch_shapes=scratch,
        compiler_params=pltpu.CompilerParams(vmem_limit_bytes=126 * 1024 * 1024),
    )(
        jnp.swapaxes(A_x, 1, 2).reshape(DM, S), A_mem0.reshape(M, DM),
        A_Wq.reshape(DM * H, E), A_Wk.reshape(DM * H, E), A_Wv.reshape(DM * H, E),
        jnp.swapaxes(A_Wo, 1, 2).reshape(H * DM, E),
        jnp.swapaxes(B_x, 1, 2).reshape(DM, S), B_c_kv.reshape(S, DC),
        B_w_q.reshape(DM * H, E), B_w_uk.reshape(DC * H, E), B_w_uv.reshape(DC * H, E),
        jnp.swapaxes(B_w_o, 1, 2).reshape(H * DM, E),
    )
    return out.reshape(1, S, 2 * DM)
```

```python
import functools

import jax
import jax.numpy as jnp
from jax import lax
from jax.experimental import pallas as pl
from jax.experimental.pallas import tpu as pltpu

BF = jnp.bfloat16
F32 = jnp.float32
U32 = jnp.uint32
NT = (((1,), (1,)), ((), ()))
NEG = -1000000000.0


def _bf(x32):
    return pltpu.bitcast(x32, BF)


def _u32(xb):
    return pltpu.bitcast(xb, U32)


def _dot(a, b):
    return jnp.dot(a, b, preferred_element_type=F32)


def _dot_nt(a, b):
    return lax.dot_general(a, b, NT, preferred_element_type=F32)


def _deint(raw32, j, r0, gate=None):
    ev = raw32[pl.ds(r0 * 8 + j, 8, stride=16), :]
    od = raw32[pl.ds(r0 * 8 + j + 8, 8, stride=16), :]
    if gate is not None:
        ev = ev | gate
    lo = (ev & jnp.uint32(0xFFFF)) | (od << 16)
    hi = (ev >> 16) | (od & jnp.uint32(0xFFFF0000))
    return lo, hi


def _deint_block(raw32, nrows, store, chain):
    done = []
    for r0 in range(0, nrows, 16):
        for j in range(8):
            gate = _zero_after(done[-chain]) if 0 < chain <= len(done) else None
            lo, hi = _deint(raw32, j, r0, gate)
            store(2 * j, r0 // 2, lo)
            store(2 * j + 1, r0 // 2, hi)
            done.append(hi)


def _zero_after(x):
    return (pltpu.bitcast(x, U32) >> 16) >> 16


def _softmax_rows(sc, mask):
    sc = jnp.where(mask, sc, NEG)
    m = jnp.max(sc, axis=1, keepdims=True)
    p = jnp.exp(sc - m)
    l = jnp.sum(p, axis=1, keepdims=True)
    return p * (1.0 / l)


def _kernel(xa_hbm, mem0_ref, awq_hbm, awk_hbm, awv_hbm, awo_hbm,
            xb_hbm, c_hbm, bwq_hbm, bwuk_hbm, bwuv_hbm, bwo_hbm,
            out_hbm,
            xbt, xb, c, bwq_raw, bwuk_raw, bwuv_raw, bwot, bwq_d0, bwq_d1, wkv_d, q_all, kv, acct, s_buf0, s_buf1, p_buf0, p_buf1, ctx_last,
            xat, xa, a_raw, awot, aw_d, awo_d, mem, zq, zk, zv, oxe, oxo, obuf,
            sems, osems,
            *, S, DM, H, E, DC, M, SEG):
    HE = H * E
    NSEG = S // SEG
    scale = E ** -0.5
    s_buf = (s_buf0, s_buf1)
    p_buf = (p_buf0, p_buf1)
    bwq_d = (bwq_d0, bwq_d1)

    nsem = [0]

    def copy(src, dst):
        nsem[0] += 1
        return pltpu.make_async_copy(src, dst, sems.at[nsem[0] - 1])

    def slab(src, dst, part):
        nr = src.shape[0] // 2
        rows = pl.ds(part * nr, nr)
        return [copy(src.at[rows, pl.ds(i * 128, 128)], dst.at[i, rows]) for i in range(2)]

    def rows_half(src, dst, part):
        nr = src.shape[0] // 2
        return copy(src.at[pl.ds(part * nr, nr)], dst.at[pl.ds(part * nr, nr)])

    SP = 5
    cp_bwq0 = [copy(bwq_hbm.at[rows, pl.ds(0, 128)], bwq_raw.at[0, rows])
               for rows in (pl.ds(0, SP * 64 * H), pl.ds(SP * 64 * H, (DM - SP * 64) * H))]
    cp_bwq1 = copy(bwq_hbm.at[:, pl.ds(128, 128)], bwq_raw.at[1])
    cp_xb = [copy(xb_hbm.at[:, 0:512], xbt.at[:, 0:512]), copy(xb_hbm.at[:, 512:S], xbt.at[:, 512:S])]
    cp_c = copy(c_hbm, c)
    cp_xa = copy(xa_hbm, xat)
    cp_wkv = [slab(bwuk_hbm, bwuk_raw, p) + slab(bwuv_hbm, bwuv_raw, p) for p in range(2)]
    cp_late = [[rows_half(bwo_hbm, bwot, p), rows_half(awo_hbm, awot, p)]
               + slab(awq_hbm, a_raw.at[0], p) + slab(awk_hbm, a_raw.at[1], p) + slab(awv_hbm, a_raw.at[2], p)
               for p in range(2)]

    def start(cps):
        for cp in cps:
            cp.start()

    def wait(cps):
        for cp in cps:
            cp.wait()

    TQP = 512
    PADL = 512 - DM
    ZR = 512 // 16
    scale2 = scale * 1.4426950408889634

    def xb_t(i):
        cc = pl.ds(pl.multiple_of(i * 256, 256), 256)
        xb[cc, :] = xbt[:, cc].T

    def deint_bwq(src, half, t, nr, chain):
        r32 = bwq_raw.at[src].bitcast(U32).at[pl.ds(pl.multiple_of(t * nr * 8, 128), nr * 8)]
        dst = bwq_d[half].at[pl.ds(pl.multiple_of(t * (nr // 2), 8), nr // 2)]

        def store(hd, r, v):
            dst[r:r + 8, hd * 128:(hd + 1) * 128] = v

        _deint_block(r32, nr, store, chain)

    def q_step(half, t):
        i = lax.shift_right_logical(t, 1)
        n = lax.bitwise_and(t, 1)
        r0 = pl.multiple_of(i * TQP, TQP)
        c0 = pl.multiple_of(n * 1024, 1024)
        z = _dot(xb[pl.ds(r0, TQP), :], _bf(bwq_d[half][:, pl.ds(c0, 1024)])) * scale2
        z = _u32(z.astype(BF))
        rr = pl.ds(pl.multiple_of(i * (TQP // 2), TQP // 2), TQP // 2)
        for hh in range(8):
            q_all[n * 8 + hh, rr, half * 128:(half + 1) * 128] = z[:, hh * 128:(hh + 1) * 128]
        acct[pl.ds(pl.multiple_of((half * 8 + t) * ZR, ZR), ZR), :] = jnp.zeros((ZR, S), F32)

    def xb_t0(i, carry):
        xb_t(i)
        return carry

    def deint_bwq0(t, carry):
        @pl.when(t == SP)
        def _():
            cp_bwq0[1].wait()
            cp_xb[1].start()

        deint_bwq(0, 0, t, 64, 0)
        return carry

    start([cp_xb[0]] + cp_bwq0)
    cp_xb[0].wait()
    lax.fori_loop(0, 2, xb_t0, 0)
    cp_bwq0[0].wait()
    lax.fori_loop(0, DM // 64, deint_bwq0, 0)
    start([cp_bwq1] + cp_wkv[0])

    DCH = 1

    def deint_kv(t):
        for w_i, raw in enumerate((bwuk_raw, bwuv_raw)):
            for half in range(2):
                r32 = raw.at[half].bitcast(U32).at[pl.ds(pl.multiple_of(t * 1024, 1024), 1024)]
                dst = wkv_d.at[:, pl.ds(pl.multiple_of(t * 64, 64), 64)]

                def store(hd, r, v, c0=w_i * E + half * 128, dst=dst):
                    dst[hd, r:r + 8, c0:c0 + 128] = v

                _deint_block(r32, 128, store, DCH)

    W3, W4 = 4, 2

    def q_lo(t, carry):
        q_step(0, t)
        deint_bwq(lax.shift_right_logical(t, 2), 1, lax.bitwise_and(t, 3), DM // 4, DCH)
        j = jnp.minimum(lax.shift_right_logical(t + 1, 1), S // 512 - 1)
        xb_t(2 * j)
        xb_t(2 * j + 1)

        @pl.when(t == W3 - 1)
        def _():
            start(cp_wkv[1] + [cp_c])

        @pl.when(t == 0)
        def _():
            cp_xb[1].wait()

        @pl.when(t == 3)
        def _():
            cp_bwq1.wait()

        return carry

    def q_hi(t, carry):
        q_step(1, t)
        deint_kv(t)

        @pl.when(t == W4 - 1)
        def _():
            start([cp_xa] + cp_late[0])

        @pl.when(t == 3)
        def _():
            wait(cp_wkv[1])

        return carry

    lax.fori_loop(0, 8, q_lo, 0)
    wait(cp_wkv[0])
    lax.fori_loop(0, 8, q_hi, 0)
    cp_c.wait()

    TQ = 256
    NQ = S // TQ
    HQ = TQ // 2

    def kv_chunk(h, slot, r0, nr, c0=0, c1=2 * E):
        z = _dot(c[pl.ds(r0, nr), :], _bf(wkv_d[h, :, c0:c1]))
        kv[slot, pl.ds(r0 // 2, nr // 2), c0:c1] = _u32(z.astype(BF))

    kv_chunk(0, 0, 0, TQ)
    wait([cp_xa] + cp_late[0])
    start(cp_late[1])

    RG = 8
    CHL = [4, 3, 2, 2, 2, 2, 2, 3]

    def attention(h, slot, filler, CHS):
        wot_h = bwot[pl.ds(pl.multiple_of(h * DM, DM), DM), :]
        row = lax.broadcasted_iota(jnp.int32, (TQ, HQ), 0)
        col = lax.broadcasted_iota(jnp.int32, (TQ, HQ), 1)
        tri_main = row >= col
        tri_tail = tri_main[0:HQ]
        blocks = list(range(NQ))

        def scores(idx):
            i, b = blocks[idx], idx % 2
            n = (i + 1) * TQ
            nm = n - HQ
            nf = n - TQ
            q = _bf(q_all[h, pl.ds(i * TQ // 2, TQ // 2), :])
            if nf > 0:
                s_buf[b][:, 0:nf] = _dot_nt(q, _bf(kv[slot, pl.ds(0, nf // 2), 0:E]))
            s_mid = _dot_nt(q, _bf(kv[slot, pl.ds(nf // 2, HQ // 2), 0:E]))
            s_buf[b][:, nf:nm] = jnp.where(tri_main, s_mid, NEG)
            s_tail = _dot_nt(q[HQ:TQ], _bf(kv[slot, pl.ds(nm // 2, HQ // 2), 0:E]))
            s_buf[b][HQ:TQ, nm:n] = jnp.where(tri_tail, s_tail, NEG)

        def softmax(idx):
            i, b, CH = blocks[idx], idx % 2, CHS[idx]
            n = (i + 1) * TQ
            nm = n - HQ
            ls = []
            sms = []
            for g in range(TQ // RG):
                ne = nm if g * RG < HQ else n
                rows = slice(g * RG, (g + 1) * RG)
                mx = s_buf[b][rows, 0:128]
                if g >= CH:
                    mx = pltpu.bitcast(_u32(mx) | _zero_after(sms[g - CH]), F32)
                for t in range(1, ne // 128):
                    mx = jnp.maximum(mx, s_buf[b][rows, t * 128:(t + 1) * 128])
                m = jnp.broadcast_to(jnp.max(mx, axis=1, keepdims=True), (RG, 128))
                sm = None
                for t0 in range(0, ne, 256):
                    pgs = []
                    for t in range(t0, min(t0 + 256, ne), 128):
                        pg = jnp.exp2(s_buf[b][rows, t:t + 128] - m)
                        sm = pg if sm is None else sm + pg
                        pgs.append(pg)
                    p_buf[b][rows, t0:t0 + 128 * len(pgs)] = jnp.concatenate(pgs, axis=1).astype(BF)
                sms.append(sm)
                ls.append(jnp.sum(sm, axis=1, keepdims=True))
            return jnp.concatenate(ls, axis=0)

        def context(idx, l):
            i, b = blocks[idx], idx % 2
            n = (i + 1) * TQ
            nm = n - HQ
            ctx = _dot(p_buf[b][:, 0:nm], _bf(kv[slot, pl.ds(0, nm // 2), E:2 * E]))
            ctx_t = _dot(p_buf[b][HQ:TQ, nm:n], _bf(kv[slot, pl.ds(nm // 2, HQ // 2), E:2 * E]))
            ctx = jnp.concatenate([ctx[0:HQ], ctx[HQ:TQ] + ctx_t], axis=0)
            return (ctx * (1.0 / l)).astype(BF)

        def out_proj(idx, ctx):
            acct[PADL:PADL + DM, pl.ds(blocks[idx] * TQ, TQ)] += _dot_nt(wot_h, ctx)

        filler(-1)
        scores(0)
        hp = jnp.maximum(h - 1, 0)
        acct[PADL:PADL + DM, pl.ds(S - TQ, TQ)] += _dot_nt(
            bwot[pl.ds(pl.multiple_of(hp * DM, DM), DM), :], ctx_last[...])
        ctx = None
        for idx in range(NQ):
            l = softmax(idx)
            filler(idx)
            if idx + 1 < NQ:
                scores(idx + 1)
            if ctx is not None:
                out_proj(idx - 1, ctx)
            ctx = context(idx, l)
        ctx_last[...] = ctx

    def deint_a(t):
        dst = aw_d.at[pl.ds(pl.multiple_of(t * 16, 16), 16)]
        for w_i in range(3):
            for half in range(2):
                r32 = a_raw.at[w_i, half].bitcast(U32).at[pl.ds(pl.multiple_of(t * 256, 256), 256)]

                def store(hd, r, v, c0=w_i * HE + half * 128):
                    dst[r:r + 8, c0 + hd * E:c0 + hd * E + 128] = v

                _deint_block(r32, 32, store, DCH)

    def prep_a(t):
        awo_d[pl.ds(pl.multiple_of(t * (E // 2), E // 2), E // 2), :] = _u32(
            awot[pl.ds(pl.multiple_of(t * DM, DM), DM), :].T)
        cc = pl.ds(pl.multiple_of(t * 128, 128), 128)
        xa[cc, :] = xat[:, cc].T

    def head(h, carry):
        slot = lax.bitwise_and(h, 1)
        hn = jnp.minimum(h + 1, H - 1)

        def filler(idx):
            if idx < 0:
                kv_chunk(h, slot, TQ, TQ, 0, E)
            elif idx == 0:
                kv_chunk(h, slot, TQ, TQ, E, 2 * E)
            elif idx < NQ - 1:
                kv_chunk(h, slot, (idx + 1) * TQ, TQ)
            else:
                kv_chunk(hn, 1 - slot, 0, TQ)
            if idx == 2:
                deint_a(jnp.minimum(h, DM // 32 - 1))
            if idx == 3:
                prep_a(h)

        attention(h, slot, filler, CHL)
        return carry

    def head_group(g, carry):
        @pl.when(g == 1)
        def _():
            wait(cp_late[1])

        return lax.fori_loop(g * (DM // 64), DM // 64 + g * (H - DM // 64), head, carry)

    ctx_last[...] = jnp.zeros(ctx_last.shape, BF)
    lax.fori_loop(0, 2, head_group, 0)
    acct[PADL:PADL + DM, S - TQ:S] += _dot_nt(bwot[(H - 1) * DM:H * DM, :], ctx_last[...])

    L = 48
    LV = M + SEG
    PR = 2 * SEG
    XE = 40
    XO = PR - XE
    NP = NSEG // 2
    OC = 4
    NOC = NP // OC
    ORS = OC * PR

    zpad = jnp.zeros((2, L - LV, HE), BF)
    zq[:, LV:L, :] = zpad
    zk[:, LV:L, :] = zpad
    zv[:, LV:L, :] = zpad
    oxe[...] = jnp.zeros(oxe.shape, BF)
    oxo[...] = jnp.zeros(oxo.shape, BF)
    mem[...] = mem0_ref[...].astype(F32)

    OP = SEG

    def out_copy(k):
        r0 = pl.multiple_of(k * ORS, ORS)
        return pltpu.make_async_copy(obuf.at[pl.ds(pl.multiple_of(r0 + OP, OP), ORS), :],
                                     out_hbm.at[pl.ds(r0, ORS), :], osems.at[k])

    def b_out(t):
        r = pl.ds(pl.multiple_of(lax.shift_right_logical(t, 1) * 128, 128), 128)
        f0 = pl.multiple_of(lax.bitwise_and(t, 1) * 256, 256)
        blk = acct[pl.ds(f0, 256), r].astype(BF)
        ro = pl.ds(pl.multiple_of(lax.shift_right_logical(t, 1) * 128 + OP, OP), 128)
        obuf[ro, pl.ds(pl.multiple_of(DM - PADL + f0, 128), 256)] = blk.T

    def substep(odd, r0, ro, mask_m, mask_x, filler):
        cur = int(odd)
        nx = XO if odd else XE
        x0 = XE if odd else 0
        R = nx + M
        oxo_lhs = oxo if odd else oxe

        def scatter(dst, z):
            if odd:
                dst[1, XE - SEG:SEG, :] = z[0:XO].astype(BF)
            else:
                dst[0, 0:SEG, :] = z[0:SEG].astype(BF)
                dst[1, 0:XE - SEG, :] = z[SEG:XE].astype(BF)

        lhs = jnp.concatenate([xa[pl.ds(r0 + x0, nx), :].astype(F32), mem[...]], axis=0).astype(BF)
        zqk = _dot(lhs, _bf(aw_d[:, 0:2 * HE]))
        zqs = zqk[:, 0:HE] * scale
        scatter(zq, zqs)
        zq[cur, SEG:LV, :] = zqs[nx:R].astype(BF)
        scatter(zk, zqk[:, HE:2 * HE])
        zk[cur, SEG:LV, :] = zqk[nx:R, HE:2 * HE].astype(BF)
        sc = [_dot_nt(zq[cur, :, h * E:(h + 1) * E], zk[cur, :, h * E:(h + 1) * E]) for h in range(H)]
        zvv = _dot(lhs, _bf(aw_d[:, 2 * HE:3 * HE]))
        scatter(zv, zvv)
        zv[cur, SEG:LV, :] = zvv[nx:R].astype(BF)
        pm = _softmax_rows(jnp.concatenate([a[SEG:LV] for a in sc], axis=0), mask_m)
        px = _softmax_rows(jnp.concatenate([a[0:SEG] for a in sc], axis=0), mask_x).astype(BF)
        no = PR - nx
        def m_pv(h):
            oxo_lhs[no:no + M, h * E:(h + 1) * E] = _dot(
                pm[h * M:(h + 1) * M].astype(BF), zv[cur, :, h * E:(h + 1) * E]).astype(BF)

        NL = 2
        for h in range(H - NL):
            m_pv(h)

        def x_pv(h):
            oh = _dot(px[h * SEG:(h + 1) * SEG], zv[cur, :, h * E:(h + 1) * E])
            cols = slice(h * E, (h + 1) * E)
            if odd:
                oxe[0:XO, cols] = oh[0:XO].astype(BF)
                return oh[XO:SEG].astype(BF)
            else:
                oxo[XE - SEG:XE, cols] = oh.astype(BF)

        filler()
        NE = 4
        early = [x_pv(h) for h in range(NE)]
        for h in range(H - NL, H):
            m_pv(h)
        o = _dot(oxo_lhs[...], _bf(awo_d[...]))
        obuf[pl.ds(ro, no), 0:DM] = o[0:no].astype(BF)
        mem[...] = o[no:no + M]
        late = [x_pv(h) for h in range(NE, H)]
        if odd:
            for h, v in enumerate(early + late):
                oxo[0:XE - SEG, h * E:(h + 1) * E] = v

    def pair(t, carry):
        colm = lax.broadcasted_iota(jnp.int32, (H * M, L), 1)
        mask_m = colm < LV
        rowx = lax.bitwise_and(lax.broadcasted_iota(jnp.int32, (H * SEG, L), 0), SEG - 1)
        colx = lax.broadcasted_iota(jnp.int32, (H * SEG, L), 1)
        mask_x = (colx < LV) & ((rowx >= colx) | (colx >= SEG))
        r0 = pl.multiple_of(t * PR, PR)
        substep(False, r0, pl.multiple_of(r0 + OP - SEG, SEG), mask_m, mask_x, lambda: b_out(t))
        substep(True, r0, pl.multiple_of(r0 + OP - (XE - SEG), 8), mask_m, mask_x, lambda: None)

        @pl.when(jnp.logical_and(lax.bitwise_and(t, OC - 1) == 0, t > 0))
        def _():
            out_copy(lax.shift_right_logical(t, 2) - 1).start()

        return carry

    lax.fori_loop(0, NP, pair, 0)
    tail = [pltpu.make_async_copy(obuf.at[a + OP:b + OP, :], out_hbm.at[a:b, :], osems.at[k])
            for a, b, k in ((S - ORS, S - SEG, NOC - 1), (S - SEG, S, NOC))]
    tail[0].start()
    last = jnp.concatenate([oxe[0:XO, :].astype(F32), oxo[0:XE - SEG, :].astype(F32)], axis=0).astype(BF)
    obuf[S + OP - SEG:S + OP, 0:DM] = _dot(last, _bf(awo_d[...])).astype(BF)
    tail[1].start()
    for k in range(NOC - 1):
        out_copy(k).wait()
    wait(tail)


@functools.partial(jax.jit, static_argnames=("A_seg_len",))
def pallas_concat_heads__memory_aug_recurrent_mem_tr__compressed_kv_cla__prompt_kernel(
    A_x, A_mem0, A_Wq, A_Wk, A_Wv, A_Wo, A_seg_len,
    B_x, B_c_kv, B_w_q, B_w_uk, B_w_uv, B_w_o,
):
    _, S, DM = A_x.shape
    _, H, E = A_Wq.shape
    M = A_mem0.shape[1]
    DC = B_c_kv.shape[2]
    SEG = int(A_seg_len)
    assert (S, DM, H, E, M, DC, SEG) == (2048, 448, 16, 256, 8, 1024, 32)
    HE = H * E
    any_spec = pl.BlockSpec(memory_space=pl.ANY)
    vm = pltpu.VMEM
    scratch = [
        vm((DM, S), BF), vm((S, DM), BF), vm((S, DC), BF),
        vm((2, DM * H, 128), BF), vm((2, DC * H, 128), BF), vm((2, DC * H, 128), BF),
        vm((H * DM, E), BF),
        vm((DM // 2, HE // 2), U32), vm((DM // 2, HE // 2), U32),
        vm((H, DC // 2, 2 * E), U32),
        vm((H, S // 2, E), U32), vm((2, S // 2, 2 * E), U32),
        vm((512, S), F32),
        vm((256, S), F32), vm((256, S), F32), vm((256, S), BF), vm((256, S), BF), vm((256, E), BF),
        vm((DM, S), BF), vm((S, DM), BF),
        vm((3, 2, DM * H, 128), BF), vm((H * DM, E), BF),
        vm((DM // 2, 3 * HE), U32), vm((HE // 2, DM), U32),
        vm((M, DM), F32),
        vm((2, 48, HE), BF), vm((2, 48, HE), BF), vm((2, 48, HE), BF),
        vm((32, HE), BF), vm((48, HE), BF),
        vm((S + SEG, 2 * DM), BF),
        pltpu.SemaphoreType.DMA((31,)), pltpu.SemaphoreType.DMA((9,)),
    ]
    out = pl.pallas_call(
        functools.partial(_kernel, S=S, DM=DM, H=H, E=E, DC=DC, M=M, SEG=SEG),
        out_shape=jax.ShapeDtypeStruct((S, 2 * DM), BF),
        in_specs=[any_spec, pl.BlockSpec(memory_space=pltpu.VMEM)] + [any_spec] * 10,
        out_specs=any_spec,
        scratch_shapes=scratch,
        compiler_params=pltpu.CompilerParams(vmem_limit_bytes=126 * 1024 * 1024),
    )(
        jnp.swapaxes(A_x, 1, 2).reshape(DM, S), A_mem0.reshape(M, DM),
        A_Wq.reshape(DM * H, E), A_Wk.reshape(DM * H, E), A_Wv.reshape(DM * H, E),
        jnp.swapaxes(A_Wo, 1, 2).reshape(H * DM, E),
        jnp.swapaxes(B_x, 1, 2).reshape(DM, S), B_c_kv.reshape(S, DC),
        B_w_q.reshape(DM * H, E), B_w_uk.reshape(DC * H, E), B_w_uv.reshape(DC * H, E),
        jnp.swapaxes(B_w_o, 1, 2).reshape(H * DM, E),
    )
    return out.reshape(1, S, 2 * DM)
```

```python
import functools

import jax
import jax.numpy as jnp
from jax import lax
from jax.experimental import pallas as pl
from jax.experimental.pallas import tpu as pltpu

BF = jnp.bfloat16
F32 = jnp.float32
U32 = jnp.uint32
NT = (((1,), (1,)), ((), ()))
NEG = -1000000000.0


def _bf(x32):
    return pltpu.bitcast(x32, BF)


def _u32(xb):
    return pltpu.bitcast(xb, U32)


def _dot(a, b):
    return jnp.dot(a, b, preferred_element_type=F32)


def _dot_nt(a, b):
    return lax.dot_general(a, b, NT, preferred_element_type=F32)


def _deint(raw32, j, r0, gate=None):
    ev = raw32[pl.ds(r0 * 8 + j, 8, stride=16), :]
    od = raw32[pl.ds(r0 * 8 + j + 8, 8, stride=16), :]
    if gate is not None:
        ev = ev | gate
    lo = (ev & jnp.uint32(0xFFFF)) | (od << 16)
    hi = (ev >> 16) | (od & jnp.uint32(0xFFFF0000))
    return lo, hi


def _deint_block(raw32, nrows, store, chain, pairs=range(8)):
    done = []
    for r0 in range(0, nrows, 16):
        for j in pairs:
            gate = _zero_after(done[-chain]) if 0 < chain <= len(done) else None
            lo, hi = _deint(raw32, j, r0, gate)
            store(2 * j, r0 // 2, lo)
            store(2 * j + 1, r0 // 2, hi)
            done.append(hi)
    return done[-1]


def _zero_after(x):
    return (pltpu.bitcast(x, U32) >> 16) >> 16


def _softmax_rows(sc, mask):
    sc = jnp.where(mask, sc, NEG)
    m = jnp.max(sc, axis=1, keepdims=True)
    p = jnp.exp(sc - m)
    l = jnp.sum(p, axis=1, keepdims=True)
    return p * (1.0 / l)


def _kernel(xa_hbm, mem0_ref, awq_hbm, awk_hbm, awv_hbm, awo_hbm,
            xb_hbm, c_hbm, bwq_hbm, bwuk_hbm, bwuv_hbm, bwo_hbm,
            out_hbm,
            xbt, xb, c, bwq_raw, bwuk_raw, bwuv_raw, bwot, bwq_d0, bwq_d1, wkv_d, q_all, kv, acct, s_buf0, s_buf1, p_buf0, p_buf1,
            xat, xa, a_raw, awot, awv_d, aw_d, wu, mem, zq, zk, ua, obuf,
            sems,
            *, S, DM, H, E, DC, M, SEG):
    HE = H * E
    NSEG = S // SEG
    scale = E ** -0.5
    s_buf = (s_buf0, s_buf1)
    p_buf = (p_buf0, p_buf1)
    bwq_d = (bwq_d0, bwq_d1)

    def copy(src, dst, sem):
        return pltpu.make_async_copy(src, dst, sems.at[sem])

    def lanes(src, dst, rows, sem, halves=(0, 1)):
        return [copy(src.at[rows, pl.ds(i * 128, 128)], dst.at[i, rows], sem) for i in halves]

    SP = 5
    HG = 2
    a_v, a_q, a_k = (a_raw.at[pl.ds(2 * w, 2)] for w in range(3))
    all_d = pl.ds(0, DM * H)
    cp_bwq0 = (lanes(bwq_hbm, bwq_raw, pl.ds(0, SP * 64 * H), 0, (0,))
               + lanes(bwq_hbm, bwq_raw, pl.ds(SP * 64 * H, (DM - SP * 64) * H), 1, (0,)))
    cp_bwq1 = lanes(bwq_hbm, bwq_raw, all_d, 2, (1,))[0]
    cp_xb = [copy(xb_hbm.at[:, 0:512], xbt.at[:, 0:512], 3), copy(xb_hbm.at[:, 512:S], xbt.at[:, 512:S], 4)]
    cp_c = copy(c_hbm, c, 5)
    cp_wkv = [lanes(bwuk_hbm, bwuk_raw, pl.ds(p * DC * H // 2, DC * H // 2), 6 + p)
              + lanes(bwuv_hbm, bwuv_raw, pl.ds(p * DC * H // 2, DC * H // 2), 6 + p)
              + lanes(awv_hbm, a_v, all_d, 6 + p, (p,)) for p in range(2)]
    cp_late = []
    for p in range(2):
        part = lambda n, tot: pl.ds(n, tot - n) if p else pl.ds(0, n)
        xc, wr = part(HG * 128, S), part(HG * DM, H * DM)
        cp_late.append([copy(xa_hbm.at[:, xc], xat.at[:, xc], 8 + p), copy(bwo_hbm.at[wr], bwot.at[wr], 8 + p),
                        copy(awo_hbm.at[wr], awot.at[wr], 8 + p)]
                       + lanes(awq_hbm, a_q, part(HG * DM * H // 4, DM * H), 8 + p, (0,)))
    cp_late[1] += lanes(awq_hbm, a_q, all_d, 9, (1,)) + lanes(awk_hbm, a_k, all_d, 9)

    def start(cps):
        for cp in cps:
            cp.start()

    def wait(cps):
        for cp in cps:
            cp.wait()

    TQP = 512
    PADL = 512 - DM
    ZR = 512 // 16
    scale2 = scale * 1.4426950408889634

    def xb_t(i):
        cc = pl.ds(pl.multiple_of(i * 256, 256), 256)
        xb[cc, :] = xbt[:, cc].T

    def deint_bwq(src, half, t, nr, chain):
        r32 = bwq_raw.at[src].bitcast(U32).at[pl.ds(pl.multiple_of(t * nr * 8, 128), nr * 8)]
        dst = bwq_d[half].at[pl.ds(pl.multiple_of(t * (nr // 2), 8), nr // 2)]

        def store(hd, r, v):
            dst[r:r + 8, hd * 128:(hd + 1) * 128] = v

        _deint_block(r32, nr, store, chain)

    def q_step(half, t):
        i = lax.shift_right_logical(t, 1)
        n = lax.bitwise_and(t, 1)
        r0 = pl.multiple_of(i * TQP, TQP)
        c0 = pl.multiple_of(n * 1024, 1024)
        z = _dot(xb[pl.ds(r0, TQP), :], _bf(bwq_d[half][:, pl.ds(c0, 1024)])) * scale2
        z = _u32(z.astype(BF))
        rr = pl.ds(pl.multiple_of(i * (TQP // 2), TQP // 2), TQP // 2)
        for hh in range(8):
            q_all[n * 8 + hh, rr, half * 128:(half + 1) * 128] = z[:, hh * 128:(hh + 1) * 128]
        acct[pl.ds(pl.multiple_of((half * 8 + t) * ZR, ZR), ZR), :] = jnp.zeros((ZR, S + 128), F32)

    def xb_t0(i, carry):
        xb_t(i)
        return carry

    def deint_bwq0(t, carry):
        @pl.when(t == SP)
        def _():
            cp_bwq0[1].wait()
            cp_xb[1].start()

        deint_bwq(0, 0, t, 64, 0)
        return carry

    start([cp_xb[0]] + cp_bwq0)
    cp_xb[0].wait()
    lax.fori_loop(0, 2, xb_t0, 0)
    cp_bwq0[0].wait()
    lax.fori_loop(0, DM // 64, deint_bwq0, 0)
    start([cp_bwq1] + cp_wkv[0])

    DCH = 1

    def deint_kv(t):
        for w_i, raw in enumerate((bwuk_raw, bwuv_raw)):
            for half in range(2):
                r32 = raw.at[half].bitcast(U32).at[pl.ds(pl.multiple_of(t * 1024, 1024), 1024)]
                dst = wkv_d.at[:, pl.ds(pl.multiple_of(t * 64, 64), 64)]

                def store(hd, r, v, c0=w_i * E + half * 128, dst=dst):
                    dst[hd, r:r + 8, c0:c0 + 128] = v

                _deint_block(r32, 128, store, DCH)

    W3, W4 = 4, 2

    QR = DM // 4

    def deint_a(w0, u, dst_ref):
        sl = lax.shift_right_logical(u, 2)
        dq = lax.bitwise_and(u, 3)
        outs = []
        for jq in range(2):
            r32 = a_raw.at[2 * w0 + sl].bitcast(U32).at[pl.ds(pl.multiple_of(dq * (QR * 8), 8), QR * 8)]
            dst = dst_ref.at[pl.ds(sl * H, H), pl.ds(pl.multiple_of(dq * (QR // 2), 8), QR // 2)]

            def store(hd, r, v, dst=dst):
                dst[hd, r:r + 8, :] = v

            outs.append(_deint_block(r32, QR, store, DCH, range(4 * jq, 4 * jq + 4)))
        return outs

    def q_lo(t, carry):
        q_step(0, t)
        deint_bwq(lax.shift_right_logical(t, 2), 1, lax.bitwise_and(t, 3), DM // 4, DCH)
        j = jnp.minimum(lax.shift_right_logical(t + 1, 1), S // 512 - 1)
        xb_t(2 * j)
        xb_t(2 * j + 1)

        @pl.when(t == W3 - 1)
        def _():
            start(cp_wkv[1] + [cp_c])

        @pl.when(t == 0)
        def _():
            cp_xb[1].wait()

        @pl.when(t == 3)
        def _():
            cp_bwq1.wait()

        return carry

    def q_hi(t, carry):
        q_step(1, t)
        deint_kv(t)
        deint_a(0, t, awv_d)

        @pl.when(t == W4 - 1)
        def _():
            start(cp_late[0])

        @pl.when(t == 3)
        def _():
            wait(cp_wkv[1])

        return carry

    lax.fori_loop(0, 8, q_lo, 0)
    wait(cp_wkv[0])
    lax.fori_loop(0, 8, q_hi, 0)
    cp_c.wait()

    TQ = 256
    NQ = S // TQ
    HQ = TQ // 2

    def kv_chunk(h, slot, r0, nr, c0=0, c1=2 * E):
        z = _dot(c[pl.ds(r0, nr), :], _bf(wkv_d[h, :, c0:c1]))
        kv[slot, pl.ds(r0 // 2, nr // 2), c0:c1] = _u32(z.astype(BF))

    MAINC = DM // 128 * 128

    def prep_a(t):
        wv = _bf(jnp.concatenate([awv_d[t], awv_d[H + t]], axis=1))
        r0 = pl.multiple_of(t * DM, DM)
        wo = jnp.concatenate([awot[pl.ds(r0, DM), :],
                              awot[pl.ds(pl.multiple_of(r0 + MAINC, 64), DM - MAINC), :]], axis=0)
        z = _u32(_dot_nt(wv, wo).astype(BF))
        odd = lax.bitwise_and(t, 1)
        t0 = lax.shift_right_logical(t, 1) * 7
        for n in range(3):
            wu[t0 + 4 * odd + n] = z[:, n * 128:(n + 1) * 128]
        own = lax.shift_right_logical(lax.broadcasted_iota(jnp.int32, (DM // 2, 128), 1), 6) == odd
        wu[t0 + 3] = jnp.where(own, z[:, MAINC:MAINC + 128], wu[t0 + 3])

    def xa_t(t):
        cc = pl.ds(pl.multiple_of(t * 128, 128), 128)
        v = xat[:, cc].T
        xa[cc, :] = v
        return _u32(v[112:128, 256:384])

    kv_chunk(0, 0, 0, TQ)
    wait(cp_late[0])
    start(cp_late[1])

    RG = 8
    CHL = [4, 3, 2, 2, 2, 2, 2, 2]

    ND = 4

    gates = {}

    def attention(h, slot, filler, CHS):
        wot_h = bwot[pl.ds(pl.multiple_of(h * DM, DM), DM), :]
        row = lax.broadcasted_iota(jnp.int32, (TQ, HQ), 0)
        col = lax.broadcasted_iota(jnp.int32, (TQ, HQ), 1)
        tri_main = row >= col
        tri_tail = tri_main[0:HQ]
        blocks = list(range(NQ))

        def scores(idx):
            i, b = blocks[idx], idx % 2
            n = (i + 1) * TQ
            nm = n - HQ
            nf = n - TQ
            q = _bf(q_all[h, pl.ds(i * TQ // 2, TQ // 2), :])
            if nf > 0:
                s_buf[b][:, 0:nf] = _dot_nt(q, _bf(kv[slot, pl.ds(0, nf // 2), 0:E]))
            s_mid = _dot_nt(q, _bf(kv[slot, pl.ds(nf // 2, HQ // 2), 0:E]))
            s_buf[b][:, nf:nm] = jnp.where(tri_main, s_mid, NEG)
            s_tail = _dot_nt(q[HQ:TQ], _bf(kv[slot, pl.ds(nm // 2, HQ // 2), 0:E]))
            s_buf[b][HQ:TQ, nm:n] = jnp.where(tri_tail, s_tail, NEG)

        def softmax(idx):
            i, b, CH = blocks[idx], idx % 2, CHS[idx]
            n = (i + 1) * TQ
            nm = n - HQ
            ls = []
            sms = []
            for g in range(TQ // RG):
                ne = nm if g * RG < HQ else n
                rows = slice(g * RG, (g + 1) * RG)
                mx = s_buf[b][rows, 0:128]
                if g == 0:
                    for v in gates.pop(idx, []):
                        mx = pltpu.bitcast(_u32(mx) | _zero_after(v), F32)
                if g >= CH:
                    mx = pltpu.bitcast(_u32(mx) | _zero_after(sms[g - CH]), F32)
                for t in range(1, ne // 128):
                    mx = jnp.maximum(mx, s_buf[b][rows, t * 128:(t + 1) * 128])
                m = jnp.broadcast_to(jnp.max(mx, axis=1, keepdims=True), (RG, 128))
                sm = None
                for t0 in range(0, ne, 256):
                    pgs = []
                    for t in range(t0, min(t0 + 256, ne), 128):
                        pg = jnp.exp2(s_buf[b][rows, t:t + 128] - m)
                        sm = pg if sm is None else sm + pg
                        pgs.append(pg)
                    p_buf[b][rows, t0:t0 + 128 * len(pgs)] = jnp.concatenate(pgs, axis=1).astype(BF)
                sms.append(sm)
                ls.append(jnp.sum(sm, axis=1, keepdims=True))
            return jnp.concatenate(ls, axis=0)

        def context(idx, l):
            i, b = blocks[idx], idx % 2
            n = (i + 1) * TQ
            nm = n - HQ
            ctx = _dot(p_buf[b][:, 0:nm], _bf(kv[slot, pl.ds(0, nm // 2), E:2 * E]))
            ctx_t = _dot(p_buf[b][HQ:TQ, nm:n], _bf(kv[slot, pl.ds(nm // 2, HQ // 2), E:2 * E]))
            ctx = jnp.concatenate([ctx[0:HQ], ctx[HQ:TQ] + ctx_t], axis=0)
            return (ctx * (1.0 / l)).astype(BF)

        def out_proj(idx, ctx):
            acct[PADL:PADL + DM, pl.ds(blocks[idx] * TQ, TQ)] += _dot_nt(wot_h, ctx)

        filler(-1)
        scores(0)
        ctx = None
        for idx in range(NQ):
            l = softmax(idx)
            filler(idx)
            if idx + 1 < NQ:
                scores(idx + 1)
            if ctx is not None:
                out_proj(idx - 1, ctx)
            ctx = context(idx, l)
            if idx >= NQ - ND:
                q_all[h, pl.ds(idx * TQ // 2, TQ // 2), :] = _u32(ctx)
                ctx = None

    def head(h, carry):
        slot = lax.bitwise_and(h, 1)
        hn = jnp.minimum(h + 1, H - 1)

        def filler(idx):
            if idx < 0:
                kv_chunk(h, slot, TQ, TQ, 0, E)
            elif idx == 0:
                kv_chunk(h, slot, TQ, TQ, E, 2 * E)
            elif idx < NQ - 1:
                kv_chunk(h, slot, (idx + 1) * TQ, TQ)
            else:
                kv_chunk(hn, 1 - slot, 0, TQ)
            if idx < 0:
                gates[2] = deint_a(1, h, aw_d)
                gates[6] = [xa_t(h)]
            if idx == NQ - 1:
                prep_a(h)

        attention(h, slot, filler, CHL)
        return carry

    def head_group(g, carry):
        @pl.when(g == 1)
        def _():
            wait(cp_late[1])

        return lax.fori_loop(g * HG, HG + g * (H - HG), head, carry)

    lax.fori_loop(0, 2, head_group, 0)

    NPRE = 8

    def b_piece(p):
        al = (lambda v, m: v) if isinstance(p, int) else pl.multiple_of
        hh = p & (H - 1)
        q0 = S - ND * TQ + (p >> 4) * 128
        qr = q0 if isinstance(p, int) else jnp.minimum(q0, S - 128)
        ctx = _bf(q_all[hh, pl.ds(al(qr >> 1, 64), 64), :])
        for m0 in range(0, DM, DM // 2):
            acct[PADL + m0:PADL + m0 + DM // 2, pl.ds(al(q0, 128), 128)] += _dot_nt(
                bwot[pl.ds(al(hh * DM + m0, DM // 2), DM // 2), :], ctx)

    for p in range(NPRE):
        b_piece(p)

    L = 48
    LV = M + SEG
    PR = 2 * SEG
    XE = 40
    XO = PR - XE
    NP = NSEG // 2
    OC = 2
    NOC = NP // OC
    ORS = OC * PR
    NT_ = (H + 2) // 3

    zpad = jnp.zeros((2, L - LV, HE), BF)
    zq[:, LV:L, :] = zpad
    zk[:, LV:L, :] = zpad
    for T in range(NT_):
        r = T * 128 + LV * min(3, H - 3 * T)
        ua[:, r:r + 8, :] = jnp.zeros((2, 8, 512), BF)
    mem[...] = mem0_ref[...].astype(F32)

    def out_copy(k):
        r = pl.ds(pl.multiple_of(k * ORS, ORS), ORS)
        return pltpu.make_async_copy(obuf.at[r, :], out_hbm.at[r, :], sems.at[10])

    def b_out(t):
        r = pl.ds(pl.multiple_of(lax.shift_right_logical(t, 1) * 128, 128), 128)
        f0 = pl.multiple_of(lax.bitwise_and(t, 1) * 256, 256)
        blk = acct[pl.ds(f0, 256), r].astype(BF)
        obuf[r, pl.ds(pl.multiple_of(DM - PADL + f0, 128), 256)] = blk.T

    def substep(odd, seg, r0, mask, filler, last):
        cur = int(odd)
        nx = XO if odd else XE
        x0 = XE if odd else 0
        R = nx + M

        def scatter(dst, z, base=0, cols=slice(None)):
            if odd:
                dst[1, base + XE - SEG:base + SEG, cols] = z[0:XO].astype(BF)
            else:
                dst[0, base:base + SEG, cols] = z[0:SEG].astype(BF)
                dst[1, base:base + XE - SEG, cols] = z[SEG:XE].astype(BF)
            dst[cur, base + SEG:base + LV, cols] = z[nx:R].astype(BF)

        lhs = jnp.concatenate([xa[pl.ds(r0 + x0, nx), :].astype(F32), mem[...]], axis=0).astype(BF)
        wqk = jnp.concatenate([aw_d[(2 * w + i) * H + h] for w in range(2) for h in range(H) for i in range(2)], axis=1)
        zqk = _dot(lhs, _bf(wqk))
        scatter(zq, zqk[:, 0:HE] * scale)
        scatter(zk, zqk[:, HE:2 * HE])
        sc = [_dot_nt(zq[cur, :, h * E:(h + 1) * E], zk[cur, :, h * E:(h + 1) * E]) for h in range(H)]
        zu = _dot(lhs, _bf(jnp.concatenate([wu[n] for n in range(H // 2 * 7)], axis=1)))
        lane_hi = lax.broadcasted_iota(jnp.int32, (R, 128), 1) >= 64
        for h in range(H):
            base = h // 3 * 128 + h % 3 * LV
            c0 = (h // 2 * 7 + h % 2 * 4) * 128
            ct = (h // 2 * 7 + 3) * 128
            scatter(ua, zu[:, c0:c0 + MAINC], base, slice(0, MAINC))
            zt = zu[:, ct:ct + 128]
            scatter(ua, jnp.where(lane_hi, zt, 0.0) if h % 2 else jnp.where(lane_hi, 0.0, zt), base, slice(MAINC, 512))
        p = _softmax_rows(jnp.concatenate([a[0:LV] for a in sc], axis=0), mask)
        pts = [jnp.concatenate([p[h * LV:(h + 1) * LV, 0:LV] for h in range(3 * T, 3 * T + 3)]
                               + [jnp.zeros((LV, 128 - 3 * LV), F32)], axis=1).astype(BF)
               for T in range(NT_ - 1)] + [p[(H - 1) * LV:H * LV].astype(BF)]
        filler()
        b_piece(2 * seg + NPRE)
        a = functools.reduce(lambda x, y: x + y, [
            _dot(pt, ua[cur, T * 128:T * 128 + pt.shape[1], :]) for T, pt in enumerate(pts)])
        tail, main = a[:, MAINC:512], a[:, 0:MAINC]
        o = jnp.concatenate([main, tail[:, 0:64] + tail[:, 64:128]], axis=1)
        mem[...] = o[SEG:LV]
        last()
        obuf[pl.ds(pl.multiple_of(r0 + cur * SEG, SEG), SEG), 0:DM] = o[0:SEG].astype(BF)
        b_piece(2 * seg + NPRE + 1)

    def pair(t, carry):
        row = lax.broadcasted_iota(jnp.int32, (LV, L), 0)
        col = lax.broadcasted_iota(jnp.int32, (LV, L), 1)
        lim = jnp.concatenate([jnp.where(row < SEG, row, SEG) - col] * H, axis=0)
        col = jnp.concatenate([col] * H, axis=0)
        mask = (col < LV) & ((lim >= 0) | (col >= SEG))
        r0 = pl.multiple_of(t * PR, PR)

        def flush():
            @pl.when(jnp.logical_and(lax.bitwise_and(t, OC - 1) == 0, t > 0))
            def _():
                out_copy(lax.shift_right_logical(t, 1) - 1).start()

        substep(False, 2 * t, r0, mask, lambda: b_out(t), lambda: None)
        substep(True, 2 * t + 1, r0, mask, lambda: None, flush)
        return carry

    lax.fori_loop(0, NP, pair, 0)
    out_copy(NOC - 1).start()
    for k in range(NOC):
        out_copy(k).wait()


@functools.partial(jax.jit, static_argnames=("A_seg_len",))
def pallas_concat_heads__memory_aug_recurrent_mem_tr__compressed_kv_cla__prompt_kernel(
    A_x, A_mem0, A_Wq, A_Wk, A_Wv, A_Wo, A_seg_len,
    B_x, B_c_kv, B_w_q, B_w_uk, B_w_uv, B_w_o,
):
    _, S, DM = A_x.shape
    _, H, E = A_Wq.shape
    M = A_mem0.shape[1]
    DC = B_c_kv.shape[2]
    SEG = int(A_seg_len)
    assert (S, DM, H, E, M, DC, SEG) == (2048, 448, 16, 256, 8, 1024, 32)
    HE = H * E
    any_spec = pl.BlockSpec(memory_space=pl.ANY)
    vm = pltpu.VMEM
    scratch = [
        vm((DM, S), BF), vm((S, DM), BF), vm((S, DC), BF),
        vm((2, DM * H, 128), BF), vm((2, DC * H, 128), BF), vm((2, DC * H, 128), BF),
        vm((H * DM, E), BF),
        vm((DM // 2, HE // 2), U32), vm((DM // 2, HE // 2), U32),
        vm((H, DC // 2, 2 * E), U32),
        vm((H, S // 2, E), U32), vm((2, S // 2, 2 * E), U32),
        vm((512, S + 128), F32),
        vm((256, S), F32), vm((256, S), F32), vm((256, S), BF), vm((256, S), BF),
        vm((DM, S), BF), vm((S, DM), BF),
        vm((6, DM * H, 128), BF), vm((H * DM, E), BF),
        vm((2 * H, DM // 2, 128), U32), vm((4 * H, DM // 2, 128), U32), vm((H // 2 * 7, DM // 2, 128), U32),
        vm((M, DM), F32),
        vm((2, 48, HE), BF), vm((2, 48, HE), BF), vm((2, 688, 512), BF),
        vm((S, 2 * DM), BF),
        pltpu.SemaphoreType.DMA((11,)),
    ]
    out = pl.pallas_call(
        functools.partial(_kernel, S=S, DM=DM, H=H, E=E, DC=DC, M=M, SEG=SEG),
        out_shape=jax.ShapeDtypeStruct((S, 2 * DM), BF),
        in_specs=[any_spec, pl.BlockSpec(memory_space=pltpu.VMEM)] + [any_spec] * 10,
        out_specs=any_spec,
        scratch_shapes=scratch,
        compiler_params=pltpu.CompilerParams(vmem_limit_bytes=126 * 1024 * 1024),
    )(
        jnp.swapaxes(A_x, 1, 2).reshape(DM, S), A_mem0.reshape(M, DM),
        A_Wq.reshape(DM * H, E), A_Wk.reshape(DM * H, E), A_Wv.reshape(DM * H, E),
        jnp.swapaxes(A_Wo, 1, 2).reshape(H * DM, E),
        jnp.swapaxes(B_x, 1, 2).reshape(DM, S), B_c_kv.reshape(S, DC),
        B_w_q.reshape(DM * H, E), B_w_uk.reshape(DC * H, E), B_w_uv.reshape(DC * H, E),
        jnp.swapaxes(B_w_o, 1, 2).reshape(H * DM, E),
    )
    return out.reshape(1, S, 2 * DM)
```

```python
import functools

import jax
import jax.numpy as jnp
from jax import lax
from jax.experimental import pallas as pl
from jax.experimental.pallas import tpu as pltpu

BF = jnp.bfloat16
F32 = jnp.float32
U32 = jnp.uint32
NT = (((1,), (1,)), ((), ()))
NEG = -1000000000.0


def _bf(x32):
    return pltpu.bitcast(x32, BF)


def _u32(xb):
    return pltpu.bitcast(xb, U32)


def _dot(a, b):
    return jnp.dot(a, b, preferred_element_type=F32)


def _dot_nt(a, b):
    return lax.dot_general(a, b, NT, preferred_element_type=F32)


def _deint(raw32, j, r0, gate=None):
    ev = raw32[pl.ds(r0 * 8 + j, 8, stride=16), :]
    od = raw32[pl.ds(r0 * 8 + j + 8, 8, stride=16), :]
    if gate is not None:
        ev = ev | gate
    lo = (ev & jnp.uint32(0xFFFF)) | (od << 16)
    hi = (ev >> 16) | (od & jnp.uint32(0xFFFF0000))
    return lo, hi


def _deint_block(raw32, nrows, store, chain, pairs=range(8)):
    done = []
    for r0 in range(0, nrows, 16):
        for j in pairs:
            gate = _zero_after(done[-chain]) if 0 < chain <= len(done) else None
            lo, hi = _deint(raw32, j, r0, gate)
            store(2 * j, r0 // 2, lo)
            store(2 * j + 1, r0 // 2, hi)
            done.append(hi)
    return done[-1]


def _zero_after(x):
    return (pltpu.bitcast(x, U32) >> 16) >> 16


def _softmax_rows(sc, mask):
    sc = jnp.where(mask, sc, NEG)
    m = jnp.max(sc, axis=1, keepdims=True)
    p = jnp.exp(sc - m)
    l = jnp.sum(p, axis=1, keepdims=True)
    return p * (1.0 / l)


def _kernel(xa_hbm, mem0_ref, awq_hbm, awk_hbm, awv_hbm, awo_hbm,
            xb_hbm, c_hbm, bwq_hbm, bwuk_hbm, bwuv_hbm, bwo_hbm,
            out_hbm,
            xbt, xb, c, bwuk_raw, bwuv_raw, bwot, bwq_d0, bwq_d1, wkv_d, q_all, kv, acct, s_buf0, s_buf1, p_buf0, p_buf1,
            xa, a_raw, wab, wu, mem, ya, ua, obuf,
            sems,
            *, S, DM, H, E, DC, M, SEG):
    HE = H * E
    NSEG = S // SEG
    scale = E ** -0.5
    s_buf = (s_buf0, s_buf1)
    p_buf = (p_buf0, p_buf1)
    bwq_d = (bwq_d0, bwq_d1)

    def copy(src, dst, sem):
        return pltpu.make_async_copy(src, dst, sems.at[sem])

    def lanes(src, dst, rows, sem, halves=(0, 1)):
        return [copy(src.at[rows, pl.ds(i * 128, 128)], dst.at[i, rows], sem) for i in halves]

    SP = 5
    HG = 2
    a_v, a_q, a_k = (a_raw.at[pl.ds(2 * w, 2)] for w in range(3))
    bwq_raw, xat = a_q, xbt
    all_d = pl.ds(0, DM * H)
    cp_bwq0 = (lanes(bwq_hbm, bwq_raw, pl.ds(0, SP * 64 * H), 0, (0,))
               + lanes(bwq_hbm, bwq_raw, pl.ds(SP * 64 * H, (DM - SP * 64) * H), 1, (0,)))
    cp_bwq1 = lanes(bwq_hbm, bwq_raw, all_d, 2, (1,))[0]
    cp_xb = [copy(xb_hbm.at[:, 0:512], xbt.at[:, 0:512], 3), copy(xb_hbm.at[:, 512:S], xbt.at[:, 512:S], 4)]
    cp_c = copy(c_hbm, c, 5)
    cp_wkv = [lanes(bwuk_hbm, bwuk_raw, pl.ds(p * DC * H // 2, DC * H // 2), 6 + p)
              + lanes(bwuv_hbm, bwuv_raw, pl.ds(p * DC * H // 2, DC * H // 2), 6 + p)
              + lanes(awv_hbm, a_v, all_d, 6 + p, (p,)) for p in range(2)]
    cp_late = []
    for p in range(2):
        part = lambda n, tot: pl.ds(n, tot - n) if p else pl.ds(0, n)
        xc, wr = part(HG * 128, S), part(HG * DM, H * DM)
        cp_late.append([copy(xa_hbm.at[:, xc], xat.at[:, xc], 8 + p), copy(bwo_hbm.at[wr], bwot.at[wr], 8 + p)]
                       + lanes(awo_hbm, wab.at[pl.ds(6, 2)], part(2 * HG * DM, H * DM), 8 + p)
                       + lanes(awq_hbm, a_q, all_d, 8 + p, (p,)))
    cp_late[1] += lanes(awk_hbm, a_k, all_d, 9)
    wab32 = wab.bitcast(U32)

    def start(cps):
        for cp in cps:
            cp.start()

    def wait(cps):
        for cp in cps:
            cp.wait()

    TQP = 512
    PADL = 512 - DM
    ZR = 512 // 16
    scale2 = scale * 1.4426950408889634

    def xb_t(i):
        cc = pl.ds(pl.multiple_of(i * 256, 256), 256)
        xb[cc, :] = xbt[:, cc].T

    def deint_bwq(src, half, t, nr, chain):
        r32 = a_raw.at[2 + src].bitcast(U32).at[pl.ds(pl.multiple_of(t * nr * 8, 128), nr * 8)]
        dst = bwq_d[half].at[pl.ds(pl.multiple_of(t * (nr // 2), 8), nr // 2)]

        def store(hd, r, v):
            dst[r:r + 8, hd * 128:(hd + 1) * 128] = v

        _deint_block(r32, nr, store, chain)

    def q_step(half, t):
        i = lax.shift_right_logical(t, 1)
        n = lax.bitwise_and(t, 1)
        r0 = pl.multiple_of(i * TQP, TQP)
        c0 = pl.multiple_of(n * 1024, 1024)
        z = _dot(xb[pl.ds(r0, TQP), :], _bf(bwq_d[half][:, pl.ds(c0, 1024)])) * scale2
        z = _u32(z.astype(BF))
        rr = pl.ds(pl.multiple_of(i * (TQP // 2), TQP // 2), TQP // 2)
        for hh in range(8):
            q_all[n * 8 + hh, rr, half * 128:(half + 1) * 128] = z[:, hh * 128:(hh + 1) * 128]
        acct[pl.ds(pl.multiple_of((half * 8 + t) * ZR, ZR), ZR), :] = jnp.zeros((ZR, S + 128), F32)

    def xb_t0(i, carry):
        xb_t(i)
        return carry

    def deint_bwq0(t, carry):
        @pl.when(t == SP)
        def _():
            cp_bwq0[1].wait()
            cp_xb[1].start()

        deint_bwq(0, 0, t, 64, 0)
        return carry

    start([cp_xb[0]] + cp_bwq0)
    cp_xb[0].wait()
    lax.fori_loop(0, 2, xb_t0, 0)
    cp_bwq0[0].wait()
    lax.fori_loop(0, DM // 64, deint_bwq0, 0)
    start([cp_bwq1] + cp_wkv[0])

    DCH = 1

    def deint_kv(t):
        for w_i, raw in enumerate((bwuk_raw, bwuv_raw)):
            for half in range(2):
                r32 = raw.at[half].bitcast(U32).at[pl.ds(pl.multiple_of(t * 1024, 1024), 1024)]
                dst = wkv_d.at[:, pl.ds(pl.multiple_of(t * 64, 64), 64)]

                def store(hd, r, v, c0=w_i * E + half * 128, dst=dst):
                    dst[hd, r:r + 8, c0:c0 + 128] = v

                _deint_block(r32, 128, store, DCH)

    W3 = 4

    QR = DM // 4

    def deint_a(u, nch=2):
        sl = lax.shift_right_logical(u, 2)
        dq = lax.bitwise_and(u, 3)
        r32 = a_raw.at[sl].bitcast(U32).at[pl.ds(pl.multiple_of(dq * (QR * 8), 8), QR * 8)]
        dst = wab32.at[sl].at[pl.ds(pl.multiple_of(dq * (QR // 2), 8), DM * H // 2 - 3 * QR // 2)]

        def store(hd, r, v):
            dst[hd * (DM // 2) + r:hd * (DM // 2) + r + 8, :] = v

        return [_deint_block(r32, QR, store, DCH, range(8 // nch * jq, 8 // nch * (jq + 1))) for jq in range(nch)]

    def q_lo(t, carry):
        q_step(0, t)
        deint_bwq(lax.shift_right_logical(t, 2), 1, lax.bitwise_and(t, 3), DM // 4, DCH)
        j = jnp.minimum(lax.shift_right_logical(t + 1, 1), S // 512 - 1)
        xb_t(2 * j)
        xb_t(2 * j + 1)

        @pl.when(t == W3 - 1)
        def _():
            start(cp_wkv[1] + [cp_c])

        @pl.when(t == 0)
        def _():
            cp_xb[1].wait()

        @pl.when(t == 3)
        def _():
            cp_bwq1.wait()

        return carry

    def q_hi(t, carry):
        q_step(1, t)
        deint_kv(t)
        deint_a(t)

        return carry

    def q_hi_group(g, carry):
        @pl.when(g == 1)
        def _():
            wait(cp_wkv[1])
            start(cp_late[0])

        return lax.fori_loop(4 * g, 4 * g + 4, q_hi, carry)

    lax.fori_loop(0, 8, q_lo, 0)
    wait(cp_wkv[0])
    lax.fori_loop(0, 2, q_hi_group, 0)
    cp_c.wait()

    TQ = 256
    NQ = S // TQ
    HQ = TQ // 2

    def kv_chunk(h, slot, r0, nr, c0=0, c1=2 * E):
        z = _dot(c[pl.ds(r0, nr), :], _bf(wkv_d[h, :, c0:c1]))
        kv[slot, pl.ds(r0 // 2, nr // 2), c0:c1] = _u32(z.astype(BF))

    MAINC = DM // 128 * 128

    def prep_a(p):
        w = lax.shift_right_logical(p, 4)
        r0 = pl.multiple_of(lax.bitwise_and(p, H - 1) * (DM // 2), DM // 2)
        rt = pl.ds(pl.multiple_of(r0 + MAINC // 2, 32), (DM - MAINC) // 2)
        lhs = jnp.concatenate([wab32[2 * w + i, pl.ds(r0, DM // 2), :] for i in range(2)], axis=1)
        rhs = jnp.concatenate([jnp.concatenate([wab32[6 - 2 * w + i, pl.ds(r0, DM // 2), :],
                                                wab32[6 - 2 * w + i, rt, :]], axis=0) for i in range(2)], axis=1)
        z = _dot_nt(_bf(lhs), _bf(rhs)) * jnp.where(w == 1, scale, 1.0)
        z = _u32(z.astype(BF))
        odd = lax.bitwise_and(p, 1)
        t0 = lax.shift_right_logical(p, 1) * 7
        for n in range(3):
            wu[t0 + 4 * odd + n] = z[:, n * 128:(n + 1) * 128]
        own = lax.shift_right_logical(lax.broadcasted_iota(jnp.int32, (DM // 2, 128), 1), 6) == odd
        wu[t0 + 3] = jnp.where(own, z[:, MAINC:MAINC + 128], wu[t0 + 3])

    def xa_t(t):
        cc = pl.ds(pl.multiple_of(t * 128, 128), 128)
        v = xat[:, cc].T
        xa[cc, :] = v
        return _u32(v[112:128, 256:384])

    kv_chunk(0, 0, 0, TQ)
    wait(cp_late[0])
    start(cp_late[1])

    RG = 8
    CHL = [4, 3, 2, 2, 2, 2, 2, 2]

    ND = 4

    gates = {}

    def attention(h, slot, filler, CHS):
        wot_h = bwot[pl.ds(pl.multiple_of(h * DM, DM), DM), :]
        row = lax.broadcasted_iota(jnp.int32, (TQ, HQ), 0)
        col = lax.broadcasted_iota(jnp.int32, (TQ, HQ), 1)
        tri_main = row >= col
        tri_tail = tri_main[0:HQ]
        blocks = list(range(NQ))

        def scores(idx):
            i, b = blocks[idx], idx % 2
            n = (i + 1) * TQ
            nm = n - HQ
            nf = n - TQ
            q = _bf(q_all[h, pl.ds(i * TQ // 2, TQ // 2), :])
            if nf > 0:
                s_buf[b][:, 0:nf] = _dot_nt(q, _bf(kv[slot, pl.ds(0, nf // 2), 0:E]))
            s_mid = _dot_nt(q, _bf(kv[slot, pl.ds(nf // 2, HQ // 2), 0:E]))
            s_buf[b][:, nf:nm] = jnp.where(tri_main, s_mid, NEG)
            s_tail = _dot_nt(q[HQ:TQ], _bf(kv[slot, pl.ds(nm // 2, HQ // 2), 0:E]))
            s_buf[b][HQ:TQ, nm:n] = jnp.where(tri_tail, s_tail, NEG)

        def softmax(idx):
            i, b, CH = blocks[idx], idx % 2, CHS[idx]
            n = (i + 1) * TQ
            nm = n - HQ
            ls = []
            sms = []
            for g in range(TQ // RG):
                ne = nm if g * RG < HQ else n
                rows = slice(g * RG, (g + 1) * RG)
                mx = s_buf[b][rows, 0:128]
                if g == 0:
                    for v in gates.pop(idx, []):
                        mx = pltpu.bitcast(_u32(mx) | _zero_after(v), F32)
                if g >= CH:
                    mx = pltpu.bitcast(_u32(mx) | _zero_after(sms[g - CH]), F32)
                for t in range(1, ne // 128):
                    mx = jnp.maximum(mx, s_buf[b][rows, t * 128:(t + 1) * 128])
                m = jnp.broadcast_to(jnp.max(mx, axis=1, keepdims=True), (RG, 128))
                sm = None
                for t0 in range(0, ne, 256):
                    pgs = []
                    for t in range(t0, min(t0 + 256, ne), 128):
                        pg = jnp.exp2(s_buf[b][rows, t:t + 128] - m)
                        sm = pg if sm is None else sm + pg
                        pgs.append(pg)
                    p_buf[b][rows, t0:t0 + 128 * len(pgs)] = jnp.concatenate(pgs, axis=1).astype(BF)
                sms.append(sm)
                ls.append(jnp.sum(sm, axis=1, keepdims=True))
            return jnp.concatenate(ls, axis=0)

        def context(idx, l):
            i, b = blocks[idx], idx % 2
            n = (i + 1) * TQ
            nm = n - HQ
            ctx = _dot(p_buf[b][:, 0:nm], _bf(kv[slot, pl.ds(0, nm // 2), E:2 * E]))
            ctx_t = _dot(p_buf[b][HQ:TQ, nm:n], _bf(kv[slot, pl.ds(nm // 2, HQ // 2), E:2 * E]))
            ctx = jnp.concatenate([ctx[0:HQ], ctx[HQ:TQ] + ctx_t], axis=0)
            return (ctx * (1.0 / l)).astype(BF)

        def out_proj(idx, ctx):
            acct[PADL:PADL + DM, pl.ds(blocks[idx] * TQ, TQ)] += _dot_nt(wot_h, ctx)

        filler(-1)
        scores(0)
        ctx = None
        for idx in range(NQ):
            l = softmax(idx)
            filler(idx)
            if idx + 1 < NQ:
                scores(idx + 1)
            if ctx is not None:
                out_proj(idx - 1, ctx)
            ctx = context(idx, l)
            if idx >= NQ - ND:
                q_all[h, pl.ds(idx * TQ // 2, TQ // 2), :] = _u32(ctx)
                ctx = None

    def head(h, carry):
        slot = lax.bitwise_and(h, 1)
        hn = jnp.minimum(h + 1, H - 1)

        def filler(idx):
            if idx < 0:
                kv_chunk(h, slot, TQ, TQ, 0, E)
            elif idx == 0:
                kv_chunk(h, slot, TQ, TQ, E, 2 * E)
            elif idx < NQ - 1:
                kv_chunk(h, slot, (idx + 1) * TQ, TQ)
            else:
                kv_chunk(hn, 1 - slot, 0, TQ)
            if idx < 0:
                u0 = 8 + 2 * jnp.minimum(h, 7)
                gates[2] = deint_a(u0, 1)
                gates[4] = deint_a(u0 + 1, 1)
                gates[6] = [xa_t(h)]
            if idx == NQ - 1:
                prep_a(2 * h + 1)
            if idx == NQ - 2:
                prep_a(2 * h)

        attention(h, slot, filler, CHL)
        return carry

    def head_group(g, carry):
        @pl.when(g == 1)
        def _():
            wait(cp_late[1])

        return lax.fori_loop(g * HG, HG + g * (H - HG), head, carry)

    lax.fori_loop(0, 2, head_group, 0)

    NPRE = 8

    def b_piece(p):
        al = (lambda v, m: v) if isinstance(p, int) else pl.multiple_of
        hh = p & (H - 1)
        q0 = S - ND * TQ + (p >> 4) * 128
        qr = q0 if isinstance(p, int) else jnp.minimum(q0, S - 128)
        ctx = _bf(q_all[hh, pl.ds(al(qr >> 1, 64), 64), :])
        for m0 in range(0, DM, DM // 2):
            acct[PADL + m0:PADL + m0 + DM // 2, pl.ds(al(q0, 128), 128)] += _dot_nt(
                bwot[pl.ds(al(hh * DM + m0, DM // 2), DM // 2), :], ctx)

    for p in range(NPRE):
        b_piece(p)

    L = 48
    LV = M + SEG
    PR = 2 * SEG
    XE = 40
    XO = PR - XE
    NP = NSEG // 2
    OC = 2
    NOC = NP // OC
    ORS = OC * PR
    NT_ = (H + 2) // 3

    for T in range(NT_):
        r = T * 128 + LV * min(3, H - 3 * T)
        ua[:, r:r + 8, :] = jnp.zeros((2, 8, 512), BF)
        ya[:, r:r + 8, :] = jnp.zeros((2, 8, 512), BF)
    mem[...] = mem0_ref[...].astype(F32)

    def out_copy(k):
        r = pl.ds(pl.multiple_of(k * ORS, ORS), ORS)
        return pltpu.make_async_copy(obuf.at[r, :], out_hbm.at[r, :], sems.at[10])

    def b_out(t):
        r = pl.ds(pl.multiple_of(lax.shift_right_logical(t, 1) * 128, 128), 128)
        f0 = pl.multiple_of(lax.bitwise_and(t, 1) * 256, 256)
        blk = acct[pl.ds(f0, 256), r].astype(BF)
        obuf[r, pl.ds(pl.multiple_of(DM - PADL + f0, 128), 256)] = blk.T

    def substep(odd, seg, r0, mask, filler, last):
        cur = int(odd)
        nx = XO if odd else XE
        x0 = XE if odd else 0
        R = nx + M

        def scatter(dst, z, base=0, cols=slice(None)):
            if odd:
                dst[1, base + XE - SEG:base + SEG, cols] = z[0:XO].astype(BF)
            else:
                dst[0, base:base + SEG, cols] = z[0:SEG].astype(BF)
                dst[1, base:base + XE - SEG, cols] = z[SEG:XE].astype(BF)
            dst[cur, base + SEG:base + LV, cols] = z[nx:R].astype(BF)

        lane_hi = lax.broadcasted_iota(jnp.int32, (R, 128), 1) >= 64

        def project(dst, n0):
            z = _dot(lhs, _bf(jnp.concatenate([wu[n0 + n] for n in range(H // 2 * 7)], axis=1)))
            for h in range(H):
                base = h // 3 * 128 + h % 3 * LV
                c0 = (h // 2 * 7 + h % 2 * 4) * 128
                zt = z[:, (h // 2 * 7 + 3) * 128:(h // 2 * 7 + 4) * 128]
                scatter(dst, z[:, c0:c0 + MAINC], base, slice(0, MAINC))
                scatter(dst, jnp.where(lane_hi, zt, 0.0) if h % 2 else jnp.where(lane_hi, 0.0, zt),
                        base, slice(MAINC, 512))

        memv = mem[...]
        lhs = jnp.concatenate([xa[pl.ds(r0 + x0, nx), :].astype(F32), memv], axis=0).astype(BF)
        hk = jnp.concatenate([xa[pl.ds(pl.multiple_of(r0 + cur * SEG, SEG), SEG), :].astype(F32), memv,
                              jnp.zeros((L - LV, DM), F32)], axis=0)
        hk = jnp.concatenate([hk, hk[:, MAINC:DM]], axis=1).astype(BF)
        project(ya, H // 2 * 7)
        st = [_dot_nt(hk, ya[cur, T * 128:min(T * 128 + 128, ya.shape[1]), :]) for T in range(NT_)]
        project(ua, 0)
        pts = []
        for T in range(NT_):
            w = st[T].shape[1]
            sc = jnp.where(mask[:, 0:w], st[T], NEG)
            e = jnp.exp(sc - jnp.max(sc, axis=0, keepdims=True))
            e = e * (1.0 / jnp.sum(e, axis=0, keepdims=True))
            if w < 128:
                e = jnp.concatenate([e, jnp.zeros((L, 128 - w), F32)], axis=1)
            pt = jnp.concatenate([e, jnp.zeros((128 - L, 128), F32)], axis=0).T
            if w < 128:
                pts.append(pt[0:LV, 0:L].astype(BF))
            else:
                pts.append(jnp.concatenate([pt[r * LV:(r + 1) * LV, 0:LV] for r in range(3)]
                                           + [jnp.zeros((LV, 128 - 3 * LV), F32)], axis=1).astype(BF))
        filler()
        b_piece(2 * seg + NPRE)
        a = functools.reduce(lambda x, y: x + y, [
            _dot(pt, ua[cur, T * 128:T * 128 + pt.shape[1], :]) for T, pt in enumerate(pts)])
        tail, main = a[:, MAINC:512], a[:, 0:MAINC]
        o = jnp.concatenate([main, tail[:, 0:64] + tail[:, 64:128]], axis=1)
        mem[...] = o[SEG:LV]
        last()
        obuf[pl.ds(pl.multiple_of(r0 + cur * SEG, SEG), SEG), 0:DM] = o[0:SEG].astype(BF)
        b_piece(2 * seg + NPRE + 1)

    def pair(t, carry):
        key = lax.broadcasted_iota(jnp.int32, (L, 128), 0)
        lane = lax.broadcasted_iota(jnp.int32, (L, 128), 1)
        qry = lane - jnp.where(lane >= 2 * LV, 2 * LV, jnp.where(lane >= LV, LV, 0))
        mask = (key < LV) & ((qry >= SEG) | (key >= SEG) | (key <= qry))
        r0 = pl.multiple_of(t * PR, PR)

        def flush():
            @pl.when(jnp.logical_and(lax.bitwise_and(t, OC - 1) == 0, t > 0))
            def _():
                out_copy(lax.shift_right_logical(t, 1) - 1).start()

        substep(False, 2 * t, r0, mask, lambda: b_out(t), lambda: None)
        substep(True, 2 * t + 1, r0, mask, lambda: None, flush)
        return carry

    lax.fori_loop(0, NP, pair, 0)
    out_copy(NOC - 1).start()
    for k in range(NOC):
        out_copy(k).wait()


@functools.partial(jax.jit, static_argnames=("A_seg_len",))
def pallas_concat_heads__memory_aug_recurrent_mem_tr__compressed_kv_cla__prompt_kernel(
    A_x, A_mem0, A_Wq, A_Wk, A_Wv, A_Wo, A_seg_len,
    B_x, B_c_kv, B_w_q, B_w_uk, B_w_uv, B_w_o,
):
    _, S, DM = A_x.shape
    _, H, E = A_Wq.shape
    M = A_mem0.shape[1]
    DC = B_c_kv.shape[2]
    SEG = int(A_seg_len)
    assert (S, DM, H, E, M, DC, SEG) == (2048, 448, 16, 256, 8, 1024, 32)
    HE = H * E
    any_spec = pl.BlockSpec(memory_space=pl.ANY)
    vm = pltpu.VMEM
    scratch = [
        vm((DM, S), BF), vm((S, DM), BF), vm((S, DC), BF),
        vm((2, DC * H, 128), BF), vm((2, DC * H, 128), BF),
        vm((H * DM, E), BF),
        vm((DM // 2, HE // 2), U32), vm((DM // 2, HE // 2), U32),
        vm((H, DC // 2, 2 * E), U32),
        vm((H, S // 2, E), U32), vm((2, S // 2, 2 * E), U32),
        vm((512, S + 128), F32),
        vm((256, S), F32), vm((256, S), F32), vm((256, S), BF), vm((256, S), BF),
        vm((S, DM), BF),
        vm((6, DM * H, 128), BF), vm((8, DM * H, 128), BF),
        vm((H * 7, DM // 2, 128), U32),
        vm((M, DM), F32),
        vm((2, 688, 512), BF), vm((2, 688, 512), BF),
        vm((S, 2 * DM), BF),
        pltpu.SemaphoreType.DMA((11,)),
    ]
    out = pl.pallas_call(
        functools.partial(_kernel, S=S, DM=DM, H=H, E=E, DC=DC, M=M, SEG=SEG),
        out_shape=jax.ShapeDtypeStruct((S, 2 * DM), BF),
        in_specs=[any_spec, pl.BlockSpec(memory_space=pltpu.VMEM)] + [any_spec] * 10,
        out_specs=any_spec,
        scratch_shapes=scratch,
        compiler_params=pltpu.CompilerParams(vmem_limit_bytes=126 * 1024 * 1024),
    )(
        jnp.swapaxes(A_x, 1, 2).reshape(DM, S), A_mem0.reshape(M, DM),
        A_Wq.reshape(DM * H, E), A_Wk.reshape(DM * H, E), A_Wv.reshape(DM * H, E),
        jnp.swapaxes(A_Wo, 1, 2).reshape(H * DM, E),
        jnp.swapaxes(B_x, 1, 2).reshape(DM, S), B_c_kv.reshape(S, DC),
        B_w_q.reshape(DM * H, E), B_w_uk.reshape(DC * H, E), B_w_uv.reshape(DC * H, E),
        jnp.swapaxes(B_w_o, 1, 2).reshape(H * DM, E),
    )
    return out.reshape(1, S, 2 * DM)
```

```python
import functools

import jax
import jax.numpy as jnp
from jax import lax
from jax.experimental import pallas as pl
from jax.experimental.pallas import tpu as pltpu

BF = jnp.bfloat16
F32 = jnp.float32
U32 = jnp.uint32
NT = (((1,), (1,)), ((), ()))
NEG = -1000000000.0


def _bf(x32):
    return pltpu.bitcast(x32, BF)


def _u32(xb):
    return pltpu.bitcast(xb, U32)


def _dot(a, b):
    return jnp.dot(a, b, preferred_element_type=F32)


def _dot_nt(a, b):
    return lax.dot_general(a, b, NT, preferred_element_type=F32)


def _deint(raw32, j, r0, gate=None):
    ev = raw32[pl.ds(r0 * 8 + j, 8, stride=16), :]
    od = raw32[pl.ds(r0 * 8 + j + 8, 8, stride=16), :]
    if gate is not None:
        ev = ev | gate
    lo = (ev & jnp.uint32(0xFFFF)) | (od << 16)
    hi = (ev >> 16) | (od & jnp.uint32(0xFFFF0000))
    return lo, hi


def _deint_block(raw32, nrows, store, chain, pairs=range(8)):
    done = []
    for r0 in range(0, nrows, 16):
        for j in pairs:
            gate = _zero_after(done[-chain]) if 0 < chain <= len(done) else None
            lo, hi = _deint(raw32, j, r0, gate)
            store(2 * j, r0 // 2, lo)
            store(2 * j + 1, r0 // 2, hi)
            done.append(hi)
    return done[-1]


def _zero_after(x):
    return (pltpu.bitcast(x, U32) >> 16) >> 16


def _kernel(xa_hbm, mem0_ref, awq_hbm, awk_hbm, awv_hbm, awo_hbm,
            xb_hbm, c_hbm, bwq_hbm, bwuk_hbm, bwuv_hbm, bwo_hbm,
            out_hbm,
            xbt, xb, c, bwuk_raw, bwuv_raw, bwot, bwq_d0, bwq_d1, wkv_d, q_all, kv, acct, s_buf0, s_buf1, p_buf0, p_buf1,
            xa, a_raw, wab, wu, mem, ya, ua, obuf,
            sems,
            *, S, DM, H, E, DC, M, SEG):
    NSEG = S // SEG
    scale = E ** -0.5
    s_buf = (s_buf0, s_buf1)
    p_buf = (p_buf0, p_buf1)
    bwq_d = (bwq_d0, bwq_d1)

    def copy(src, dst, sem):
        return pltpu.make_async_copy(src, dst, sems.at[sem])

    def lanes(src, dst, rows, sem, halves=(0, 1)):
        return [copy(src.at[rows, pl.ds(i * 128, 128)], dst.at[i, rows], sem) for i in halves]

    SP = 5
    HG = 2
    a_v, a_q, a_k = (a_raw.at[pl.ds(2 * w, 2)] for w in range(3))
    bwq_raw, xat = a_q, xbt
    all_d = pl.ds(0, DM * H)
    cp_bwq0 = (lanes(bwq_hbm, bwq_raw, pl.ds(0, SP * 64 * H), 0, (0,))
               + lanes(bwq_hbm, bwq_raw, pl.ds(SP * 64 * H, (DM - SP * 64) * H), 1, (0,)))
    cp_bwq1 = lanes(bwq_hbm, bwq_raw, all_d, 2, (1,))[0]
    cp_xb = [copy(xb_hbm.at[:, 0:512], xbt.at[:, 0:512], 3), copy(xb_hbm.at[:, 512:S], xbt.at[:, 512:S], 4)]
    cp_c = copy(c_hbm, c, 5)
    cp_wkv = [lanes(bwuk_hbm, bwuk_raw, pl.ds(p * DC * H // 2, DC * H // 2), 6 + p)
              + lanes(bwuv_hbm, bwuv_raw, pl.ds(p * DC * H // 2, DC * H // 2), 6 + p)
              + lanes(awv_hbm, a_v, all_d, 6 + p, (p,)) for p in range(2)]
    cp_late = []
    for p in range(2):
        part = lambda n, tot: pl.ds(n, tot - n) if p else pl.ds(0, n)
        xc, wr = part(HG * 128, S), part(HG * DM, H * DM)
        cp_late.append([copy(xa_hbm.at[:, xc], xat.at[:, xc], 8 + p), copy(bwo_hbm.at[wr], bwot.at[wr], 8 + p)]
                       + lanes(awo_hbm, wab.at[pl.ds(6, 2)], part(2 * HG * DM, H * DM), 8 + p)
                       + lanes(awq_hbm, a_q, all_d, 8 + p, (p,)))
    cp_late[1] += lanes(awk_hbm, a_k, all_d, 9)
    wab32 = wab.bitcast(U32)

    def start(cps):
        for cp in cps:
            cp.start()

    def wait(cps):
        for cp in cps:
            cp.wait()

    TQP = 512
    PADL = 512 - DM
    ZR = 512 // 16
    scale2 = scale * 1.4426950408889634

    def xb_t(i):
        cc = pl.ds(pl.multiple_of(i * 256, 256), 256)
        xb[cc, :] = xbt[:, cc].T

    def deint_bwq(src, half, t, nr, chain):
        r32 = a_raw.at[2 + src].bitcast(U32).at[pl.ds(pl.multiple_of(t * nr * 8, 128), nr * 8)]
        dst = bwq_d[half].at[pl.ds(pl.multiple_of(t * (nr // 2), 8), nr // 2)]

        def store(hd, r, v):
            dst[r:r + 8, hd * 128:(hd + 1) * 128] = v

        _deint_block(r32, nr, store, chain)

    def q_step(half, t):
        i = lax.shift_right_logical(t, 1)
        n = lax.bitwise_and(t, 1)
        r0 = pl.multiple_of(i * TQP, TQP)
        c0 = pl.multiple_of(n * 1024, 1024)
        z = _dot(xb[pl.ds(r0, TQP), :], _bf(bwq_d[half][:, pl.ds(c0, 1024)])) * scale2
        z = _u32(z.astype(BF))
        rr = pl.ds(pl.multiple_of(i * (TQP // 2), TQP // 2), TQP // 2)
        for hh in range(8):
            q_all[n * 8 + hh, rr, half * 128:(half + 1) * 128] = z[:, hh * 128:(hh + 1) * 128]
        acct[pl.ds(pl.multiple_of((half * 8 + t) * ZR, ZR), ZR), :] = jnp.zeros((ZR, S + 128), F32)

    def xb_t0(i, carry):
        xb_t(i)
        return carry

    def deint_bwq0(t, carry):
        @pl.when(t == SP)
        def _():
            cp_bwq0[1].wait()
            cp_xb[1].start()

        deint_bwq(0, 0, t, 64, 0)
        return carry

    start([cp_xb[0]] + cp_bwq0)
    cp_xb[0].wait()
    lax.fori_loop(0, 2, xb_t0, 0)
    cp_bwq0[0].wait()
    lax.fori_loop(0, DM // 64, deint_bwq0, 0)
    start([cp_bwq1] + cp_wkv[0])

    DCH = 1

    def deint_kv(t):
        for w_i, raw in enumerate((bwuk_raw, bwuv_raw)):
            for half in range(2):
                r32 = raw.at[half].bitcast(U32).at[pl.ds(pl.multiple_of(t * 1024, 1024), 1024)]
                dst = wkv_d.at[:, pl.ds(pl.multiple_of(t * 64, 64), 64)]

                def store(hd, r, v, c0=w_i * E + half * 128, dst=dst):
                    dst[hd, r:r + 8, c0:c0 + 128] = v

                _deint_block(r32, 128, store, DCH)

    W3 = 4

    QR = DM // 4

    def deint_a(u, nch=2):
        sl = lax.shift_right_logical(u, 2)
        dq = lax.bitwise_and(u, 3)
        r32 = a_raw.at[sl].bitcast(U32).at[pl.ds(pl.multiple_of(dq * (QR * 8), 8), QR * 8)]
        dst = wab32.at[sl].at[pl.ds(pl.multiple_of(dq * (QR // 2), 8), DM * H // 2 - 3 * QR // 2)]

        def store(hd, r, v):
            dst[hd * (DM // 2) + r:hd * (DM // 2) + r + 8, :] = v

        return [_deint_block(r32, QR, store, DCH, range(8 // nch * jq, 8 // nch * (jq + 1))) for jq in range(nch)]

    def q_lo(t, carry):
        q_step(0, t)
        deint_bwq(lax.shift_right_logical(t, 2), 1, lax.bitwise_and(t, 3), DM // 4, DCH)
        j = jnp.minimum(lax.shift_right_logical(t + 1, 1), S // 512 - 1)
        xb_t(2 * j)
        xb_t(2 * j + 1)

        @pl.when(t == W3 - 1)
        def _():
            start(cp_wkv[1] + [cp_c])

        @pl.when(t == 0)
        def _():
            cp_xb[1].wait()

        @pl.when(t == 3)
        def _():
            cp_bwq1.wait()

        return carry

    def q_hi(t, carry):
        q_step(1, t)
        deint_kv(t)
        deint_a(t)

        return carry

    def q_hi_group(g, carry):
        @pl.when(g == 1)
        def _():
            wait(cp_wkv[1])
            start(cp_late[0])

        return lax.fori_loop(4 * g, 4 * g + 4, q_hi, carry)

    lax.fori_loop(0, 8, q_lo, 0)
    wait(cp_wkv[0])
    lax.fori_loop(0, 2, q_hi_group, 0)
    cp_c.wait()

    TQ = 256
    NQ = S // TQ
    HQ = TQ // 2

    def kv_chunk(h, slot, r0, nr, c0=0, c1=2 * E):
        z = _dot(c[pl.ds(r0, nr), :], _bf(wkv_d[h, :, c0:c1]))
        kv[slot, pl.ds(r0 // 2, nr // 2), c0:c1] = _u32(z.astype(BF))

    MAINC = DM // 128 * 128

    def prep_a(p):
        w = lax.shift_right_logical(p, 4)
        r0 = pl.multiple_of(lax.bitwise_and(p, H - 1) * (DM // 2), DM // 2)
        rt = pl.ds(pl.multiple_of(r0 + MAINC // 2, 32), (DM - MAINC) // 2)
        lhs = jnp.concatenate([wab32[2 * w + i, pl.ds(r0, DM // 2), :] for i in range(2)], axis=1)
        rhs = jnp.concatenate([jnp.concatenate([wab32[6 - 2 * w + i, pl.ds(r0, DM // 2), :],
                                                wab32[6 - 2 * w + i, rt, :]], axis=0) for i in range(2)], axis=1)
        z = _dot_nt(_bf(lhs), _bf(rhs)) * jnp.where(w == 1, scale, 1.0)
        z = _u32(z.astype(BF))
        odd = lax.bitwise_and(p, 1)
        t0 = lax.shift_right_logical(p, 1) * 7
        for n in range(3):
            wu[t0 + 4 * odd + n] = z[:, n * 128:(n + 1) * 128]
        own = lax.shift_right_logical(lax.broadcasted_iota(jnp.int32, (DM // 2, 128), 1), 6) == odd
        wu[t0 + 3] = jnp.where(own, z[:, MAINC:MAINC + 128], wu[t0 + 3])

    def xa_t(t):
        cc = pl.ds(pl.multiple_of(t * 128, 128), 128)
        v = xat[:, cc].T
        xa[cc, :] = v
        return _u32(v[112:128, 256:384])

    kv_chunk(0, 0, 0, TQ)
    wait(cp_late[0])
    start(cp_late[1])

    RG = 8
    CHL = [4, 3, 2, 2, 2, 2, 2, 2]

    ND = 4

    gates = {}

    def attention(h, slot, filler, CHS):
        wot_h = bwot[pl.ds(pl.multiple_of(h * DM, DM), DM), :]
        row = lax.broadcasted_iota(jnp.int32, (TQ, HQ), 0)
        col = lax.broadcasted_iota(jnp.int32, (TQ, HQ), 1)
        tri_main = row >= col
        tri_tail = tri_main[0:HQ]
        blocks = list(range(NQ))

        def scores(idx):
            i, b = blocks[idx], idx % 2
            n = (i + 1) * TQ
            nm = n - HQ
            nf = n - TQ
            q = _bf(q_all[h, pl.ds(i * TQ // 2, TQ // 2), :])
            if nf > 0:
                s_buf[b][:, 0:nf] = _dot_nt(q, _bf(kv[slot, pl.ds(0, nf // 2), 0:E]))
            s_mid = _dot_nt(q, _bf(kv[slot, pl.ds(nf // 2, HQ // 2), 0:E]))
            s_buf[b][:, nf:nm] = jnp.where(tri_main, s_mid, NEG)
            s_tail = _dot_nt(q[HQ:TQ], _bf(kv[slot, pl.ds(nm // 2, HQ // 2), 0:E]))
            s_buf[b][HQ:TQ, nm:n] = jnp.where(tri_tail, s_tail, NEG)

        def softmax(idx):
            i, b, CH = blocks[idx], idx % 2, CHS[idx]
            n = (i + 1) * TQ
            nm = n - HQ
            ls = []
            sms = []
            for g in range(TQ // RG):
                ne = nm if g * RG < HQ else n
                rows = slice(g * RG, (g + 1) * RG)
                mx = s_buf[b][rows, 0:128]
                if g == 0:
                    for v in gates.pop(idx, []):
                        mx = pltpu.bitcast(_u32(mx) | _zero_after(v), F32)
                if g >= CH:
                    mx = pltpu.bitcast(_u32(mx) | _zero_after(sms[g - CH]), F32)
                for t in range(1, ne // 128):
                    mx = jnp.maximum(mx, s_buf[b][rows, t * 128:(t + 1) * 128])
                m = jnp.broadcast_to(jnp.max(mx, axis=1, keepdims=True), (RG, 128))
                sm = None
                for t0 in range(0, ne, 256):
                    pgs = []
                    for t in range(t0, min(t0 + 256, ne), 128):
                        pg = jnp.exp2(s_buf[b][rows, t:t + 128] - m)
                        sm = pg if sm is None else sm + pg
                        pgs.append(pg)
                    p_buf[b][rows, t0:t0 + 128 * len(pgs)] = jnp.concatenate(pgs, axis=1).astype(BF)
                sms.append(sm)
                ls.append(jnp.sum(sm, axis=1, keepdims=True))
            return jnp.concatenate(ls, axis=0)

        def context(idx, l):
            i, b = blocks[idx], idx % 2
            n = (i + 1) * TQ
            nm = n - HQ
            ctx = _dot(p_buf[b][:, 0:nm], _bf(kv[slot, pl.ds(0, nm // 2), E:2 * E]))
            ctx_t = _dot(p_buf[b][HQ:TQ, nm:n], _bf(kv[slot, pl.ds(nm // 2, HQ // 2), E:2 * E]))
            ctx = jnp.concatenate([ctx[0:HQ], ctx[HQ:TQ] + ctx_t], axis=0)
            return (ctx * (1.0 / l)).astype(BF)

        def out_proj(idx, ctx):
            acct[PADL:PADL + DM, pl.ds(blocks[idx] * TQ, TQ)] += _dot_nt(wot_h, ctx)

        filler(-1)
        scores(0)
        ctx = None
        for idx in range(NQ):
            l = softmax(idx)
            filler(idx)
            if idx + 1 < NQ:
                scores(idx + 1)
            if ctx is not None:
                out_proj(idx - 1, ctx)
            ctx = context(idx, l)
            if idx >= NQ - ND:
                q_all[h, pl.ds(idx * TQ // 2, TQ // 2), :] = _u32(ctx)
                ctx = None

    def head(h, carry):
        slot = lax.bitwise_and(h, 1)
        hn = jnp.minimum(h + 1, H - 1)

        def filler(idx):
            if idx < 0:
                kv_chunk(h, slot, TQ, TQ, 0, E)
            elif idx == 0:
                kv_chunk(h, slot, TQ, TQ, E, 2 * E)
            elif idx < NQ - 1:
                kv_chunk(h, slot, (idx + 1) * TQ, TQ)
            else:
                kv_chunk(hn, 1 - slot, 0, TQ)
            if idx < 0:
                u0 = 8 + 2 * jnp.minimum(h, 7)
                gates[2] = deint_a(u0, 1)
                gates[4] = deint_a(u0 + 1, 1)
                gates[6] = [xa_t(h)]
            if idx == NQ - 1:
                prep_a(2 * h + 1)
            if idx == NQ - 2:
                prep_a(2 * h)

        attention(h, slot, filler, CHL)
        return carry

    def head_group(g, carry):
        @pl.when(g == 1)
        def _():
            wait(cp_late[1])

        return lax.fori_loop(g * HG, HG + g * (H - HG), head, carry)

    lax.fori_loop(0, 2, head_group, 0)

    NPRE = 8

    def b_piece(p):
        al = (lambda v, m: v) if isinstance(p, int) else pl.multiple_of
        hh = p & (H - 1)
        q0 = S - ND * TQ + (p >> 4) * 128
        qr = q0 if isinstance(p, int) else jnp.minimum(q0, S - 128)
        ctx = _bf(q_all[hh, pl.ds(al(qr >> 1, 64), 64), :])
        for m0 in range(0, DM, DM // 2):
            acct[PADL + m0:PADL + m0 + DM // 2, pl.ds(al(q0, 128), 128)] += _dot_nt(
                bwot[pl.ds(al(hh * DM + m0, DM // 2), DM // 2), :], ctx)

    for p in range(NPRE):
        b_piece(p)

    L = 48
    LV = M + SEG
    PR = 2 * SEG
    XE = 40
    XO = PR - XE
    NP = NSEG // 2
    OC = 2
    NOC = NP // OC
    ORS = OC * PR
    NT_ = (H + 2) // 3

    for T in range(NT_):
        r = T * 128 + LV * min(3, H - 3 * T)
        ua[:, r:r + 8, :] = jnp.zeros((2, 8, 512), BF)
        ya[:, r:r + 8, :] = jnp.zeros((2, 8, 512), BF)
    mem[...] = mem0_ref[...].astype(F32)

    def out_copy(k):
        r = pl.ds(pl.multiple_of(k * ORS, ORS), ORS)
        return pltpu.make_async_copy(obuf.at[r, :], out_hbm.at[r, :], sems.at[10])

    def b_out(t):
        r = pl.ds(pl.multiple_of(lax.shift_right_logical(t, 1) * 128, 128), 128)
        f0 = pl.multiple_of(lax.bitwise_and(t, 1) * 256, 256)
        blk = acct[pl.ds(f0, 256), r].astype(BF)
        obuf[r, pl.ds(pl.multiple_of(DM - PADL + f0, 128), 256)] = blk.T

    def substep(odd, seg, r0, mask, filler, last):
        cur = int(odd)
        nx = XO if odd else XE
        x0 = XE if odd else 0
        R = nx + M

        def scatter(dst, z, base=0, cols=slice(None)):
            if odd:
                dst[1, base + XE - SEG:base + SEG, cols] = z[0:XO].astype(BF)
            else:
                dst[0, base:base + SEG, cols] = z[0:SEG].astype(BF)
                dst[1, base:base + XE - SEG, cols] = z[SEG:XE].astype(BF)
            dst[cur, base + SEG:base + LV, cols] = z[nx:R].astype(BF)

        lane_hi = lax.broadcasted_iota(jnp.int32, (R, 128), 1) >= 64

        def project(dst, n0):
            z = _dot(lhs, _bf(jnp.concatenate([wu[n0 + n] for n in range(H // 2 * 7)], axis=1)))
            for h in range(H):
                base = h // 3 * 128 + h % 3 * LV
                c0 = (h // 2 * 7 + h % 2 * 4) * 128
                zt = z[:, (h // 2 * 7 + 3) * 128:(h // 2 * 7 + 4) * 128]
                scatter(dst, z[:, c0:c0 + MAINC], base, slice(0, MAINC))
                scatter(dst, jnp.where(lane_hi, zt, 0.0) if h % 2 else jnp.where(lane_hi, 0.0, zt),
                        base, slice(MAINC, 512))

        memv = mem[...]
        lhs = jnp.concatenate([xa[pl.ds(r0 + x0, nx), :].astype(F32), memv], axis=0).astype(BF)
        hk = jnp.concatenate([xa[pl.ds(pl.multiple_of(r0 + cur * SEG, SEG), SEG), :].astype(F32), memv,
                              jnp.zeros((L - LV, DM), F32)], axis=0)
        hk = jnp.concatenate([hk, hk[:, MAINC:DM]], axis=1).astype(BF)
        project(ya, H // 2 * 7)
        st = [_dot_nt(hk, ya[cur, T * 128:min(T * 128 + 128, ya.shape[1]), :]) for T in range(NT_)]
        project(ua, 0)
        pts = []
        for T in range(NT_):
            w = st[T].shape[1]
            sc = jnp.where(mask[:, 0:w], st[T], NEG)
            e = jnp.exp(sc - jnp.max(sc, axis=0, keepdims=True))
            e = e * (1.0 / jnp.sum(e, axis=0, keepdims=True))
            if w < 128:
                e = jnp.concatenate([e, jnp.zeros((L, 128 - w), F32)], axis=1)
            pt = jnp.concatenate([e, jnp.zeros((128 - L, 128), F32)], axis=0).T
            if w < 128:
                pts.append(pt[0:LV, 0:L].astype(BF))
            else:
                pts.append(jnp.concatenate([pt[r * LV:(r + 1) * LV, 0:LV] for r in range(3)]
                                           + [jnp.zeros((LV, 128 - 3 * LV), F32)], axis=1).astype(BF))
        filler()
        b_piece(2 * seg + NPRE)
        a = functools.reduce(lambda x, y: x + y, [
            _dot(pt, ua[cur, T * 128:T * 128 + pt.shape[1], :]) for T, pt in enumerate(pts)])
        tail, main = a[:, MAINC:512], a[:, 0:MAINC]
        o = jnp.concatenate([main, tail[:, 0:64] + tail[:, 64:128]], axis=1)
        mem[...] = o[SEG:LV]
        last()
        obuf[pl.ds(pl.multiple_of(r0 + cur * SEG, SEG), SEG), 0:DM] = o[0:SEG].astype(BF)
        b_piece(2 * seg + NPRE + 1)

    def pair(t, carry):
        key = lax.broadcasted_iota(jnp.int32, (L, 128), 0)
        lane = lax.broadcasted_iota(jnp.int32, (L, 128), 1)
        qry = lane - jnp.where(lane >= 2 * LV, 2 * LV, jnp.where(lane >= LV, LV, 0))
        mask = (key < LV) & ((qry >= SEG) | (key >= SEG) | (key <= qry))
        r0 = pl.multiple_of(t * PR, PR)

        def flush():
            @pl.when(jnp.logical_and(lax.bitwise_and(t, OC - 1) == 0, t > 0))
            def _():
                out_copy(lax.shift_right_logical(t, 1) - 1).start()

        substep(False, 2 * t, r0, mask, lambda: b_out(t), lambda: None)
        substep(True, 2 * t + 1, r0, mask, lambda: None, flush)
        return carry

    lax.fori_loop(0, NP, pair, 0)
    out_copy(NOC - 1).start()
    for k in range(NOC):
        out_copy(k).wait()


@functools.partial(jax.jit, static_argnames=("A_seg_len",))
def pallas_concat_heads__memory_aug_recurrent_mem_tr__compressed_kv_cla__prompt_kernel(
    A_x, A_mem0, A_Wq, A_Wk, A_Wv, A_Wo, A_seg_len,
    B_x, B_c_kv, B_w_q, B_w_uk, B_w_uv, B_w_o,
):
    _, S, DM = A_x.shape
    _, H, E = A_Wq.shape
    M = A_mem0.shape[1]
    DC = B_c_kv.shape[2]
    SEG = int(A_seg_len)
    assert (S, DM, H, E, M, DC, SEG) == (2048, 448, 16, 256, 8, 1024, 32)
    HE = H * E
    any_spec = pl.BlockSpec(memory_space=pl.ANY)
    vm = pltpu.VMEM
    scratch = [
        vm((DM, S), BF), vm((S, DM), BF), vm((S, DC), BF),
        vm((2, DC * H, 128), BF), vm((2, DC * H, 128), BF),
        vm((H * DM, E), BF),
        vm((DM // 2, HE // 2), U32), vm((DM // 2, HE // 2), U32),
        vm((H, DC // 2, 2 * E), U32),
        vm((H, S // 2, E), U32), vm((2, S // 2, 2 * E), U32),
        vm((512, S + 128), F32),
        vm((256, S), F32), vm((256, S), F32), vm((256, S), BF), vm((256, S), BF),
        vm((S, DM), BF),
        vm((6, DM * H, 128), BF), vm((8, DM * H, 128), BF),
        vm((H * 7, DM // 2, 128), U32),
        vm((M, DM), F32),
        vm((2, 688, 512), BF), vm((2, 688, 512), BF),
        vm((S, 2 * DM), BF),
        pltpu.SemaphoreType.DMA((11,)),
    ]
    out = pl.pallas_call(
        functools.partial(_kernel, S=S, DM=DM, H=H, E=E, DC=DC, M=M, SEG=SEG),
        out_shape=jax.ShapeDtypeStruct((S, 2 * DM), BF),
        in_specs=[any_spec, pl.BlockSpec(memory_space=pltpu.VMEM)] + [any_spec] * 10,
        out_specs=any_spec,
        scratch_shapes=scratch,
        compiler_params=pltpu.CompilerParams(vmem_limit_bytes=126 * 1024 * 1024),
    )(
        jnp.swapaxes(A_x, 1, 2).reshape(DM, S), A_mem0.reshape(M, DM),
        A_Wq.reshape(DM * H, E), A_Wk.reshape(DM * H, E), A_Wv.reshape(DM * H, E),
        jnp.swapaxes(A_Wo, 1, 2).reshape(H * DM, E),
        jnp.swapaxes(B_x, 1, 2).reshape(DM, S), B_c_kv.reshape(S, DC),
        B_w_q.reshape(DM * H, E), B_w_uk.reshape(DC * H, E), B_w_uv.reshape(DC * H, E),
        jnp.swapaxes(B_w_o, 1, 2).reshape(H * DM, E),
    )
    return out.reshape(1, S, 2 * DM)
```
